```python
import jax
import jax.numpy as jnp

def _softmax(x, axis=-1):
    return jax.nn.softmax(x, axis=axis)
def _gelu(x):
    return jax.nn.gelu(x, approximate=True)
def _silu(x):
    return jax.nn.silu(x)
def _sigmoid(x):
    return jax.nn.sigmoid(x)
def _layernorm(x, axis=-1, eps=1e-5):
    m = jnp.mean(x, axis=axis, keepdims=True)
    v = jnp.var(x, axis=axis, keepdims=True)
    return (x - m) / jnp.sqrt(v + eps)
def _scatter_add(tgt, idx, src, axis=0):
    return tgt.at[idx].add(src)
def _segment_sum(src, seg, n):
    return jax.ops.segment_sum(src, seg, n)
class _Rng:
    def __init__(self, key):
        self._k = key
    def _next(self):
        self._k, sub = jax.random.split(self._k)
        return sub
    def normal(self, shape):
        return jax.random.normal(self._next(), shape, dtype=jnp.bfloat16)
    def randint(self, lo, hi, shape):
        return jax.random.randint(self._next(), shape, lo, hi, dtype=jnp.int32)
    def uniform(self, shape, lo=0.0, hi=1.0):
        return jax.random.uniform(self._next(), shape, jnp.bfloat16, lo, hi)
    def permutation(self, n):
        return jax.random.permutation(self._next(), n)


kernel_name = 'standalone__seq2seq_rnn_t_joint__speech'

def setup_inputs():
    _rng = _Rng(jax.random.key(int.from_bytes(__import__("os").urandom(4), "little")))
    _w = (lambda a: (lambda t: t.astype(jnp.bfloat16) if jnp.issubdtype(t.dtype, jnp.floating) else t)(jnp.asarray(a)))
    B, T, D, K = 2, 16000, 256, 31
    U = 8
    sc = (1.0 / (K * D)) ** 0.5
    sd = (1.0 / D) ** 0.5
    return {
        "x": _w((lambda *s: _rng.normal(s) * 0.05)(B, T, D) * 0.5),
        "w1": _w((lambda *s: _rng.normal(s) * 0.05)(K, D, D) * sc),
        "w2": _w((lambda *s: _rng.normal(s) * 0.05)(K, D, D) * sc),
        "g": _w((lambda *s: _rng.normal(s) * 0.05)(B, U, D) * 0.5),
        "w_f": _w((lambda *s: _rng.normal(s) * 0.05)(D, D) * sd),
        "w_g": _w((lambda *s: _rng.normal(s) * 0.05)(D, D) * sd),
        "w_o": _w((lambda *s: _rng.normal(s) * 0.05)(D, D) * sd),
    }

def reference(x, w1, w2, g, w_f, w_g, w_o):
    B, T, D = x.shape
    K = w1.shape[0]
    pad = K // 2
    xp = jnp.pad(x, ((0,0),(pad,pad),(0,0)))
    h = jnp.zeros_like(x)
    for i in range(K):
        h = h + jnp.einsum("btc,cd->btd", xp[:, i:i+T, :], w1[i])
    h = _gelu(h)[:, ::2, :]
    T1 = h.shape[1]
    hp = jnp.pad(h, ((0,0),(pad,pad),(0,0)))
    f = jnp.zeros_like(h)
    for i in range(K):
        f = f + jnp.einsum("btc,cd->btd", hp[:, i:i+T1, :], w2[i])
    f = _gelu(f)[:, ::2, :]
    fe = jnp.einsum("btd,de->bte", f, w_f)
    ge = jnp.einsum("bud,de->bue", g, w_g)
    j = jnp.tanh(fe[:, :, None, :] + ge[:, None, :, :])
    return jnp.einsum("btud,dv->btuv", j, w_o)
```

```python
import functools
import math

import numpy as np

import jax
import jax.numpy as jnp
from jax import lax
import jax.experimental.pallas as pl
import jax.experimental.pallas.tpu as pltpu


class _Prog:
    def __init__(self):
        self.ops = []
        self.cse = {}

    def _node(self, kind, a, b):
        key = (kind, a, b)
        if key not in self.cse:
            self.ops.append(key)
            self.cse[key] = len(self.ops) - 1
        return self.cse[key]

    def inp(self, i):
        return (self._node("in", i, None), 1)

    def neg(self, x):
        return None if x is None else (x[0], -x[1])

    def add(self, x, y):
        if x is None:
            return y
        if y is None:
            return x
        (a, sa), (b, sb) = x, y
        if sa == sb:
            return (self._node("add", min(a, b), max(a, b)), sa)
        if sa > 0:
            return (self._node("sub", a, b), 1)
        return (self._node("sub", b, a), 1)

    def sub(self, x, y):
        return self.add(x, self.neg(y))

    def mul(self, c, x):
        if x is None or c == 0:
            return None
        if c == 1:
            return x
        if c == -1:
            return self.neg(x)
        return (self._node("mul", x[0], abs(float(c))), x[1] * (1 if c > 0 else -1))

    def cadd(self, z, w):
        return (self.add(z[0], w[0]), self.add(z[1], w[1]))

    def csub(self, z, w):
        return (self.sub(z[0], w[0]), self.sub(z[1], w[1]))

    def cconj(self, z):
        return (z[0], self.neg(z[1]))

    def twiddle(self, z, num, den):
        num %= den
        a, b = z
        if (8 * num) % den == 0:
            e = (8 * num) // den
            r = math.sqrt(0.5)
            if e == 0:
                return (a, b)
            if e == 2:
                return (b, self.neg(a))
            if e == 4:
                return (self.neg(a), self.neg(b))
            if e == 6:
                return (self.neg(b), a)
            if e == 1:
                return (self.mul(r, self.add(a, b)), self.mul(r, self.sub(b, a)))
            if e == 3:
                return (self.mul(r, self.sub(b, a)), self.mul(-r, self.add(a, b)))
            if e == 5:
                return (self.mul(-r, self.add(a, b)), self.mul(r, self.sub(a, b)))
            return (self.mul(r, self.sub(a, b)), self.mul(r, self.add(a, b)))
        th = -2.0 * math.pi * num / den
        c, s = math.cos(th), math.sin(th)
        return (self.sub(self.mul(c, a), self.mul(s, b)), self.add(self.mul(s, a), self.mul(c, b)))

    def rfft(self, xs):
        n = len(xs)
        if n == 1:
            return [(xs[0], None)]
        if n == 2:
            return [(self.add(xs[0], xs[1]), None), (self.sub(xs[0], xs[1]), None)]
        if n == 4:
            a = self.add(xs[0], xs[2])
            b = self.sub(xs[0], xs[2])
            c = self.add(xs[1], xs[3])
            d = self.sub(xs[1], xs[3])
            return [(self.add(a, c), None), (b, self.neg(d)), (self.sub(a, c), None)]
        u = self.rfft(xs[0::2])
        z1 = self.rfft(xs[1::4])
        z3 = self.rfft(xs[3::4])

        def get_u(k):
            k %= n // 2
            return u[k] if k <= n // 4 else self.cconj(u[n // 2 - k])

        out = [None] * (n // 2 + 1)
        for k in range(n // 8 + 1):
            t1 = self.twiddle(z1[k], k, n)
            t3 = self.twiddle(z3[k], 3 * k, n)
            sm = self.cadd(t1, t3)
            df = self.csub(t1, t3)
            u0, u1 = get_u(k), get_u(k + n // 4)
            out[k] = self.cadd(u0, sm)
            out[n // 2 - k] = self.cconj(self.csub(u0, sm))
            mdf = (df[1], self.neg(df[0]))
            out[k + n // 4] = self.cadd(u1, mdf)
            if k > 0:
                out[n // 4 - k] = self.cconj(self.csub(u1, mdf))
        return out

    def order(self, outs):
        seen, order = set(), []
        for o in outs:
            if o is None or o[0] in seen:
                continue
            stack = [(o[0], False)]
            while stack:
                n, done = stack.pop()
                if done:
                    order.append(n)
                    continue
                if n in seen:
                    continue
                seen.add(n)
                stack.append((n, True))
                kind, a, b = self.ops[n]
                if kind in ("add", "sub"):
                    stack.append((b, False))
                    stack.append((a, False))
                elif kind == "mul":
                    stack.append((a, False))
        return order

    def transpose(self, outs):
        g = _Prog()
        adj = {}

        def acc(n, v):
            if v is not None:
                adj[n] = g.add(adj.get(n), v)

        for i, o in enumerate(outs):
            if o is not None:
                acc(o[0], g.mul(o[1], g.inp(i)))
        res = {}
        for n in sorted(set(self.order(outs)), reverse=True):
            kind, a, b = self.ops[n]
            v = adj.get(n)
            if v is None:
                continue
            if kind == "in":
                res[a] = v
            elif kind == "add":
                acc(a, v)
                acc(b, v)
            elif kind == "sub":
                acc(a, v)
                acc(b, g.neg(v))
            else:
                acc(a, g.mul(b, v))
        return g, res

    def run(self, outs, load, emit, keep_sign=True):
        val = {}
        want = {}
        for i, o in enumerate(outs):
            if o is not None:
                want.setdefault(o[0], []).append((i, o[1]))
        for n in self.order(outs):
            kind, a, b = self.ops[n]
            if kind == "in":
                v = load(a)
            elif kind == "add":
                v = val[a] + val[b]
            elif kind == "sub":
                v = val[a] - val[b]
            else:
                v = val[a] * np.float32(b)
            val[n] = v
            for i, sg in want.get(n, ()):
                emit(i, -v if (sg < 0 and keep_sign) else v)


def _lhs_outputs(p, spec, n):
    outs = [spec[0][0], spec[n // 2][0]]
    for k in range(1, n // 2):
        a, b = spec[k]
        outs += [p.add(a, b), a, b]
    return outs


class _Plan:
    def __init__(self, n):
        self.n = n
        self.taps = 16
        self.hop = n - self.taps + 1
        self.ns = 2 + 3 * (n // 2 - 1)
        self.fwd = _Prog()
        spec = self.fwd.rfft([self.fwd.inp(i) for i in range(n)])
        self.fwd_outs = _lhs_outputs(self.fwd, spec, n)
        lhs_sign = [o[1] for o in self.fwd_outs]
        p = _Prog()
        spec = p.rfft([p.inp(i) if i < self.hop else None for i in range(n)])
        self.inv, res = p.transpose(_lhs_outputs(p, spec, n))
        self.inv_outs = [res[t] for t in range(self.hop)]
        self.inv_src = [0, 1]
        for k in range(n // 2 - 1):
            base = 2 + 3 * k
            self.inv_src += [base, base + 2, base + 1]
        self.wprog, self.wouts, self.wtap = [], [], []
        for ph in range(2):
            p = _Prog()
            xs = [None] * n
            for j in range(self.taps):
                if not (ph == 0 and j == 0):
                    xs[j] = p.inp(2 * j - 1 if ph == 0 else 2 * j)
            spec = p.rfft(xs)
            outs = [p.mul(0.5, spec[0][0]), p.mul(0.5, spec[n // 2][0])]
            for k in range(1, n // 2):
                c, dm = spec[k]
                d = p.neg(dm)
                outs += [c, p.sub(d, c), p.neg(p.add(c, d))]
            outs = [(o[0], o[1] * s) for o, s in zip(outs, lhs_sign)]
            self.wprog.append(p)
            self.wouts.append(outs)


_FFT_N = 32
_PLAN = _Plan(_FFT_N)

_C0 = math.sqrt(2.0 / math.pi)
_KAPPA = 0.044715 / (_C0 * _C0)


def _gelu2(z):
    inner = z * (np.float32(_KAPPA) * (z * z) + np.float32(1.0))
    return z + z * jnp.tanh(inner)


_B, _T, _D, _K, _U = 2, 16000, 256, 31, 8
_T1, _T2 = _T // 2, _T // 4
_S2 = 502
_S1 = 2 * _S2
_HOP = _PLAN.hop
_NS = _PLAN.ns
_CB1, _NSTEP1 = 8, 8
_CB2, _NSTEP2 = 5, 6
_CBMAX = max(_CB1, _CB2)
_XOFF = 24
_XROWS = -(-(7 * _S1 + _HOP * (_CB1 * _NSTEP1 - 1) + _FFT_N) // 8) * 8
_HOFF = _CB1 * _HOP
_HROWS = _HOFF + _HOP * _CB1 * _NSTEP1
_FROWS = _HOP * _CB2 * _NSTEP2
_TJ = _HOP
_XPARTS = 4


def _x_piece_bounds():
    edges = []
    for s in range(8):
        for p in range(_XPARTS):
            edges.append(min(max((s * _S1 + p * (_S1 // _XPARTS) - _XOFF) // 8 * 8, 0), _T1))
    edges.append(_T1)
    edges[0] = 0
    return edges


def _kernel(x_hbm, w1_hbm, w2_hbm, g_hbm, wf_hbm, wg_hbm, wo_hbm, out_hbm,
            v1, v2, spec_a, spec_b, y_a, y_b, hbuf, xbuf, w1buf, w2buf,
            gbuf, wfbuf, wgbuf, wobuf, gebuf, fbuf, obuf,
            sem_w, sem_x, sem_o):
    plan = _PLAN
    n, hop, ns = plan.n, plan.hop, plan.ns

    xu = x_hbm.bitcast(jnp.uint32)
    edges = _x_piece_bounds()

    def x_copies(part):
        cps = []
        for s in range(8):
            r0, r1 = edges[s * _XPARTS + part], edges[s * _XPARTS + part + 1]
            for bb in range(2):
                for cs in range(2):
                    cps.append(pltpu.make_async_copy(
                        xu.at[bb, pl.ds(r0, r1 - r0), pl.ds(cs * 128, 128)],
                        xbuf.at[bb, cs, pl.ds(_XOFF + r0, r1 - r0), :],
                        sem_x.at[part]))
        return cps

    small = [pltpu.make_async_copy(src, dst, sem_w.at[2 + i]) for i, (src, dst) in
             enumerate([(g_hbm, gbuf), (wf_hbm, wfbuf), (wg_hbm, wgbuf), (wo_hbm, wobuf)])]
    cp_w1 = pltpu.make_async_copy(w1_hbm, w1buf, sem_w.at[0])
    cp_w2 = pltpu.make_async_copy(w2_hbm, w2buf, sem_w.at[1])

    cp_w1.start()
    zero8 = jnp.zeros((8, 128), jnp.uint32)
    for bb in range(2):
        for cs in range(2):
            for r in range(0, _XOFF, 8):
                xbuf[bb, cs, pl.ds(r, 8), :] = zero8
            for r in range(_XOFF + _T1, _XROWS, 8):
                xbuf[bb, cs, pl.ds(r, 8), :] = zero8
    for c in x_copies(0):
        c.start()

    def weight_transform(wbuf, vbuf, scale):
        def body(rg, carry):
            row = pl.multiple_of(rg * 16, 16)
            for ph in range(2):
                for nt in range(2):
                    def load(tap):
                        w = wbuf[tap, pl.ds(row, 16), pl.ds(nt * 128, 128)]
                        return w.astype(jnp.float32) * np.float32(scale)

                    def emit(i, v):
                        vbuf[i, nt, pl.ds(pl.multiple_of(ph * 256 + row, 16), 16), :] = (
                            v.astype(jnp.bfloat16))
                    plan.wprog[ph].run(plan.wouts[ph], load, emit)
            return carry
        lax.fori_loop(0, _D // 16, body, 0)

    cp_w1.wait()
    for c in x_copies(1):
        c.start()
    weight_transform(w1buf, v1, (2.0 / n) * _C0)

    def fwd_unit(load_in, spec, row, col, deps=(), mask=None):
        cnt = [0]

        def load(q):
            v = load_in(q, None)
            j, rem = divmod(cnt[0] * len(deps), n)
            cnt[0] += 1
            if deps and rem < len(deps):
                v = load_in(q, (mask, deps[j]))
            return v

        def emit(i, v):
            spec[i, pl.ds(row, 8), pl.ds(col, 128)] = v
        plan.fwd.run(plan.fwd_outs, load, emit, keep_sign=False)

    def x_loader(bb, cs, ph, base):
        def load_in(q, dep):
            v = xbuf[bb, cs, pl.ds(base + q, 8, stride=_S1), :]
            if dep is not None:
                v = jnp.where(dep[0], v, lax.bitcast_convert_type(dep[1](), jnp.uint32))
            v = (v << 16) if ph == 0 else (v & jnp.uint32(0xFFFF0000))
            return lax.bitcast_convert_type(v, jnp.float32)
        return load_in

    def h_loader(bb, cs, ph, base):
        def load_in(q, dep):
            v = hbuf[base + 2 * q + ph, pl.ds(bb * 8, 8), pl.ds(cs * 128, 128)]
            if dep is not None:
                v = jnp.where(dep[0], v, dep[1]())
            return v
        return load_in

    def inv_unit(ybuf, row, col, store, deps=(), mask=None):
        cnt = [0]

        def load(i):
            v = ybuf[plan.inv_src[i], pl.ds(row, 8), pl.ds(col, 128)]
            j, rem = divmod(cnt[0] * len(deps), ns)
            cnt[0] += 1
            if deps and rem < len(deps):
                v = jnp.where(mask, v, deps[j]())
            return v
        plan.inv.run(plan.inv_outs, load, store)

    def conv_step(cb, vbuf, sa, ya, sb, yb, fwd_fn, inv_fn, mask):
        m = cb * 16
        fw = [("f", be, bb, cs, ph) for be in range(cb) for bb in range(2)
              for cs in range(2) for ph in range(2)]
        iv = [("i", be, bb, nt) for be in range(cb) for bb in range(2) for nt in range(2)]
        merged, ia, ib = [], 0, 0
        while ia < len(fw) or ib < len(iv):
            if ib >= len(iv) or (ia < len(fw) and (ia + 0.5) / len(fw) <= (ib + 0.5) / len(iv)):
                merged.append(fw[ia]); ia += 1
            else:
                merged.append(iv[ib]); ib += 1
        ndep = 2
        g8 = m // 8
        nev = 2 * ns * g8 * 2
        cost = lambda u: 262 if u[0] == "f" else 350
        tot = sum(cost(u) for u in merged)
        sched, cum = [], 0
        for u in merged:
            evs = [min(int((cum + cost(u) * q / ndep) / tot * (nev - 40)) + 1, nev - 1)
                   for q in range(ndep)]
            cum += cost(u)
            sched.append((u, evs))
        results = {}

        def event(e):
            j, v = divmod(e, g8 * 2)
            rg, nn = divmod(v, 2)
            return results[j][rg * 8:(rg + 1) * 8, nn * 128:(nn + 1) * 128]

        pi = 0
        for i in range(ns):
            for h in range(2):
                w = jnp.concatenate([vbuf[i, 0, pl.ds(h * 256, 256), :],
                                     vbuf[i, 1, pl.ds(h * 256, 256), :]], axis=1)
                results[2 * i + h] = jnp.dot(sa[i, pl.ds(0, m), pl.ds(h * 256, 256)], w,
                                             preferred_element_type=jnp.float32)
                while pi < len(sched) and max(sched[pi][1]) // (g8 * 2) <= 2 * i + h:
                    u, evs = sched[pi]
                    pi += 1
                    deps = [functools.partial(event, e) for e in evs]
                    if u[0] == "f":
                        fwd_fn(sb, u[1], u[2], u[3], u[4], deps, mask)
                    else:
                        inv_fn(yb, u[1], u[2], u[3], deps, mask)
            ya[i, pl.ds(0, m), :] = results[2 * i] + results[2 * i + 1]

    def conv_phase(cb, nstep, vbuf, fwd_of, inv_of, pre_iter):
        def fill(u, carry):
            be, bb = u // 2, u % 2
            f = fwd_of(0, 0)
            for cs in range(2):
                for ph in range(2):
                    f(spec_a, be, bb, cs, ph)
            return carry
        lax.fori_loop(0, cb * 2, fill, 0)

        def body(it, carry):
            pre_iter(it)
            zd = (it * (it + 1)) & 1
            mask = jnp.full((8, 128), zd, jnp.int32) == 0
            c = 2 * it

            def s0(_, cc):
                conv_step(cb, vbuf, spec_a, y_a, spec_b, y_b,
                          fwd_of(c + 1, zd), inv_of(c - 1), mask)
                return cc

            def s1(_, cc):
                conv_step(cb, vbuf, spec_b, y_b, spec_a, y_a,
                          fwd_of(jnp.minimum(c + 2, nstep - 1), zd), inv_of(c), mask)
                return cc
            lax.fori_loop(0, 1 + zd, s0, 0)
            lax.fori_loop(0, 1 + zd, s1, 0)
            return carry
        lax.fori_loop(0, nstep // 2, body, 0)

        def drain(u, carry):
            be, bb = u // 2, u % 2
            f = inv_of(nstep - 1)
            for nt in range(2):
                f(y_b, be, bb, nt)
            return carry
        lax.fori_loop(0, cb * 2, drain, 0)

    def dyn8(v):
        return v if isinstance(v, int) else pl.multiple_of(v, 8)

    def fwd1_of(chunk, zd):
        def f(spec, be, bb, cs, ph, deps=(), mask=None):
            base = (chunk * _CB1 + be) * hop
            if ph == 1:
                base = base + zd
            fwd_unit(x_loader(bb, cs, ph, base), spec, dyn8(be * 16 + bb * 8),
                     ph * 256 + cs * 128, deps, mask)
        return f

    def inv1_of(chunk):
        def f(ybuf, be, bb, nt, deps=(), mask=None):
            base = _HOFF + (chunk * _CB1 + be) * hop

            def store(t, z):
                hbuf[base + t, pl.ds(dyn8(bb * 8), 8), pl.ds(nt * 128, 128)] = _gelu2(z)
            inv_unit(ybuf, dyn8(be * 16 + bb * 8), nt * 128, store, deps, mask)
        return f

    def pre1(it):
        for p in range(1, _XPARTS):
            @pl.when(it == p - 1)
            def _():
                for c in x_copies(p):
                    c.wait()

    for c in x_copies(0):
        c.wait()
    cp_w2.start()
    for p in range(2, _XPARTS):
        for c in x_copies(p):
            c.start()
    for c in small:
        c.start()
    conv_phase(_CB1, _NSTEP1, v1, fwd1_of, inv1_of, pre1)

    sub = lax.broadcasted_iota(jnp.int32, (16, 256), 0) % 8

    def mask_lo(r, carry):
        hbuf[_HOFF + r] = jnp.where(sub == 0, 0.0, hbuf[_HOFF + r])
        return carry
    lax.fori_loop(0, 16, mask_lo, 0)
    hi0 = _T1 - 7 * _S1 + 16

    def mask_hi(r, carry):
        hbuf[_HOFF + hi0 + r] = jnp.where(sub == 7, 0.0, hbuf[_HOFF + hi0 + r])
        return carry
    lax.fori_loop(0, _HROWS - _HOFF - hi0, mask_hi, 0)

    cp_w2.wait()
    weight_transform(w2buf, v2, (2.0 / n) * 0.5)

    def fwd2_of(chunk, zd):
        def f(spec, be, bb, cs, ph, deps=(), mask=None):
            base = _HOFF + (chunk * _CB2 + be) * 2 * hop
            fwd_unit(h_loader(bb, cs, ph, base), spec, dyn8(be * 16 + bb * 8),
                     ph * 256 + cs * 128, deps, mask)
        return f

    def inv2_of(chunk):
        def f(ybuf, be, bb, nt, deps=(), mask=None):
            base = _CB2 * hop + (chunk * _CB2 + be) * hop

            def store(t, z):
                fbuf[base + t, pl.ds(dyn8(bb * 8), 8), pl.ds(nt * 128, 128)] = (
                    _gelu2(z) * np.float32(0.5 / _C0))
            inv_unit(ybuf, dyn8(be * 16 + bb * 8), nt * 128, store, deps, mask)
        return f

    conv_phase(_CB2, _NSTEP2, v2, fwd2_of, inv2_of, lambda it: None)

    for c in small:
        c.wait()
    foff = _CB2 * hop
    gebuf[...] = jnp.dot(gbuf[...].reshape(_B * _U, _D), wgbuf[...],
                         preferred_element_type=jnp.float32).reshape(_B, _U, _D)

    def fe_body(i, carry):
        r0 = foff + i * hop
        f = fbuf[pl.ds(r0, hop)].reshape(hop * 16, _D)
        fbuf[pl.ds(r0, hop)] = jnp.dot(
            f, wfbuf[...], preferred_element_type=jnp.float32).reshape(hop, 16, _D)
        return carry
    lax.fori_loop(0, _FROWS // hop, fe_body, 0)

    def out_copies(slot, t0, rows_of):
        cps = []
        for r in range(16):
            bb, s = divmod(r, 8)
            rows = rows_of(s)
            if rows > 0:
                cps.append(pltpu.make_async_copy(
                    obuf.at[slot, r, pl.ds(0, rows)],
                    out_hbm.at[bb, pl.ds(s * _S2 + t0, rows)],
                    sem_o.at[slot]))
        return cps

    def joint_tile(slot, t0, tj):
        rows = []
        for tt in range(tj):
            for r in range(16):
                fr = fbuf[foff + t0 + tt, pl.ds(r, 1), :]
                rows.append(jnp.tanh(jnp.broadcast_to(fr, (_U, _D)) + gebuf[r // 8]))
        j = jnp.concatenate(rows, axis=0)
        o = jnp.dot(j, wobuf[...], preferred_element_type=jnp.float32)
        o = o.reshape(tj, 16, _U, _D).astype(jnp.bfloat16)
        for tt in range(tj):
            obuf[slot, :, tt] = o[tt]

    full = lambda s: _TJ
    nfull = (_T2 - 7 * _S2) // _TJ
    assert nfull % 2 == 0

    def joint_body(i2, carry):
        for slot in range(2):
            t0 = (2 * i2 + slot) * _TJ

            @pl.when(i2 > 0)
            def _():
                for c in out_copies(slot, t0 - 2 * _TJ, full):
                    c.wait()
            joint_tile(slot, t0, _TJ)
            for c in out_copies(slot, t0, full):
                c.start()
        return carry
    lax.fori_loop(0, nfull // 2, joint_body, 0)

    ntiles = -(-_S2 // _TJ)
    pending = {0: out_copies(0, (nfull - 2) * _TJ, full),
               1: out_copies(1, (nfull - 1) * _TJ, full)}
    for i in range(nfull, ntiles):
        slot, t0 = i % 2, i * _TJ
        tj = min(_TJ, _S2 - t0)
        rows_of = lambda s, t0=t0, tj=tj: max(0, min(tj, (_T2 - 7 * _S2 if s == 7 else _S2) - t0))
        for c in pending[slot]:
            c.wait()
        joint_tile(slot, t0, tj)
        pending[slot] = out_copies(slot, t0, rows_of)
        for c in pending[slot]:
            c.start()
    for slot in range(2):
        for c in pending[slot]:
            c.wait()


@jax.jit
def pallas_standalone__seq2seq_rnn_t_joint__speech_kernel(
    x: jax.Array,
    w1: jax.Array,
    w2: jax.Array,
    g: jax.Array,
    w_f: jax.Array,
    w_g: jax.Array,
    w_o: jax.Array,
):
    assert x.shape == (_B, _T, _D) and w1.shape == (_K, _D, _D) and w2.shape == (_K, _D, _D)
    assert g.shape == (_B, _U, _D)
    bf, f32 = jnp.bfloat16, jnp.float32
    m = _CBMAX * 16
    scratch = [
        pltpu.VMEM((_NS, 2, 512, 128), bf),
        pltpu.VMEM((_NS, 2, 512, 128), bf),
        pltpu.VMEM((_NS, m, 512), f32),
        pltpu.VMEM((_NS, m, 512), f32),
        pltpu.VMEM((_NS, m, 256), f32),
        pltpu.VMEM((_NS, m, 256), f32),
        pltpu.VMEM((_HROWS, 16, _D), f32),
        pltpu.VMEM((2, 2, _XROWS, 128), jnp.uint32),
        pltpu.VMEM((_K, _D, _D), bf),
        pltpu.VMEM((_K, _D, _D), bf),
        pltpu.VMEM((_B, _U, _D), bf),
        pltpu.VMEM((_D, _D), bf),
        pltpu.VMEM((_D, _D), bf),
        pltpu.VMEM((_D, _D), bf),
        pltpu.VMEM((_B, _U, _D), f32),
        pltpu.VMEM((_CB2 * _HOP + _FROWS, 16, _D), f32),
        pltpu.VMEM((2, 16, _TJ, _U, _D), bf),
        pltpu.SemaphoreType.DMA((6,)),
        pltpu.SemaphoreType.DMA((_XPARTS,)),
        pltpu.SemaphoreType.DMA((2,)),
    ]
    any_spec = pl.BlockSpec(memory_space=pl.ANY)
    return pl.pallas_call(
        _kernel,
        out_shape=jax.ShapeDtypeStruct((_B, _T2, _U, _D), bf),
        in_specs=[any_spec] * 7,
        out_specs=any_spec,
        scratch_shapes=scratch,
        compiler_params=pltpu.CompilerParams(vmem_limit_bytes=127 * 1024 * 1024),
    )(x, w1, w2, g, w_f, w_g, w_o)
```

```python
import functools
import math

import numpy as np

import jax
import jax.numpy as jnp
from jax import lax
import jax.experimental.pallas as pl
import jax.experimental.pallas.tpu as pltpu


class _Prog:
    def __init__(self):
        self.ops = []
        self.cse = {}

    def _node(self, kind, a, b):
        key = (kind, a, b)
        if key not in self.cse:
            self.ops.append(key)
            self.cse[key] = len(self.ops) - 1
        return self.cse[key]

    def inp(self, i):
        return (self._node("in", i, None), 1)

    def neg(self, x):
        return None if x is None else (x[0], -x[1])

    def add(self, x, y):
        if x is None:
            return y
        if y is None:
            return x
        (a, sa), (b, sb) = x, y
        if sa == sb:
            return (self._node("add", min(a, b), max(a, b)), sa)
        if sa > 0:
            return (self._node("sub", a, b), 1)
        return (self._node("sub", b, a), 1)

    def sub(self, x, y):
        return self.add(x, self.neg(y))

    def mul(self, c, x):
        if x is None or c == 0:
            return None
        if c == 1:
            return x
        if c == -1:
            return self.neg(x)
        return (self._node("mul", x[0], abs(float(c))), x[1] * (1 if c > 0 else -1))

    def cadd(self, z, w):
        return (self.add(z[0], w[0]), self.add(z[1], w[1]))

    def csub(self, z, w):
        return (self.sub(z[0], w[0]), self.sub(z[1], w[1]))

    def cconj(self, z):
        return (z[0], self.neg(z[1]))

    def twiddle(self, z, num, den):
        num %= den
        a, b = z
        if (8 * num) % den == 0:
            e = (8 * num) // den
            r = math.sqrt(0.5)
            if e == 0:
                return (a, b)
            if e == 2:
                return (b, self.neg(a))
            if e == 4:
                return (self.neg(a), self.neg(b))
            if e == 6:
                return (self.neg(b), a)
            if e == 1:
                return (self.mul(r, self.add(a, b)), self.mul(r, self.sub(b, a)))
            if e == 3:
                return (self.mul(r, self.sub(b, a)), self.mul(-r, self.add(a, b)))
            if e == 5:
                return (self.mul(-r, self.add(a, b)), self.mul(r, self.sub(a, b)))
            return (self.mul(r, self.sub(a, b)), self.mul(r, self.add(a, b)))
        th = -2.0 * math.pi * num / den
        c, s = math.cos(th), math.sin(th)
        return (self.sub(self.mul(c, a), self.mul(s, b)), self.add(self.mul(s, a), self.mul(c, b)))

    def rfft(self, xs):
        n = len(xs)
        if n == 1:
            return [(xs[0], None)]
        if n == 2:
            return [(self.add(xs[0], xs[1]), None), (self.sub(xs[0], xs[1]), None)]
        if n == 4:
            a = self.add(xs[0], xs[2])
            b = self.sub(xs[0], xs[2])
            c = self.add(xs[1], xs[3])
            d = self.sub(xs[1], xs[3])
            return [(self.add(a, c), None), (b, self.neg(d)), (self.sub(a, c), None)]
        u = self.rfft(xs[0::2])
        z1 = self.rfft(xs[1::4])
        z3 = self.rfft(xs[3::4])

        def get_u(k):
            k %= n // 2
            return u[k] if k <= n // 4 else self.cconj(u[n // 2 - k])

        out = [None] * (n // 2 + 1)
        for k in range(n // 8 + 1):
            t1 = self.twiddle(z1[k], k, n)
            t3 = self.twiddle(z3[k], 3 * k, n)
            sm = self.cadd(t1, t3)
            df = self.csub(t1, t3)
            u0, u1 = get_u(k), get_u(k + n // 4)
            out[k] = self.cadd(u0, sm)
            out[n // 2 - k] = self.cconj(self.csub(u0, sm))
            mdf = (df[1], self.neg(df[0]))
            out[k + n // 4] = self.cadd(u1, mdf)
            if k > 0:
                out[n // 4 - k] = self.cconj(self.csub(u1, mdf))
        return out

    def order(self, outs):
        seen, order = set(), []
        for o in outs:
            if o is None or o[0] in seen:
                continue
            stack = [(o[0], False)]
            while stack:
                n, done = stack.pop()
                if done:
                    order.append(n)
                    continue
                if n in seen:
                    continue
                seen.add(n)
                stack.append((n, True))
                kind, a, b = self.ops[n]
                if kind in ("add", "sub"):
                    stack.append((b, False))
                    stack.append((a, False))
                elif kind == "mul":
                    stack.append((a, False))
        return order

    def transpose(self, outs):
        g = _Prog()
        adj = {}

        def acc(n, v):
            if v is not None:
                adj[n] = g.add(adj.get(n), v)

        for i, o in enumerate(outs):
            if o is not None:
                acc(o[0], g.mul(o[1], g.inp(i)))
        res = {}
        for n in sorted(set(self.order(outs)), reverse=True):
            kind, a, b = self.ops[n]
            v = adj.get(n)
            if v is None:
                continue
            if kind == "in":
                res[a] = v
            elif kind == "add":
                acc(a, v)
                acc(b, v)
            elif kind == "sub":
                acc(a, v)
                acc(b, g.neg(v))
            else:
                acc(a, g.mul(b, v))
        return g, res

    def run(self, outs, load, emit, keep_sign=True):
        val = {}
        want = {}
        for i, o in enumerate(outs):
            if o is not None:
                want.setdefault(o[0], []).append((i, o[1]))
        for n in self.order(outs):
            kind, a, b = self.ops[n]
            if kind == "in":
                v = load(a)
            elif kind == "add":
                v = val[a] + val[b]
            elif kind == "sub":
                v = val[a] - val[b]
            else:
                v = val[a] * np.float32(b)
            val[n] = v
            for i, sg in want.get(n, ()):
                emit(i, -v if (sg < 0 and keep_sign) else v)


def _lhs_outputs(p, spec, n):
    outs = [spec[0][0], spec[n // 2][0]]
    for k in range(1, n // 2):
        a, b = spec[k]
        outs += [p.add(a, b), a, b]
    return outs


class _Plan:
    def __init__(self, n):
        self.n = n
        self.taps = 16
        self.hop = n - self.taps + 1
        self.ns = 2 + 3 * (n // 2 - 1)
        self.fwd = _Prog()
        spec = self.fwd.rfft([self.fwd.inp(i) for i in range(n)])
        self.fwd_outs = _lhs_outputs(self.fwd, spec, n)
        lhs_sign = [o[1] for o in self.fwd_outs]
        p = _Prog()
        spec = p.rfft([p.inp(i) if i < self.hop else None for i in range(n)])
        self.inv, res = p.transpose(_lhs_outputs(p, spec, n))
        self.inv_outs = [res[t] for t in range(self.hop)]
        self.inv_src = [0, 1]
        for k in range(n // 2 - 1):
            base = 2 + 3 * k
            self.inv_src += [base, base + 2, base + 1]
        self.wprog, self.wouts, self.wtap = [], [], []
        for ph in range(2):
            p = _Prog()
            xs = [None] * n
            for j in range(self.taps):
                if not (ph == 0 and j == 0):
                    xs[j] = p.inp(2 * j - 1 if ph == 0 else 2 * j)
            spec = p.rfft(xs)
            outs = [p.mul(0.5, spec[0][0]), p.mul(0.5, spec[n // 2][0])]
            for k in range(1, n // 2):
                c, dm = spec[k]
                d = p.neg(dm)
                outs += [c, p.sub(d, c), p.neg(p.add(c, d))]
            outs = [(o[0], o[1] * s) for o, s in zip(outs, lhs_sign)]
            self.wprog.append(p)
            self.wouts.append(outs)


_FFT_N = 32
_PLAN = _Plan(_FFT_N)

_C0 = math.sqrt(2.0 / math.pi)
_KAPPA = 0.044715 / (_C0 * _C0)


def _gelu2(z):
    inner = z * (np.float32(_KAPPA) * (z * z) + np.float32(1.0))
    return z + z * jnp.tanh(inner)


_B, _T, _D, _K, _U = 2, 16000, 256, 31, 8
_T1, _T2 = _T // 2, _T // 4
_S2 = 502
_S1 = 2 * _S2
_HOP = _PLAN.hop
_NS = _PLAN.ns
_CB = 8
_C1 = [5] + [_CB] * 7
_CB2, _NSTEP2 = 5, 6
_NB1 = sum(_C1)
_XOFF = 24
_XROWS = -(-(7 * _S1 + _HOP * (_NB1 - 1) + _FFT_N) // 8) * 8
_HROWS = 2 * _HOP * (_CB2 * _NSTEP2 - 1) + 2 * _FFT_N
_FROWS = _HOP * _CB2 * _NSTEP2
_TJ = _HOP
_XPARTS = 8
_WPARTS = 4
_NDEP = 2
_COST = {"fx": 262, "fh": 230, "inv": 350, "w": 280}


def _x_piece_bounds():
    edges = []
    for s in range(8):
        for p in range(_XPARTS):
            edges.append(min(max((s * _S1 + p * (_S1 // _XPARTS) - _XOFF) // 8 * 8, 0), _T1))
    edges.append(_T1)
    return edges


def _merge(*lists):
    lists = [l for l in lists if l]
    pos = [0] * len(lists)
    out = []
    for _ in range(sum(len(l) for l in lists)):
        j = min((q for q in range(len(lists)) if pos[q] < len(lists[q])),
                key=lambda q: (pos[q] + 0.5) / len(lists[q]))
        out.append(lists[j][pos[j]])
        pos[j] += 1
    return out


def _dyn8(v):
    return v if isinstance(v, int) else pl.multiple_of(v, 8)


def _emit_step(items, units, mask):
    starts = np.cumsum([0] + [2 * (rows // 8) for rows, _, _ in items])
    nev = int(starts[-1])
    tot = sum(c for c, _ in units) or 1
    margin = min(40, nev // 8)
    sched, cum = [], 0
    for cost, fn in units:
        evs = [min(int((cum + cost * q / _NDEP) / tot * (nev - margin)) + 1, nev - 1)
               for q in range(_NDEP)]
        cum += cost
        sched.append((fn, evs))
    results = {}

    def event(e):
        j = int(np.searchsorted(starts, e, side="right")) - 1
        rg, nn = divmod(e - int(starts[j]), 2)
        return results[j][rg * 8:(rg + 1) * 8, nn * 128:(nn + 1) * 128]

    pi = 0
    for j, (rows, dot_fn, post_fn) in enumerate(items):
        results[j] = dot_fn()
        while pi < len(sched) and max(sched[pi][1]) < starts[j + 1]:
            fn, evs = sched[pi]
            pi += 1
            fn([functools.partial(event, e) for e in evs])
        post_fn(results[j])
    assert pi == len(sched)


def _pick(cnt, total, deps):
    if not deps:
        return None
    j, rem = divmod(cnt * len(deps), total)
    return j if rem < len(deps) else None


def _kernel(x_hbm, w1_hbm, w2_hbm, g_hbm, wf_hbm, wg_hbm, wo_hbm, out_hbm,
            v1, v2, spec_a, spec_b, y_a, y_b, hbuf, xbuf, w1buf, w2buf,
            gbuf, wfbuf, wgbuf, wobuf, gebuf, fbuf, febuf, obuf,
            sem_w, sem_s, sem_x, sem_o):
    plan = _PLAN
    n, hop, ns = plan.n, plan.hop, plan.ns
    specs, ys = (spec_a, spec_b), (y_a, y_b)

    xu = x_hbm.bitcast(jnp.uint32)
    edges = _x_piece_bounds()

    def x_copies(part):
        cps = []
        for s in range(8):
            r0, r1 = edges[s * _XPARTS + part], edges[s * _XPARTS + part + 1]
            for bb in range(2):
                for cs in range(2):
                    cps.append(pltpu.make_async_copy(
                        xu.at[bb, pl.ds(r0, r1 - r0), pl.ds(cs * 128, 128)],
                        xbuf.at[bb, cs, pl.ds(_XOFF + r0, r1 - r0), :],
                        sem_x.at[part]))
        return cps

    wrows = _D // _WPARTS
    w1_copies = [pltpu.make_async_copy(w1_hbm.at[:, pl.ds(p * wrows, wrows), :],
                                       w1buf.at[:, pl.ds(p * wrows, wrows), :], sem_w.at[p])
                 for p in range(_WPARTS)]
    cp_w2 = pltpu.make_async_copy(w2_hbm, w2buf, sem_w.at[_WPARTS])
    small = [pltpu.make_async_copy(src, dst, sem_s.at[i]) for i, (src, dst) in
             enumerate([(g_hbm, gbuf), (wf_hbm, wfbuf), (wg_hbm, wgbuf), (wo_hbm, wobuf)])]

    for c in w1_copies:
        c.start()
    zero8 = jnp.zeros((8, 128), jnp.uint32)
    for bb in range(2):
        for cs in range(2):
            for r in range(0, _XOFF, 8):
                xbuf[bb, cs, pl.ds(r, 8), :] = zero8
            for r in range(_XOFF + _T1, _XROWS, 8):
                xbuf[bb, cs, pl.ds(r, 8), :] = zero8
    zrow = jnp.zeros((16, _D), jnp.float32)
    for r in range(_NB1 * hop, _HROWS):
        hbuf[r] = zrow

    def w_unit(wbuf, vbuf, scale, row, half, ph, nt, deps=(), mask=None):
        cnt = [0]

        def load(tap):
            w = wbuf[tap, pl.ds(_dyn8(row + 8 * half), 8), pl.ds(nt * 128, 128)].astype(jnp.float32)
            j = _pick(cnt[0], 16, deps)
            cnt[0] += 1
            if j is not None:
                w = jnp.where(mask, w, deps[j]())
            return w * np.float32(scale)

        def emit(i, v):
            vbuf[i, nt, pl.ds(_dyn8(ph * 128 + row // 2) + 4 * half, 4), :] = pltpu.bitcast(
                v.astype(jnp.bfloat16), jnp.uint32)
        plan.wprog[ph].run(plan.wouts[ph], load, emit)

    def fwd_unit(load_in, spec, row, col, deps, mask):
        cnt = [0]

        def load(q):
            j = _pick(cnt[0], n, deps)
            cnt[0] += 1
            return load_in(q, None if j is None else deps[j], mask)

        def emit(i, v):
            spec[i, pl.ds(row, 8), pl.ds(col, 128)] = v
        plan.fwd.run(plan.fwd_outs, load, emit, keep_sign=False)

    def fx_unit(spec, blk, be, bb, cs, ph, zd, deps=(), mask=None):
        base = blk * hop
        if ph == 1:
            base = base + zd

        def load_in(q, dep, mask):
            v = xbuf[bb, cs, pl.ds(base + q, 8, stride=_S1), :]
            if dep is not None:
                v = jnp.where(mask, v, lax.bitcast_convert_type(dep(), jnp.uint32))
            v = (v << 16) if ph == 0 else (v & jnp.uint32(0xFFFF0000))
            return lax.bitcast_convert_type(v, jnp.float32)
        fwd_unit(load_in, spec, _dyn8(be * 16 + bb * 8), ph * 256 + cs * 128, deps, mask)

    def fh_unit(spec, blk, be, bb, cs, ph, deps=(), mask=None):
        base = blk * 2 * hop + ph

        def load_in(q, dep, mask):
            v = hbuf[base + 2 * q, pl.ds(_dyn8(bb * 8), 8), pl.ds(cs * 128, 128)]
            if dep is not None:
                v = jnp.where(mask, v, dep())
            return v
        fwd_unit(load_in, spec, _dyn8(be * 16 + bb * 8), ph * 256 + cs * 128, deps, mask)

    def inv_unit(ybuf, dst, scale, blk, be, bb, nt, deps=(), mask=None):
        cnt = [0]
        row = _dyn8(be * 16 + bb * 8)

        def load(i):
            v = ybuf[plan.inv_src[i], pl.ds(row, 8), pl.ds(nt * 128, 128)]
            j = _pick(cnt[0], ns, deps)
            cnt[0] += 1
            if j is not None:
                v = jnp.where(mask, v, deps[j]())
            return v

        def store(t, z):
            hval = _gelu2(z)
            if scale != 1.0:
                hval = hval * np.float32(scale)
            dst[blk * hop + t, pl.ds(_dyn8(bb * 8), 8), pl.ds(nt * 128, 128)] = hval
        plan.inv.run(plan.inv_outs, load, store)

    def fx_units(spec, blk0, nblk, zd, mask):
        return [(_COST["fx"], functools.partial(fx_unit, spec, blk0 + be, be, bb, cs, ph, zd, mask=mask))
                for be in range(nblk) for bb in range(2) for cs in range(2) for ph in range(2)]

    def fh_units(spec, blk0, nblk, mask):
        return [(_COST["fh"], functools.partial(fh_unit, spec, blk0 + be, be, bb, cs, ph, mask=mask))
                for be in range(nblk) for bb in range(2) for cs in range(2) for ph in range(2)]

    def inv_units(ybuf, dst, scale, blk0, nblk, mask):
        return [(_COST["inv"], functools.partial(inv_unit, ybuf, dst, scale, blk0 + be, be, bb, nt, mask=mask))
                for be in range(nblk) for bb in range(2) for nt in range(2)]

    def w2_units(rg0, nrg, mask):
        return [(_COST["w"], functools.partial(
                    w_unit, w2buf, v2, (2.0 / n) * 0.5, pl.multiple_of((rg0 + r) * 16, 16)
                    if not isinstance(rg0, int) else (rg0 + r) * 16, half, ph, nt, mask=mask))
                for r in range(nrg) for half in range(2) for ph in range(2) for nt in range(2)]

    def conv_items(vbuf, spec, ybuf, m):
        items = []
        for i in range(ns):
            hold = []

            def dot_fn(i=i, h=0):
                w = jnp.concatenate(
                    [pltpu.bitcast(vbuf[i, nt, pl.ds(h * 128, 128), :], jnp.bfloat16)
                     for nt in range(2)], axis=1)
                return jnp.dot(spec[i, pl.ds(0, m), pl.ds(h * 256, 256)], w,
                               preferred_element_type=jnp.float32)

            def post0(r, hold=hold):
                hold.append(r)

            def post1(r, i=i, hold=hold):
                ybuf[i, pl.ds(0, m), :] = hold[0] + r
            items.append((m, functools.partial(dot_fn, i, 0), post0))
            items.append((m, functools.partial(dot_fn, i, 1), post1))
        return items

    def block(fn, zd):
        def body(_, c):
            fn()
            return c
        lax.fori_loop(0, 1 + zd, body, 0)

    def opaque_zero(i):
        return (i * (i + 1)) & 1

    def true_mask(zd):
        return jnp.full((8, 128), zd, jnp.int32) == 0

    c1_start = [int(v) for v in np.cumsum([0] + _C1)]

    def v1_body(rg, carry):
        for p in range(_WPARTS):
            @pl.when(rg == p * (wrows // 16))
            def _():
                w1_copies[p].wait()
                if p == 0:
                    for c in x_copies(0):
                        c.start()
                if p == 2:
                    for c in x_copies(1):
                        c.start()
        row = pl.multiple_of(rg * 16, 16)
        for half in range(2):
            for ph in range(2):
                for nt in range(2):
                    w_unit(w1buf, v1, (2.0 / n) * _C0, row, half, ph, nt)
        return carry
    with jax.named_scope("v1"):
        lax.fori_loop(0, _D // 16, v1_body, 0)

    zd0 = opaque_zero(xbuf[0, 0, 0, 0].astype(jnp.int32))
    mask0 = true_mask(zd0)

    need = {0: [1], 1: [2], 2: [3, 4], 3: [5], 4: [6], 5: [7], 6: []}

    def start_parts(c):
        for p in need.get(c, []):
            for cp in x_copies(p):
                cp.start()

    def wait_parts(c):
        for p in need.get(c, []):
            for cp in x_copies(p):
                cp.wait()

    with jax.named_scope("x0wait"):
        for c in x_copies(0):
            c.wait()
    cp_w2.start()
    start_parts(1)

    def fill_body(u, carry):
        zd = opaque_zero(u)
        for cs in range(2):
            for ph in range(2):
                fx_unit(spec_a, u // 2, u // 2, u % 2, cs, ph, zd)
        return carry
    with jax.named_scope("fill"):
        lax.fori_loop(0, _C1[0] * 2, fill_body, 0)

    with jax.named_scope("x1wait"):
        wait_parts(0)

    def step0_body():
        zd, mask = zd0, mask0
        _emit_step(conv_items(v1, spec_a, y_a, _C1[0] * 16),
                   fx_units(spec_b, c1_start[1], _CB, zd, mask), mask)
    with jax.named_scope("step0"):
        block(step0_body, zd0)

    def conv1_body(it, carry):
        zd = opaque_zero(it)
        mask = true_mask(zd)
        for par in (1, 0):
            c = 2 * it + (1 if par == 1 else 2)
            blk_c = _C1[0] + (c - 1) * _CB
            for k in range(3):
                @pl.when(it == k)
                def _():
                    ck = 2 * k + (1 if par == 1 else 2)
                    wait_parts(ck)
                    start_parts(ck + 1)
                    if ck == 1:
                        cp_w2.wait()
                    if ck == 5:
                        for cp in small:
                            cp.start()
            block(lambda: _emit_step(
                conv_items(v1, specs[par], ys[par], _CB * 16),
                _merge(fx_units(specs[1 - par], blk_c + _CB, _CB, zd, mask),
                       inv_units(ys[1 - par], hbuf, 1.0,
                                 jnp.maximum(blk_c - _CB, 0), _CB, mask),
                       w2_units(2 * c - 2, 2, mask)), mask), zd)
        return carry
    with jax.named_scope("conv1"):
        lax.fori_loop(0, 3, conv1_body, 0)

    sub = lax.broadcasted_iota(jnp.int32, (16, _D), 0) % 8

    def mask_rows(r0, r1, s):
        def body(r, carry):
            hbuf[r] = jnp.where(sub == s, 0.0, hbuf[r])
            return carry
        lax.fori_loop(r0, r1, body, 0)
    mask_rows(0, 16, 0)

    def step7_body():
        zd, mask = zd0, mask0
        _emit_step(conv_items(v1, spec_b, y_b, _CB * 16),
                   _merge(fh_units(spec_a, 0, _CB2, mask),
                          inv_units(y_a, hbuf, 1.0, c1_start[6], _CB, mask),
                          w2_units(12, 4, mask)), mask)
    with jax.named_scope("step7"):
        block(step7_body, zd0)

    fscale = 0.5 / _C0

    def step8_body():
        zd, mask = zd0, mask0
        _emit_step(conv_items(v2, spec_a, y_a, _CB2 * 16),
                   _merge(fh_units(spec_b, _CB2, _CB2, mask),
                          inv_units(y_b, hbuf, 1.0, c1_start[7], _CB, mask)), mask)
    with jax.named_scope("step8"):
        block(step8_body, zd0)
    mask_rows(_T1 - 7 * _S1 + 16, _NB1 * hop, 7)

    def conv2_body(it, carry):
        zd = opaque_zero(it)
        mask = true_mask(zd)
        for par in (1, 0):
            c = 2 * it + (1 if par == 1 else 2)
            block(lambda: _emit_step(
                conv_items(v2, specs[par], ys[par], _CB2 * 16),
                _merge(fh_units(specs[1 - par], (c + 1) * _CB2, _CB2, mask),
                       inv_units(ys[1 - par], fbuf, fscale, (c - 1) * _CB2, _CB2, mask)),
                mask), zd)
        return carry
    with jax.named_scope("conv2"):
        lax.fori_loop(0, 2, conv2_body, 0)

    for c in small:
        c.wait()
    gebuf[...] = jnp.dot(gbuf[...].reshape(_B * _U, _D), wgbuf[...],
                         preferred_element_type=jnp.float32).reshape(_B, _U, _D)

    def fe_item(slot, tile):
        def dot_fn():
            f = fbuf[pl.ds(tile * _TJ, _TJ)].reshape(_TJ * 16, _D)
            return jnp.dot(f, wfbuf[...], preferred_element_type=jnp.float32)

        def post(r):
            febuf[slot] = r.reshape(_TJ, 16, _D)
        return (_TJ * 16, dot_fn, post)

    def step13_body():
        zd, mask = zd0, mask0
        _emit_step(conv_items(v2, spec_b, y_b, _CB2 * 16) + [fe_item(0, 0)],
                   inv_units(y_a, fbuf, fscale, 4 * _CB2, _CB2, mask), mask)
    with jax.named_scope("step13"):
        block(step13_body, zd0)

    def out_copies(slot, t0, rows_of):
        cps = []
        for r in range(16):
            bb, s = divmod(r, 8)
            rows = rows_of(s)
            if rows > 0:
                cps.append(pltpu.make_async_copy(
                    obuf.at[slot, r, pl.ds(0, rows)],
                    out_hbm.at[bb, pl.ds(s * _S2 + t0, rows)],
                    sem_o.at[slot]))
        return cps

    def joint_item(slot, tj):
        def dot_fn():
            rows = []
            for tt in range(tj):
                for r in range(16):
                    fr = febuf[slot, tt, pl.ds(r, 1), :]
                    rows.append(jnp.tanh(jnp.broadcast_to(fr, (_U, _D)) + gebuf[r // 8]))
            return jnp.dot(jnp.concatenate(rows, axis=0), wobuf[...],
                           preferred_element_type=jnp.float32)

        def post(o):
            o = o.reshape(tj, 16, _U, _D).astype(jnp.bfloat16)
            for tt in range(tj):
                obuf[slot, :, tt] = o[tt]
        return (tj * 16 * _U, dot_fn, post)

    full = lambda s: _TJ
    ntiles = -(-_S2 // _TJ)
    nfull = (_T2 - 7 * _S2) // _TJ
    assert nfull % 2 == 0

    def first_body():
        zd, mask = zd0, mask0
        _emit_step([fe_item(1, 1), joint_item(0, _TJ), fe_item(0, 2), joint_item(1, _TJ)],
                   inv_units(y_b, fbuf, fscale, 5 * _CB2, _CB2, mask), mask)
        for slot in range(2):
            for c in out_copies(slot, slot * _TJ, full):
                c.start()
    with jax.named_scope("first"):
        block(first_body, zd0)

    def joint_body(i2, carry):
        for slot in range(2):
            tile = 2 * i2 + slot
            t0 = tile * _TJ
            for c in out_copies(slot, t0 - 2 * _TJ, full):
                c.wait()
            _emit_step([fe_item(1 - slot, jnp.minimum(tile + 1, ntiles - 1)), joint_item(slot, _TJ)],
                       [], None)
            for c in out_copies(slot, t0, full):
                c.start()
        return carry
    with jax.named_scope("joint"):
        lax.fori_loop(1, nfull // 2, joint_body, 0)

    pending = {0: out_copies(0, (nfull - 2) * _TJ, full),
               1: out_copies(1, (nfull - 1) * _TJ, full)}
    for tile in range(nfull, ntiles):
        slot, t0 = tile % 2, tile * _TJ
        tj = min(_TJ, _S2 - t0)
        rows_of = lambda s, t0=t0, tj=tj: max(0, min(tj, (_T2 - 7 * _S2 if s == 7 else _S2) - t0))
        for c in pending[slot]:
            c.wait()
        items = ([fe_item(1 - slot, tile + 1)] if tile + 1 < ntiles else []) + [joint_item(slot, tj)]
        _emit_step(items, [], None)
        pending[slot] = out_copies(slot, t0, rows_of)
        for c in pending[slot]:
            c.start()
    for slot in range(2):
        for c in pending[slot]:
            c.wait()


@jax.jit
def pallas_standalone__seq2seq_rnn_t_joint__speech_kernel(
    x: jax.Array,
    w1: jax.Array,
    w2: jax.Array,
    g: jax.Array,
    w_f: jax.Array,
    w_g: jax.Array,
    w_o: jax.Array,
):
    assert x.shape == (_B, _T, _D) and w1.shape == (_K, _D, _D) and w2.shape == (_K, _D, _D)
    assert g.shape == (_B, _U, _D)
    bf, f32 = jnp.bfloat16, jnp.float32
    m = _CB * 16
    scratch = [
        pltpu.VMEM((_NS, 2, 256, 128), jnp.uint32),
        pltpu.VMEM((_NS, 2, 256, 128), jnp.uint32),
        pltpu.VMEM((_NS, m, 512), f32),
        pltpu.VMEM((_NS, m, 512), f32),
        pltpu.VMEM((_NS, m, 256), f32),
        pltpu.VMEM((_NS, m, 256), f32),
        pltpu.VMEM((_HROWS, 16, _D), f32),
        pltpu.VMEM((2, 2, _XROWS, 128), jnp.uint32),
        pltpu.VMEM((_K, _D, _D), bf),
        pltpu.VMEM((_K, _D, _D), bf),
        pltpu.VMEM((_B, _U, _D), bf),
        pltpu.VMEM((_D, _D), bf),
        pltpu.VMEM((_D, _D), bf),
        pltpu.VMEM((_D, _D), bf),
        pltpu.VMEM((_B, _U, _D), f32),
        pltpu.VMEM((_FROWS, 16, _D), f32),
        pltpu.VMEM((2, _TJ, 16, _D), f32),
        pltpu.VMEM((2, 16, _TJ, _U, _D), bf),
        pltpu.SemaphoreType.DMA((_WPARTS + 1,)),
        pltpu.SemaphoreType.DMA((4,)),
        pltpu.SemaphoreType.DMA((_XPARTS,)),
        pltpu.SemaphoreType.DMA((2,)),
    ]
    any_spec = pl.BlockSpec(memory_space=pl.ANY)
    return pl.pallas_call(
        _kernel,
        out_shape=jax.ShapeDtypeStruct((_B, _T2, _U, _D), bf),
        in_specs=[any_spec] * 7,
        out_specs=any_spec,
        scratch_shapes=scratch,
        compiler_params=pltpu.CompilerParams(vmem_limit_bytes=127 * 1024 * 1024),
    )(x, w1, w2, g, w_f, w_g, w_o)
```

```python
import functools
import math

import numpy as np

import jax
import jax.numpy as jnp
from jax import lax
import jax.experimental.pallas as pl
import jax.experimental.pallas.tpu as pltpu


class _Prog:
    def __init__(self):
        self.ops = []
        self.cse = {}

    def _node(self, kind, a, b):
        key = (kind, a, b)
        if key not in self.cse:
            self.ops.append(key)
            self.cse[key] = len(self.ops) - 1
        return self.cse[key]

    def inp(self, i):
        return (self._node("in", i, None), 1)

    def neg(self, x):
        return None if x is None else (x[0], -x[1])

    def add(self, x, y):
        if x is None:
            return y
        if y is None:
            return x
        (a, sa), (b, sb) = x, y
        if sa == sb:
            return (self._node("add", min(a, b), max(a, b)), sa)
        if sa > 0:
            return (self._node("sub", a, b), 1)
        return (self._node("sub", b, a), 1)

    def sub(self, x, y):
        return self.add(x, self.neg(y))

    def mul(self, c, x):
        if x is None or c == 0:
            return None
        if c == 1:
            return x
        if c == -1:
            return self.neg(x)
        return (self._node("mul", x[0], abs(float(c))), x[1] * (1 if c > 0 else -1))

    def cadd(self, z, w):
        return (self.add(z[0], w[0]), self.add(z[1], w[1]))

    def csub(self, z, w):
        return (self.sub(z[0], w[0]), self.sub(z[1], w[1]))

    def cconj(self, z):
        return (z[0], self.neg(z[1]))

    def twiddle(self, z, num, den):
        num %= den
        a, b = z
        if (8 * num) % den == 0:
            e = (8 * num) // den
            r = math.sqrt(0.5)
            if e == 0:
                return (a, b)
            if e == 2:
                return (b, self.neg(a))
            if e == 4:
                return (self.neg(a), self.neg(b))
            if e == 6:
                return (self.neg(b), a)
            if e == 1:
                return (self.mul(r, self.add(a, b)), self.mul(r, self.sub(b, a)))
            if e == 3:
                return (self.mul(r, self.sub(b, a)), self.mul(-r, self.add(a, b)))
            if e == 5:
                return (self.mul(-r, self.add(a, b)), self.mul(r, self.sub(a, b)))
            return (self.mul(r, self.sub(a, b)), self.mul(r, self.add(a, b)))
        th = -2.0 * math.pi * num / den
        c, s = math.cos(th), math.sin(th)
        return (self.sub(self.mul(c, a), self.mul(s, b)), self.add(self.mul(s, a), self.mul(c, b)))

    def rfft(self, xs):
        n = len(xs)
        if n == 1:
            return [(xs[0], None)]
        if n == 2:
            return [(self.add(xs[0], xs[1]), None), (self.sub(xs[0], xs[1]), None)]
        if n == 4:
            a = self.add(xs[0], xs[2])
            b = self.sub(xs[0], xs[2])
            c = self.add(xs[1], xs[3])
            d = self.sub(xs[1], xs[3])
            return [(self.add(a, c), None), (b, self.neg(d)), (self.sub(a, c), None)]
        u = self.rfft(xs[0::2])
        z1 = self.rfft(xs[1::4])
        z3 = self.rfft(xs[3::4])

        def get_u(k):
            k %= n // 2
            return u[k] if k <= n // 4 else self.cconj(u[n // 2 - k])

        out = [None] * (n // 2 + 1)
        for k in range(n // 8 + 1):
            t1 = self.twiddle(z1[k], k, n)
            t3 = self.twiddle(z3[k], 3 * k, n)
            sm = self.cadd(t1, t3)
            df = self.csub(t1, t3)
            u0, u1 = get_u(k), get_u(k + n // 4)
            out[k] = self.cadd(u0, sm)
            out[n // 2 - k] = self.cconj(self.csub(u0, sm))
            mdf = (df[1], self.neg(df[0]))
            out[k + n // 4] = self.cadd(u1, mdf)
            if k > 0:
                out[n // 4 - k] = self.cconj(self.csub(u1, mdf))
        return out

    def order(self, outs):
        seen, order = set(), []
        for o in outs:
            if o is None or o[0] in seen:
                continue
            stack = [(o[0], False)]
            while stack:
                n, done = stack.pop()
                if done:
                    order.append(n)
                    continue
                if n in seen:
                    continue
                seen.add(n)
                stack.append((n, True))
                kind, a, b = self.ops[n]
                if kind in ("add", "sub"):
                    stack.append((b, False))
                    stack.append((a, False))
                elif kind == "mul":
                    stack.append((a, False))
        return order

    def transpose(self, outs):
        g = _Prog()
        adj = {}

        def acc(n, v):
            if v is not None:
                adj[n] = g.add(adj.get(n), v)

        for i, o in enumerate(outs):
            if o is not None:
                acc(o[0], g.mul(o[1], g.inp(i)))
        res = {}
        for n in sorted(set(self.order(outs)), reverse=True):
            kind, a, b = self.ops[n]
            v = adj.get(n)
            if v is None:
                continue
            if kind == "in":
                res[a] = v
            elif kind == "add":
                acc(a, v)
                acc(b, v)
            elif kind == "sub":
                acc(a, v)
                acc(b, g.neg(v))
            else:
                acc(a, g.mul(b, v))
        return g, res

    def run(self, outs, load, emit, keep_sign=True):
        val = {}
        want = {}
        for i, o in enumerate(outs):
            if o is not None:
                want.setdefault(o[0], []).append((i, o[1]))
        for n in self.order(outs):
            kind, a, b = self.ops[n]
            if kind == "in":
                v = load(a)
            elif kind == "add":
                v = val[a] + val[b]
            elif kind == "sub":
                v = val[a] - val[b]
            else:
                v = val[a] * np.float32(b)
            val[n] = v
            for i, sg in want.get(n, ()):
                emit(i, -v if (sg < 0 and keep_sign) else v)


def _lhs_outputs(p, spec, n):
    outs = [spec[0][0], spec[n // 2][0]]
    for k in range(1, n // 2):
        a, b = spec[k]
        outs += [p.add(a, b), a, b]
    return outs


class _Plan:
    def __init__(self, n):
        self.n = n
        self.taps = 16
        self.hop = n - self.taps + 1
        self.ns = 2 + 3 * (n // 2 - 1)
        self.fwd = _Prog()
        spec = self.fwd.rfft([self.fwd.inp(i) for i in range(n)])
        self.fwd_outs = _lhs_outputs(self.fwd, spec, n)
        lhs_sign = [o[1] for o in self.fwd_outs]
        p = _Prog()
        spec = p.rfft([p.inp(i) if i < self.hop else None for i in range(n)])
        self.inv, res = p.transpose(_lhs_outputs(p, spec, n))
        self.inv_outs = [res[t] for t in range(self.hop)]
        self.inv_src = [0, 1]
        for k in range(n // 2 - 1):
            base = 2 + 3 * k
            self.inv_src += [base, base + 2, base + 1]
        self.wprog, self.wouts, self.wtap = [], [], []
        for ph in range(2):
            p = _Prog()
            xs = [None] * n
            for j in range(self.taps):
                if not (ph == 0 and j == 0):
                    xs[j] = p.inp(2 * j - 1 if ph == 0 else 2 * j)
            spec = p.rfft(xs)
            outs = [p.mul(0.5, spec[0][0]), p.mul(0.5, spec[n // 2][0])]
            for k in range(1, n // 2):
                c, dm = spec[k]
                d = p.neg(dm)
                outs += [c, p.sub(d, c), p.neg(p.add(c, d))]
            outs = [(o[0], o[1] * s) for o, s in zip(outs, lhs_sign)]
            self.wprog.append(p)
            self.wouts.append(outs)


_FFT_N = 32
_PLAN = _Plan(_FFT_N)

_C0 = math.sqrt(2.0 / math.pi)
_KAPPA = 0.044715 / (_C0 * _C0)


def _gelu2(z):
    inner = z * (np.float32(_KAPPA) * (z * z) + np.float32(1.0))
    return z + z * jnp.tanh(inner)


_B, _T, _D, _K, _U = 2, 16000, 256, 31, 8
_T1, _T2 = _T // 2, _T // 4
_S2 = 502
_S1 = 2 * _S2
_HOP = _PLAN.hop
_NS = _PLAN.ns
_CB = 8
_C1 = [5] + [_CB] * 7
_CB2, _NSTEP2 = 5, 6
_NB1 = sum(_C1)
_XOFF = 24
_XROWS = -(-(7 * _S1 + _HOP * (_NB1 - 1) + _FFT_N) // 8) * 8
_HROWS = 2 * _HOP * (_CB2 * _NSTEP2 - 1) + 2 * _FFT_N
_FROWS = _HOP * _CB2 * _NSTEP2
_TJ = _HOP
_XPARTS = 8
_WPARTS = 4
_NDEP = 2
_COST = {"fx": 262, "fh": 230, "inv": 350, "w": 280}


def _x_piece_bounds():
    edges = []
    for s in range(8):
        for p in range(_XPARTS):
            edges.append(min(max((s * _S1 + p * (_S1 // _XPARTS) - _XOFF) // 8 * 8, 0), _T1))
    edges.append(_T1)
    return edges


def _merge(*lists):
    lists = [l for l in lists if l]
    pos = [0] * len(lists)
    out = []
    for _ in range(sum(len(l) for l in lists)):
        j = min((q for q in range(len(lists)) if pos[q] < len(lists[q])),
                key=lambda q: (pos[q] + 0.5) / len(lists[q]))
        out.append(lists[j][pos[j]])
        pos[j] += 1
    return out


def _dyn8(v):
    return v if isinstance(v, int) else pl.multiple_of(v, 8)


def _emit_step(items, units, mask):
    starts = np.cumsum([0] + [2 * (rows // 8) for rows, _, _ in items])
    nev = int(starts[-1])
    tot = sum(c for c, _ in units) or 1
    margin = min(40, nev // 8)
    sched, cum = [], 0
    for cost, fn in units:
        evs = [min(int((cum + cost * q / _NDEP) / tot * (nev - margin)) + 1, nev - 1)
               for q in range(_NDEP)]
        cum += cost
        sched.append((fn, evs))
    results = {}

    def event(e):
        j = int(np.searchsorted(starts, e, side="right")) - 1
        rg, nn = divmod(e - int(starts[j]), 2)
        return results[j][rg * 8:(rg + 1) * 8, nn * 128:(nn + 1) * 128]

    pi = 0
    for j, (rows, dot_fn, post_fn) in enumerate(items):
        results[j] = dot_fn()
        while pi < len(sched) and max(sched[pi][1]) < starts[j + 1]:
            fn, evs = sched[pi]
            pi += 1
            fn([functools.partial(event, e) for e in evs])
        post_fn(results[j])
    assert pi == len(sched)


def _pick(cnt, total, deps):
    if not deps:
        return None
    j, rem = divmod(cnt * len(deps), total)
    return j if rem < len(deps) else None


def _kernel(x_hbm, w1_hbm, w2_hbm, g_hbm, wf_hbm, wg_hbm, wo_hbm, out_hbm,
            v1, v2, spec_a, spec_b, y_a, y_b, hbuf, xbuf, w1buf, w2buf,
            gbuf, wfbuf, wgbuf, wobuf, gebuf, fbuf, febuf, obuf,
            sem_w, sem_s, sem_x, sem_o):
    plan = _PLAN
    n, hop, ns = plan.n, plan.hop, plan.ns
    specs, ys = (spec_a, spec_b), (y_a, y_b)

    xu = x_hbm.bitcast(jnp.uint32)
    edges = _x_piece_bounds()

    def x_copies(part):
        cps = []
        for s in range(8):
            r0, r1 = edges[s * _XPARTS + part], edges[s * _XPARTS + part + 1]
            for cs in range(2):
                cps.append(pltpu.make_async_copy(
                    xu.at[:, pl.ds(r0, r1 - r0), pl.ds(cs * 128, 128)],
                    xbuf.at[:, cs, pl.ds(_XOFF + r0, r1 - r0), :],
                    sem_x.at[part]))
        return cps

    wrows = _D // _WPARTS
    w1_copies = [pltpu.make_async_copy(w1_hbm.at[:, pl.ds(p * wrows, wrows), :],
                                       w1buf.at[:, pl.ds(p * wrows, wrows), :], sem_w.at[p])
                 for p in range(_WPARTS)]
    cp_w2 = pltpu.make_async_copy(w2_hbm, w2buf, sem_w.at[_WPARTS])
    small = [pltpu.make_async_copy(src, dst, sem_s.at[i]) for i, (src, dst) in
             enumerate([(g_hbm, gbuf), (wf_hbm, wfbuf), (wg_hbm, wgbuf), (wo_hbm, wobuf)])]

    for c in w1_copies:
        c.start()
    zero8 = jnp.zeros((8, 128), jnp.uint32)
    for bb in range(2):
        for cs in range(2):
            for r in range(0, _XOFF, 8):
                xbuf[bb, cs, pl.ds(r, 8), :] = zero8
            for r in range(_XOFF + _T1, _XROWS, 8):
                xbuf[bb, cs, pl.ds(r, 8), :] = zero8
    zrow = jnp.zeros((16, _D), jnp.float32)
    for r in range(_NB1 * hop, _HROWS):
        hbuf[r] = zrow

    def w_unit(wbuf, vbuf, scale, row, half, ph, nt, deps=(), mask=None):
        cnt = [0]

        def load(tap):
            w = wbuf[tap, pl.ds(_dyn8(row + 8 * half), 8), pl.ds(nt * 128, 128)].astype(jnp.float32)
            j = _pick(cnt[0], 16, deps)
            cnt[0] += 1
            if j is not None:
                w = jnp.where(mask, w, deps[j]())
            return w * np.float32(scale)

        def emit(i, v):
            vbuf[i, nt, pl.ds(_dyn8(ph * 128 + row // 2) + 4 * half, 4), :] = pltpu.bitcast(
                v.astype(jnp.bfloat16), jnp.uint32)
        plan.wprog[ph].run(plan.wouts[ph], load, emit)

    def fwd_unit(load_in, spec, row, col, deps, mask):
        cnt = [0]

        def load(q):
            j = _pick(cnt[0], n, deps)
            cnt[0] += 1
            return load_in(q, None if j is None else deps[j], mask)

        def emit(i, v):
            spec[col // 128, i, pl.ds(row, 8), :] = v
        plan.fwd.run(plan.fwd_outs, load, emit, keep_sign=False)

    def fx_unit(spec, blk, be, bb, cs, ph, zd, deps=(), mask=None):
        base = blk * hop
        if ph == 1:
            base = base + zd

        def load_in(q, dep, mask):
            v = xbuf[bb, cs, pl.ds(base + q, 8, stride=_S1), :]
            if dep is not None:
                v = jnp.where(mask, v, lax.bitcast_convert_type(dep(), jnp.uint32))
            v = (v << 16) if ph == 0 else (v & jnp.uint32(0xFFFF0000))
            return lax.bitcast_convert_type(v, jnp.float32)
        fwd_unit(load_in, spec, _dyn8(be * 16 + bb * 8), ph * 256 + cs * 128, deps, mask)

    def fh_unit(spec, blk, be, bb, cs, ph, deps=(), mask=None):
        base = blk * 2 * hop + ph

        def load_in(q, dep, mask):
            v = hbuf[base + 2 * q, pl.ds(_dyn8(bb * 8), 8), pl.ds(cs * 128, 128)]
            if dep is not None:
                v = jnp.where(mask, v, dep())
            return v
        fwd_unit(load_in, spec, _dyn8(be * 16 + bb * 8), ph * 256 + cs * 128, deps, mask)

    def inv_unit(ybuf, dst, scale, blk, be, bb, nt, deps=(), mask=None):
        cnt = [0]
        row = _dyn8(be * 16 + bb * 8)

        def load(i):
            v = ybuf[nt, plan.inv_src[i], pl.ds(row, 8), :]
            j = _pick(cnt[0], ns, deps)
            cnt[0] += 1
            if j is not None:
                v = jnp.where(mask, v, deps[j]())
            return v

        def store(t, z):
            hval = _gelu2(z)
            if scale != 1.0:
                hval = hval * np.float32(scale)
            dst[blk * hop + t, pl.ds(_dyn8(bb * 8), 8), pl.ds(nt * 128, 128)] = hval
        plan.inv.run(plan.inv_outs, load, store)

    def fx_units(spec, blk0, nblk, zd, mask):
        return [(_COST["fx"], functools.partial(fx_unit, spec, blk0 + be, be, bb, cs, ph, zd, mask=mask))
                for be in range(nblk) for bb in range(2) for cs in range(2) for ph in range(2)]

    def fh_units(spec, blk0, nblk, mask):
        return [(_COST["fh"], functools.partial(fh_unit, spec, blk0 + be, be, bb, cs, ph, mask=mask))
                for be in range(nblk) for bb in range(2) for cs in range(2) for ph in range(2)]

    def inv_units(ybuf, dst, scale, blk0, nblk, mask):
        return [(_COST["inv"], functools.partial(inv_unit, ybuf, dst, scale, blk0 + be, be, bb, nt, mask=mask))
                for be in range(nblk) for bb in range(2) for nt in range(2)]

    def w2_units(rg0, nrg, mask):
        return [(_COST["w"], functools.partial(
                    w_unit, w2buf, v2, (2.0 / n) * 0.5, pl.multiple_of((rg0 + r) * 16, 16)
                    if not isinstance(rg0, int) else (rg0 + r) * 16, half, ph, nt, mask=mask))
                for r in range(nrg) for half in range(2) for ph in range(2) for nt in range(2)]

    def conv_items(vbuf, spec, ybuf, m):
        items = []
        for i in range(ns):
            hold = []

            def dot_fn(i=i, h=0):
                w = jnp.concatenate(
                    [pltpu.bitcast(vbuf[i, nt, pl.ds(h * 128, 128), :], jnp.bfloat16)
                     for nt in range(2)], axis=1)
                lhs = jnp.concatenate([spec[2 * h + q, i, pl.ds(0, m), :] for q in range(2)], axis=1)
                return jnp.dot(lhs, w, preferred_element_type=jnp.float32)

            def post0(r, hold=hold):
                hold.append(r)

            def post1(r, i=i, hold=hold):
                y = hold[0] + r
                for nt in range(2):
                    ybuf[nt, i, pl.ds(0, m), :] = y[:, nt * 128:(nt + 1) * 128]
            items.append((m, functools.partial(dot_fn, i, 0), post0))
            items.append((m, functools.partial(dot_fn, i, 1), post1))
        return items

    def block(fn, zd):
        def body(_, c):
            fn()
            return c
        lax.fori_loop(0, 1 + zd, body, 0)

    def opaque_zero(i):
        return (i * (i + 1)) & 1

    def true_mask(zd):
        return jnp.full((8, 128), zd, jnp.int32) == 0

    c1_start = [int(v) for v in np.cumsum([0] + _C1)]

    def v1_body(rg, carry):
        for p in range(_WPARTS):
            @pl.when(rg == p * (wrows // 16))
            def _():
                w1_copies[p].wait()
                if p == 0:
                    for c in x_copies(0):
                        c.start()
                if p == 2:
                    for c in x_copies(1):
                        c.start()
        row = pl.multiple_of(rg * 16, 16)
        for half in range(2):
            for ph in range(2):
                for nt in range(2):
                    w_unit(w1buf, v1, (2.0 / n) * _C0, row, half, ph, nt)
        return carry
    with jax.named_scope("v1"):
        lax.fori_loop(0, _D // 16, v1_body, 0)

    zd0 = opaque_zero(xbuf[0, 0, 0, 0].astype(jnp.int32))
    mask0 = true_mask(zd0)

    need = {0: [1], 1: [2], 2: [3, 4], 3: [5], 4: [6], 5: [7], 6: []}

    def start_parts(c):
        for p in need.get(c, []):
            for cp in x_copies(p):
                cp.start()

    def wait_parts(c):
        for p in need.get(c, []):
            for cp in x_copies(p):
                cp.wait()

    with jax.named_scope("x0wait"):
        for c in x_copies(0):
            c.wait()
    cp_w2.start()
    start_parts(1)

    def fill_body(u, carry):
        zd = opaque_zero(u)
        for cs in range(2):
            for ph in range(2):
                fx_unit(spec_a, u // 2, u // 2, u % 2, cs, ph, zd)
        return carry
    with jax.named_scope("fill"):
        lax.fori_loop(0, _C1[0] * 2, fill_body, 0)

    with jax.named_scope("x1wait"):
        wait_parts(0)

    def step0_body():
        zd, mask = zd0, mask0
        _emit_step(conv_items(v1, spec_a, y_a, _C1[0] * 16),
                   fx_units(spec_b, c1_start[1], _CB, zd, mask), mask)
    with jax.named_scope("step0"):
        block(step0_body, zd0)

    def conv1_body(it, carry):
        zd = opaque_zero(it)
        mask = true_mask(zd)
        for par in (1, 0):
            c = 2 * it + (1 if par == 1 else 2)
            blk_c = _C1[0] + (c - 1) * _CB
            for k in range(3):
                @pl.when(it == k)
                def _():
                    ck = 2 * k + (1 if par == 1 else 2)
                    wait_parts(ck)
                    start_parts(ck + 1)
                    if ck == 1:
                        cp_w2.wait()
                    if ck == 5:
                        for cp in small:
                            cp.start()
            block(lambda: _emit_step(
                conv_items(v1, specs[par], ys[par], _CB * 16),
                _merge(fx_units(specs[1 - par], blk_c + _CB, _CB, zd, mask),
                       inv_units(ys[1 - par], hbuf, 1.0,
                                 jnp.maximum(blk_c - _CB, 0), _CB, mask),
                       w2_units(2 * c - 2, 2, mask)), mask), zd)
        return carry
    with jax.named_scope("conv1"):
        lax.fori_loop(0, 3, conv1_body, 0)

    sub = lax.broadcasted_iota(jnp.int32, (16, _D), 0) % 8

    def mask_rows(r0, r1, s):
        def body(r, carry):
            hbuf[r] = jnp.where(sub == s, 0.0, hbuf[r])
            return carry
        lax.fori_loop(r0, r1, body, 0)
    mask_rows(0, 16, 0)

    def step7_body():
        zd, mask = zd0, mask0
        _emit_step(conv_items(v1, spec_b, y_b, _CB * 16),
                   _merge(fh_units(spec_a, 0, _CB2, mask),
                          inv_units(y_a, hbuf, 1.0, c1_start[6], _CB, mask),
                          w2_units(12, 4, mask)), mask)
    with jax.named_scope("step7"):
        block(step7_body, zd0)

    fscale = 0.5 / _C0

    def step8_body():
        zd, mask = zd0, mask0
        _emit_step(conv_items(v2, spec_a, y_a, _CB2 * 16),
                   _merge(fh_units(spec_b, _CB2, _CB2, mask),
                          inv_units(y_b, hbuf, 1.0, c1_start[7], _CB, mask)), mask)
    with jax.named_scope("step8"):
        block(step8_body, zd0)
    mask_rows(_T1 - 7 * _S1 + 16, _NB1 * hop, 7)

    def conv2_body(it, carry):
        zd = opaque_zero(it)
        mask = true_mask(zd)
        for par in (1, 0):
            c = 2 * it + (1 if par == 1 else 2)
            block(lambda: _emit_step(
                conv_items(v2, specs[par], ys[par], _CB2 * 16),
                _merge(fh_units(specs[1 - par], (c + 1) * _CB2, _CB2, mask),
                       inv_units(ys[1 - par], fbuf, fscale, (c - 1) * _CB2, _CB2, mask)),
                mask), zd)
        return carry
    with jax.named_scope("conv2"):
        lax.fori_loop(0, 2, conv2_body, 0)

    for c in small:
        c.wait()
    gebuf[...] = jnp.dot(gbuf[...].reshape(_B * _U, _D), wgbuf[...],
                         preferred_element_type=jnp.float32).reshape(_B, _U, _D)

    def fe_item(slot, tile):
        def dot_fn():
            f = fbuf[pl.ds(tile * _TJ, _TJ)].reshape(_TJ * 16, _D)
            return jnp.dot(f, wfbuf[...], preferred_element_type=jnp.float32)

        def post(r):
            febuf[slot] = r.reshape(_TJ, 16, _D)
        return (_TJ * 16, dot_fn, post)

    def step13_body():
        zd, mask = zd0, mask0
        _emit_step(conv_items(v2, spec_b, y_b, _CB2 * 16) + [fe_item(0, 0)],
                   inv_units(y_a, fbuf, fscale, 4 * _CB2, _CB2, mask), mask)
    with jax.named_scope("step13"):
        block(step13_body, zd0)

    def out_copies(slot, t0, rows_of):
        cps = []
        for s in range(8):
            rows = rows_of(s)
            if rows > 0:
                cps.append(pltpu.make_async_copy(
                    obuf.at[slot, :, s, pl.ds(0, rows)],
                    out_hbm.at[:, pl.ds(s * _S2 + t0, rows)],
                    sem_o.at[slot]))
        return cps

    def joint_item(slot, tj):
        def dot_fn():
            rows = []
            for tt in range(tj):
                for r in range(16):
                    fr = febuf[slot, tt, pl.ds(r, 1), :]
                    rows.append(jnp.tanh(jnp.broadcast_to(fr, (_U, _D)) + gebuf[r // 8]))
            return jnp.dot(jnp.concatenate(rows, axis=0), wobuf[...],
                           preferred_element_type=jnp.float32)

        def post(o):
            o = o.reshape(tj, _B, 8, _U, _D).astype(jnp.bfloat16)
            for tt in range(tj):
                obuf[slot, :, :, tt] = o[tt]
        return (tj * 16 * _U, dot_fn, post)

    full = lambda s: _TJ
    ntiles = -(-_S2 // _TJ)
    nfull = (_T2 - 7 * _S2) // _TJ
    assert nfull % 2 == 0

    def first_body():
        zd, mask = zd0, mask0
        _emit_step([fe_item(1, 1), joint_item(0, _TJ), fe_item(0, 2), joint_item(1, _TJ)],
                   inv_units(y_b, fbuf, fscale, 5 * _CB2, _CB2, mask), mask)
        for slot in range(2):
            for c in out_copies(slot, slot * _TJ, full):
                c.start()
    with jax.named_scope("first"):
        block(first_body, zd0)

    def joint_body(i2, carry):
        for slot in range(2):
            tile = 2 * i2 + slot
            t0 = tile * _TJ
            for c in out_copies(slot, t0 - 2 * _TJ, full):
                c.wait()
            _emit_step([fe_item(1 - slot, jnp.minimum(tile + 1, ntiles - 1)), joint_item(slot, _TJ)],
                       [], None)
            for c in out_copies(slot, t0, full):
                c.start()
        return carry
    with jax.named_scope("joint"):
        lax.fori_loop(1, nfull // 2, joint_body, 0)

    pending = {0: out_copies(0, (nfull - 2) * _TJ, full),
               1: out_copies(1, (nfull - 1) * _TJ, full)}
    for tile in range(nfull, ntiles):
        slot, t0 = tile % 2, tile * _TJ
        tj = min(_TJ, _S2 - t0)
        rows_of = lambda s, t0=t0, tj=tj: max(0, min(tj, (_T2 - 7 * _S2 if s == 7 else _S2) - t0))
        for c in pending[slot]:
            c.wait()
        items = ([fe_item(1 - slot, tile + 1)] if tile + 1 < ntiles else []) + [joint_item(slot, tj)]
        _emit_step(items, [], None)
        pending[slot] = out_copies(slot, t0, rows_of)
        for c in pending[slot]:
            c.start()
    for slot in range(2):
        for c in pending[slot]:
            c.wait()


@jax.jit
def pallas_standalone__seq2seq_rnn_t_joint__speech_kernel(
    x: jax.Array,
    w1: jax.Array,
    w2: jax.Array,
    g: jax.Array,
    w_f: jax.Array,
    w_g: jax.Array,
    w_o: jax.Array,
):
    assert x.shape == (_B, _T, _D) and w1.shape == (_K, _D, _D) and w2.shape == (_K, _D, _D)
    assert g.shape == (_B, _U, _D)
    bf, f32 = jnp.bfloat16, jnp.float32
    m = _CB * 16
    scratch = [
        pltpu.VMEM((_NS, 2, 256, 128), jnp.uint32),
        pltpu.VMEM((_NS, 2, 256, 128), jnp.uint32),
        pltpu.VMEM((4, _NS, m + 8, 128), f32),
        pltpu.VMEM((4, _NS, m + 8, 128), f32),
        pltpu.VMEM((2, _NS, m + 8, 128), f32),
        pltpu.VMEM((2, _NS, m + 8, 128), f32),
        pltpu.VMEM((_HROWS, 16, _D), f32),
        pltpu.VMEM((2, 2, _XROWS, 128), jnp.uint32),
        pltpu.VMEM((_K, _D, _D), bf),
        pltpu.VMEM((_K, _D, _D), bf),
        pltpu.VMEM((_B, _U, _D), bf),
        pltpu.VMEM((_D, _D), bf),
        pltpu.VMEM((_D, _D), bf),
        pltpu.VMEM((_D, _D), bf),
        pltpu.VMEM((_B, _U, _D), f32),
        pltpu.VMEM((_FROWS, 16, _D), f32),
        pltpu.VMEM((2, _TJ, 16, _D), f32),
        pltpu.VMEM((2, _B, 8, _TJ, _U, _D), bf),
        pltpu.SemaphoreType.DMA((_WPARTS + 1,)),
        pltpu.SemaphoreType.DMA((4,)),
        pltpu.SemaphoreType.DMA((_XPARTS,)),
        pltpu.SemaphoreType.DMA((2,)),
    ]
    any_spec = pl.BlockSpec(memory_space=pl.ANY)
    return pl.pallas_call(
        _kernel,
        out_shape=jax.ShapeDtypeStruct((_B, _T2, _U, _D), bf),
        in_specs=[any_spec] * 7,
        out_specs=any_spec,
        scratch_shapes=scratch,
        compiler_params=pltpu.CompilerParams(vmem_limit_bytes=127 * 1024 * 1024),
    )(x, w1, w2, g, w_f, w_g, w_o)
```

```python
import functools
import math

import numpy as np

import jax
import jax.numpy as jnp
from jax import lax
import jax.experimental.pallas as pl
import jax.experimental.pallas.tpu as pltpu


class _Prog:
    def __init__(self):
        self.ops = []
        self.cse = {}

    def _node(self, kind, a, b):
        key = (kind, a, b)
        if key not in self.cse:
            self.ops.append(key)
            self.cse[key] = len(self.ops) - 1
        return self.cse[key]

    def inp(self, i):
        return (self._node("in", i, None), 1)

    def neg(self, x):
        return None if x is None else (x[0], -x[1])

    def add(self, x, y):
        if x is None:
            return y
        if y is None:
            return x
        (a, sa), (b, sb) = x, y
        if sa == sb:
            return (self._node("add", min(a, b), max(a, b)), sa)
        if sa > 0:
            return (self._node("sub", a, b), 1)
        return (self._node("sub", b, a), 1)

    def sub(self, x, y):
        return self.add(x, self.neg(y))

    def mul(self, c, x):
        if x is None or c == 0:
            return None
        if c == 1:
            return x
        if c == -1:
            return self.neg(x)
        return (self._node("mul", x[0], abs(float(c))), x[1] * (1 if c > 0 else -1))

    def cadd(self, z, w):
        return (self.add(z[0], w[0]), self.add(z[1], w[1]))

    def csub(self, z, w):
        return (self.sub(z[0], w[0]), self.sub(z[1], w[1]))

    def cconj(self, z):
        return (z[0], self.neg(z[1]))

    def twiddle(self, z, num, den):
        num %= den
        a, b = z
        if (8 * num) % den == 0:
            e = (8 * num) // den
            r = math.sqrt(0.5)
            if e == 0:
                return (a, b)
            if e == 2:
                return (b, self.neg(a))
            if e == 4:
                return (self.neg(a), self.neg(b))
            if e == 6:
                return (self.neg(b), a)
            if e == 1:
                return (self.mul(r, self.add(a, b)), self.mul(r, self.sub(b, a)))
            if e == 3:
                return (self.mul(r, self.sub(b, a)), self.mul(-r, self.add(a, b)))
            if e == 5:
                return (self.mul(-r, self.add(a, b)), self.mul(r, self.sub(a, b)))
            return (self.mul(r, self.sub(a, b)), self.mul(r, self.add(a, b)))
        th = -2.0 * math.pi * num / den
        c, s = math.cos(th), math.sin(th)
        return (self.sub(self.mul(c, a), self.mul(s, b)), self.add(self.mul(s, a), self.mul(c, b)))

    def rfft(self, xs):
        n = len(xs)
        if n == 1:
            return [(xs[0], None)]
        if n == 2:
            return [(self.add(xs[0], xs[1]), None), (self.sub(xs[0], xs[1]), None)]
        if n == 4:
            a = self.add(xs[0], xs[2])
            b = self.sub(xs[0], xs[2])
            c = self.add(xs[1], xs[3])
            d = self.sub(xs[1], xs[3])
            return [(self.add(a, c), None), (b, self.neg(d)), (self.sub(a, c), None)]
        u = self.rfft(xs[0::2])
        z1 = self.rfft(xs[1::4])
        z3 = self.rfft(xs[3::4])

        def get_u(k):
            k %= n // 2
            return u[k] if k <= n // 4 else self.cconj(u[n // 2 - k])

        out = [None] * (n // 2 + 1)
        for k in range(n // 8 + 1):
            t1 = self.twiddle(z1[k], k, n)
            t3 = self.twiddle(z3[k], 3 * k, n)
            sm = self.cadd(t1, t3)
            df = self.csub(t1, t3)
            u0, u1 = get_u(k), get_u(k + n // 4)
            out[k] = self.cadd(u0, sm)
            out[n // 2 - k] = self.cconj(self.csub(u0, sm))
            mdf = (df[1], self.neg(df[0]))
            out[k + n // 4] = self.cadd(u1, mdf)
            if k > 0:
                out[n // 4 - k] = self.cconj(self.csub(u1, mdf))
        return out

    def order(self, outs):
        seen, order = set(), []
        for o in outs:
            if o is None or o[0] in seen:
                continue
            stack = [(o[0], False)]
            while stack:
                n, done = stack.pop()
                if done:
                    order.append(n)
                    continue
                if n in seen:
                    continue
                seen.add(n)
                stack.append((n, True))
                kind, a, b = self.ops[n]
                if kind in ("add", "sub"):
                    stack.append((b, False))
                    stack.append((a, False))
                elif kind == "mul":
                    stack.append((a, False))
        return order

    def transpose(self, outs):
        g = _Prog()
        adj = {}

        def acc(n, v):
            if v is not None:
                adj[n] = g.add(adj.get(n), v)

        for i, o in enumerate(outs):
            if o is not None:
                acc(o[0], g.mul(o[1], g.inp(i)))
        res = {}
        for n in sorted(set(self.order(outs)), reverse=True):
            kind, a, b = self.ops[n]
            v = adj.get(n)
            if v is None:
                continue
            if kind == "in":
                res[a] = v
            elif kind == "add":
                acc(a, v)
                acc(b, v)
            elif kind == "sub":
                acc(a, v)
                acc(b, g.neg(v))
            else:
                acc(a, g.mul(b, v))
        return g, res

    def run(self, outs, load, emit, keep_sign=True):
        val = {}
        want = {}
        for i, o in enumerate(outs):
            if o is not None:
                want.setdefault(o[0], []).append((i, o[1]))
        for n in self.order(outs):
            kind, a, b = self.ops[n]
            if kind == "in":
                v = load(a)
            elif kind == "add":
                v = val[a] + val[b]
            elif kind == "sub":
                v = val[a] - val[b]
            else:
                v = val[a] * np.float32(b)
            val[n] = v
            for i, sg in want.get(n, ()):
                emit(i, -v if (sg < 0 and keep_sign) else v)


def _lhs_outputs(p, spec, n):
    outs = [spec[0][0], spec[n // 2][0]]
    for k in range(1, n // 2):
        a, b = spec[k]
        outs += [p.add(a, b), a, b]
    return outs


class _Plan:
    def __init__(self, n):
        self.n = n
        self.taps = 16
        self.hop = n - self.taps + 1
        self.ns = 2 + 3 * (n // 2 - 1)
        self.fwd = _Prog()
        spec = self.fwd.rfft([self.fwd.inp(i) for i in range(n)])
        self.fwd_outs = _lhs_outputs(self.fwd, spec, n)
        lhs_sign = [o[1] for o in self.fwd_outs]
        p = _Prog()
        spec = p.rfft([p.inp(i) if i < self.hop else None for i in range(n)])
        self.inv, res = p.transpose(_lhs_outputs(p, spec, n))
        self.inv_outs = [res[t] for t in range(self.hop)]
        self.inv_src = [0, 1]
        for k in range(n // 2 - 1):
            base = 2 + 3 * k
            self.inv_src += [base, base + 2, base + 1]
        self.wprog, self.wouts, self.wtap = [], [], []
        for ph in range(2):
            p = _Prog()
            xs = [None] * n
            for j in range(self.taps):
                if not (ph == 0 and j == 0):
                    xs[j] = p.inp(2 * j - 1 if ph == 0 else 2 * j)
            spec = p.rfft(xs)
            outs = [p.mul(0.5, spec[0][0]), p.mul(0.5, spec[n // 2][0])]
            for k in range(1, n // 2):
                c, dm = spec[k]
                d = p.neg(dm)
                outs += [c, p.sub(d, c), p.neg(p.add(c, d))]
            outs = [(o[0], o[1] * s) for o, s in zip(outs, lhs_sign)]
            self.wprog.append(p)
            self.wouts.append(outs)


_FFT_N = 32
_PLAN = _Plan(_FFT_N)

_C0 = math.sqrt(2.0 / math.pi)
_KAPPA = 0.044715 / (_C0 * _C0)


def _gelu2(z):
    inner = z * (np.float32(_KAPPA) * (z * z) + np.float32(1.0))
    return z + z * jnp.tanh(inner)


_B, _T, _D, _K, _U = 2, 16000, 256, 31, 8
_T1, _T2 = _T // 2, _T // 4
_S2 = 502
_S1 = 2 * _S2
_HOP = _PLAN.hop
_NS = _PLAN.ns
_CB = 8
_C1 = [5] + [_CB] * 7
_CB2, _NSTEP2 = 5, 6
_NB1 = sum(_C1)
_XOFF = 24
_XROWS = -(-(7 * _S1 + _HOP * (_NB1 - 1) + _FFT_N) // 8) * 8
_HROWS = 2 * _HOP * (_CB2 * _NSTEP2 - 1) + 2 * _FFT_N
_FROWS = _HOP * _CB2 * _NSTEP2
_TJ = _HOP
_XPARTS = 8
_OSLOTS = 4
_WPARTS = 4
_NDEP = 2
_COST = {"fx": 262, "fh": 230, "inv": 350, "w": 280}


def _x_piece_bounds():
    edges = []
    for s in range(8):
        for p in range(_XPARTS):
            edges.append(min(max((s * _S1 + p * (_S1 // _XPARTS) - _XOFF) // 8 * 8, 0), _T1))
    edges.append(_T1)
    return edges


def _merge(*lists):
    lists = [l for l in lists if l]
    pos = [0] * len(lists)
    out = []
    for _ in range(sum(len(l) for l in lists)):
        j = min((q for q in range(len(lists)) if pos[q] < len(lists[q])),
                key=lambda q: (pos[q] + 0.5) / len(lists[q]))
        out.append(lists[j][pos[j]])
        pos[j] += 1
    return out


def _dyn8(v):
    return v if isinstance(v, int) else pl.multiple_of(v, 8)


def _emit_step(items, units, mask):
    starts = np.cumsum([0] + [2 * (rows // 8) for rows, _, _ in items])
    nev = int(starts[-1])
    tot = sum(c for c, _ in units) or 1
    margin = min(40, nev // 8)
    sched, cum = [], 0
    for cost, fn in units:
        evs = [min(int((cum + cost * q / _NDEP) / tot * (nev - margin)) + 1, nev - 1)
               for q in range(_NDEP)]
        cum += cost
        sched.append((fn, evs))
    results = {}

    def event(e):
        j = int(np.searchsorted(starts, e, side="right")) - 1
        rg, nn = divmod(e - int(starts[j]), 2)
        return results[j][rg * 8:(rg + 1) * 8, nn * 128:(nn + 1) * 128]

    pi = 0
    for j, (rows, dot_fn, post_fn) in enumerate(items):
        results[j] = dot_fn()
        while pi < len(sched) and max(sched[pi][1]) < starts[j + 1]:
            fn, evs = sched[pi]
            pi += 1
            fn([functools.partial(event, e) for e in evs])
        post_fn(results[j])
    assert pi == len(sched)


def _pick(cnt, total, deps):
    if not deps:
        return None
    j, rem = divmod(cnt * len(deps), total)
    return j if rem < len(deps) else None


def _kernel(x_hbm, w1_hbm, w2_hbm, g_hbm, wf_hbm, wg_hbm, wo_hbm, out_hbm,
            v1, v2, spec_a, spec_b, y_a, y_b, hbuf, xbuf, w1buf, w2buf,
            gbuf, wfbuf, wgbuf, wobuf, gebuf, fbuf, febuf, obuf,
            sem_w, sem_s, sem_x, sem_o):
    plan = _PLAN
    n, hop, ns = plan.n, plan.hop, plan.ns
    specs, ys = (spec_a, spec_b), (y_a, y_b)

    xu = x_hbm.bitcast(jnp.uint32)
    edges = _x_piece_bounds()

    def x_copies(part):
        cps = []
        for s in range(8):
            r0, r1 = edges[s * _XPARTS + part], edges[s * _XPARTS + part + 1]
            for cs in range(2):
                cps.append(pltpu.make_async_copy(
                    xu.at[:, pl.ds(r0, r1 - r0), pl.ds(cs * 128, 128)],
                    xbuf.at[:, cs, pl.ds(_XOFF + r0, r1 - r0), :],
                    sem_x.at[part]))
        return cps

    wrows = _D // _WPARTS
    w1_copies = [pltpu.make_async_copy(w1_hbm.at[:, pl.ds(p * wrows, wrows), :],
                                       w1buf.at[:, pl.ds(p * wrows, wrows), :], sem_w.at[p])
                 for p in range(_WPARTS)]
    cp_w2 = pltpu.make_async_copy(w2_hbm, w2buf, sem_w.at[_WPARTS])
    small = [pltpu.make_async_copy(src, dst, sem_s.at[i]) for i, (src, dst) in
             enumerate([(g_hbm, gbuf), (wf_hbm, wfbuf), (wg_hbm, wgbuf), (wo_hbm, wobuf)])]

    for c in w1_copies:
        c.start()
    zero8 = jnp.zeros((8, 128), jnp.uint32)
    for bb in range(2):
        for cs in range(2):
            for r in range(0, _XOFF, 8):
                xbuf[bb, cs, pl.ds(r, 8), :] = zero8
            for r in range(_XOFF + _T1, _XROWS, 8):
                xbuf[bb, cs, pl.ds(r, 8), :] = zero8
    zrow = jnp.zeros((8, 128), jnp.float32)
    for bb in range(2):
        for cs in range(2):
            for r in range(_NB1 * hop, _HROWS):
                hbuf[bb, cs, r] = zrow

    def w_unit(wbuf, vbuf, scale, row, half, ph, nt, deps=(), mask=None):
        cnt = [0]

        def load(tap):
            w = wbuf[tap, pl.ds(_dyn8(row + 8 * half), 8), pl.ds(nt * 128, 128)].astype(jnp.float32)
            j = _pick(cnt[0], 16, deps)
            cnt[0] += 1
            if j is not None:
                w = jnp.where(mask, w, deps[j]())
            return w * np.float32(scale)

        def emit(i, v):
            vbuf[i, 2 * ph + row // 128, nt, pl.ds(_dyn8((row % 128) // 2) + 4 * half, 4), :] = (
                pltpu.bitcast(v.astype(jnp.bfloat16), jnp.uint32))
        plan.wprog[ph].run(plan.wouts[ph], load, emit)

    def fwd_unit(load_in, spec, row, col, deps, mask):
        cnt = [0]

        def load(q):
            j = _pick(cnt[0], n, deps)
            cnt[0] += 1
            return load_in(q, None if j is None else deps[j], mask)

        def emit(i, v):
            spec[col // 128, i, pl.ds(row, 8), :] = v
        plan.fwd.run(plan.fwd_outs, load, emit, keep_sign=False)

    def fx_unit(spec, blk, be, bb, cs, ph, zd, deps=(), mask=None):
        base = blk * hop
        if ph == 1:
            base = base + zd

        def load_in(q, dep, mask):
            v = xbuf[bb, cs, pl.ds(base + q, 8, stride=_S1), :]
            if dep is not None:
                v = jnp.where(mask, v, lax.bitcast_convert_type(dep(), jnp.uint32))
            v = (v << 16) if ph == 0 else (v & jnp.uint32(0xFFFF0000))
            return lax.bitcast_convert_type(v, jnp.float32)
        fwd_unit(load_in, spec, _dyn8(be * 16 + bb * 8), ph * 256 + cs * 128, deps, mask)

    def fh_unit(spec, blk, be, bb, cs, ph, deps=(), mask=None):
        base = blk * 2 * hop + ph

        def load_in(q, dep, mask):
            v = hbuf[bb, cs, base + 2 * q]
            if dep is not None:
                v = jnp.where(mask, v, dep())
            return v
        fwd_unit(load_in, spec, _dyn8(be * 16 + bb * 8), ph * 256 + cs * 128, deps, mask)

    def inv_unit(ybuf, dst, scale, blk, be, bb, nt, deps=(), mask=None):
        cnt = [0]
        row = _dyn8(be * 16 + bb * 8)

        def load(i):
            v = ybuf[nt, plan.inv_src[i], pl.ds(row, 8), :]
            j = _pick(cnt[0], ns, deps)
            cnt[0] += 1
            if j is not None:
                v = jnp.where(mask, v, deps[j]())
            return v

        def store(t, z):
            hval = _gelu2(z)
            if scale != 1.0:
                hval = hval * np.float32(scale)
            dst[bb, nt, blk * hop + t] = hval
        plan.inv.run(plan.inv_outs, load, store)

    def fx_units(spec, blk0, nblk, zd, mask):
        return [(_COST["fx"], functools.partial(fx_unit, spec, blk0 + be, be, bb, cs, ph, zd, mask=mask))
                for be in range(nblk) for bb in range(2) for cs in range(2) for ph in range(2)]

    def fh_units(spec, blk0, nblk, mask):
        return [(_COST["fh"], functools.partial(fh_unit, spec, blk0 + be, be, bb, cs, ph, mask=mask))
                for be in range(nblk) for bb in range(2) for cs in range(2) for ph in range(2)]

    def inv_units(ybuf, dst, scale, blk0, nblk, mask):
        return [(_COST["inv"], functools.partial(inv_unit, ybuf, dst, scale, blk0 + be, be, bb, nt, mask=mask))
                for be in range(nblk) for bb in range(2) for nt in range(2)]

    def w2_units(rg0, nrg, mask):
        return [(_COST["w"], functools.partial(
                    w_unit, w2buf, v2, (2.0 / n) * 0.5, pl.multiple_of((rg0 + r) * 16, 16)
                    if not isinstance(rg0, int) else (rg0 + r) * 16, half, ph, nt, mask=mask))
                for r in range(nrg) for half in range(2) for ph in range(2) for nt in range(2)]

    def conv_items(vbuf, spec, ybuf, m):
        items = []
        for i in range(ns):
            hold = []

            def dot_fn(i=i, h=0):
                w = jnp.concatenate(
                    [jnp.concatenate(
                        [pltpu.bitcast(vbuf[i, 2 * h + q, nt, pl.ds(0, 64), :], jnp.bfloat16)
                         for q in range(2)], axis=0) for nt in range(2)], axis=1)
                lhs = jnp.concatenate([spec[2 * h + q, i, pl.ds(0, m), :] for q in range(2)], axis=1)
                return jnp.dot(lhs, w, preferred_element_type=jnp.float32)

            def post0(r, hold=hold):
                hold.append(r)

            def post1(r, i=i, hold=hold):
                y = hold[0] + r
                for nt in range(2):
                    ybuf[nt, i, pl.ds(0, m), :] = y[:, nt * 128:(nt + 1) * 128]
            items.append((m, functools.partial(dot_fn, i, 0), post0))
            items.append((m, functools.partial(dot_fn, i, 1), post1))
        return items

    def block(fn, zd):
        def body(_, c):
            fn()
            return c
        lax.fori_loop(0, 1 + zd, body, 0)

    def opaque_zero(i):
        return (i * (i + 1)) & 1

    def true_mask(zd):
        return jnp.full((8, 128), zd, jnp.int32) == 0

    c1_start = [int(v) for v in np.cumsum([0] + _C1)]

    def v1_body(rg, carry):
        for p in range(_WPARTS):
            @pl.when(rg == p * (wrows // 16))
            def _():
                w1_copies[p].wait()
                if p == 0:
                    for c in x_copies(0):
                        c.start()
                if p == 2:
                    for c in x_copies(1):
                        c.start()
        row = pl.multiple_of(rg * 16, 16)
        for half in range(2):
            for ph in range(2):
                for nt in range(2):
                    w_unit(w1buf, v1, (2.0 / n) * _C0, row, half, ph, nt)
        return carry
    with jax.named_scope("v1"):
        lax.fori_loop(0, _D // 16, v1_body, 0)

    zd0 = opaque_zero(xbuf[0, 0, 0, 0].astype(jnp.int32))
    mask0 = true_mask(zd0)

    need = {0: [1], 1: [2], 2: [3, 4], 3: [5], 4: [6], 5: [7], 6: []}

    def start_parts(c):
        for p in need.get(c, []):
            for cp in x_copies(p):
                cp.start()

    def wait_parts(c):
        for p in need.get(c, []):
            for cp in x_copies(p):
                cp.wait()

    with jax.named_scope("x0wait"):
        for c in x_copies(0):
            c.wait()

    def fill_body(u, carry):
        zd = opaque_zero(u)
        for cs in range(2):
            for ph in range(2):
                fx_unit(spec_a, u // 2, u // 2, u % 2, cs, ph, zd)
        return carry
    with jax.named_scope("fill"):
        lax.fori_loop(0, _C1[0] * 2, fill_body, 0)

    with jax.named_scope("x1wait"):
        wait_parts(0)
    cp_w2.start()
    start_parts(1)

    def step0_body():
        zd, mask = zd0, mask0
        _emit_step(conv_items(v1, spec_a, y_a, _C1[0] * 16),
                   fx_units(spec_b, c1_start[1], _CB, zd, mask), mask)
    with jax.named_scope("step0"):
        block(step0_body, zd0)

    def conv1_body(it, carry):
        zd = opaque_zero(it)
        mask = true_mask(zd)
        for par in (1, 0):
            c = 2 * it + (1 if par == 1 else 2)
            blk_c = _C1[0] + (c - 1) * _CB
            for k in range(3):
                @pl.when(it == k)
                def _():
                    ck = 2 * k + (1 if par == 1 else 2)
                    wait_parts(ck)
                    start_parts(ck + 1)
                    if ck == 1:
                        cp_w2.wait()
                    if ck == 5:
                        for cp in small:
                            cp.start()
            block(lambda: _emit_step(
                conv_items(v1, specs[par], ys[par], _CB * 16),
                _merge(fx_units(specs[1 - par], blk_c + _CB, _CB, zd, mask) +
                       inv_units(ys[1 - par], hbuf, 1.0,
                                 jnp.maximum(blk_c - _CB, 0), _CB, mask),
                       w2_units(2 * c - 2, 2, mask)), mask), zd)
        return carry
    with jax.named_scope("conv1"):
        lax.fori_loop(0, 3, conv1_body, 0)

    sub = lax.broadcasted_iota(jnp.int32, (8, 128), 0)

    def mask_rows(r0, r1, s):
        def body(r, carry):
            for bb in range(2):
                for cs in range(2):
                    hbuf[bb, cs, r] = jnp.where(sub == s, 0.0, hbuf[bb, cs, r])
            return carry
        lax.fori_loop(r0, r1, body, 0)
    mask_rows(0, 16, 0)

    def step7_body():
        zd, mask = zd0, mask0
        _emit_step(conv_items(v1, spec_b, y_b, _CB * 16),
                   _merge(fh_units(spec_a, 0, _CB2, mask),
                          inv_units(y_a, hbuf, 1.0, c1_start[6], _CB, mask),
                          w2_units(12, 4, mask)), mask)
    with jax.named_scope("step7"):
        block(step7_body, zd0)

    fscale = 0.5 / _C0

    def step8_body():
        zd, mask = zd0, mask0
        _emit_step(conv_items(v2, spec_a, y_a, _CB2 * 16),
                   _merge(fh_units(spec_b, _CB2, _CB2, mask),
                          inv_units(y_b, hbuf, 1.0, c1_start[7], _CB, mask)), mask)
    with jax.named_scope("step8"):
        block(step8_body, zd0)
    mask_rows(_T1 - 7 * _S1 + 16, _NB1 * hop, 7)

    def conv2_body(it, carry):
        zd = opaque_zero(it)
        mask = true_mask(zd)
        for par in (1, 0):
            c = 2 * it + (1 if par == 1 else 2)
            block(lambda: _emit_step(
                conv_items(v2, specs[par], ys[par], _CB2 * 16),
                (fh_units(specs[1 - par], (c + 1) * _CB2, _CB2, mask) +
                 inv_units(ys[1 - par], fbuf, fscale, (c - 1) * _CB2, _CB2, mask)),
                mask), zd)
        return carry
    with jax.named_scope("conv2"):
        lax.fori_loop(0, 2, conv2_body, 0)

    for c in small:
        c.wait()
    gebuf[...] = jnp.dot(gbuf[...].reshape(_B * _U, _D), wgbuf[...],
                         preferred_element_type=jnp.float32).reshape(_B, _U, _D)

    def fe_item(slot, tile):
        def dot_fn():
            f = jnp.concatenate(
                [jnp.concatenate(
                    [fbuf[bb, cs, pl.ds(tile * _TJ, _TJ)].reshape(_TJ * 8, 128) for cs in range(2)],
                    axis=1) for bb in range(2)], axis=0)
            return jnp.dot(f, wfbuf[...], preferred_element_type=jnp.float32)

        def post(r):
            febuf[slot] = r.reshape(_B, _TJ, 8, _D)
        return (_TJ * 16, dot_fn, post)

    def step13_body():
        zd, mask = zd0, mask0
        _emit_step(conv_items(v2, spec_b, y_b, _CB2 * 16) + [fe_item(0, 0)],
                   inv_units(y_a, fbuf, fscale, 4 * _CB2, _CB2, mask), mask)
    with jax.named_scope("step13"):
        block(step13_body, zd0)

    def out_copies(slot, t0, rows_of):
        cps = []
        for s in range(8):
            rows = rows_of(s)
            if rows > 0:
                cps.append(pltpu.make_async_copy(
                    obuf.at[slot, :, s, pl.ds(0, rows)],
                    out_hbm.at[:, pl.ds(s * _S2 + t0, rows)],
                    sem_o.at[slot]))
        return cps

    def joint_item(fslot, oslot, tj):
        def dot_fn():
            rows = []
            for tt in range(tj):
                for r in range(16):
                    fr = febuf[fslot, r // 8, tt, pl.ds(r % 8, 1), :]
                    rows.append(jnp.tanh(jnp.broadcast_to(fr, (_U, _D)) + gebuf[r // 8]))
            return jnp.dot(jnp.concatenate(rows, axis=0), wobuf[...],
                           preferred_element_type=jnp.float32)

        def post(o):
            o = o.reshape(tj, _B, 8, _U, _D).astype(jnp.bfloat16)
            for tt in range(tj):
                obuf[oslot, :, :, tt] = o[tt]
        return (tj * 16 * _U, dot_fn, post)

    full = lambda s: _TJ
    ntiles = -(-_S2 // _TJ)
    nfull = (_T2 - 7 * _S2) // _TJ
    assert nfull % _OSLOTS == 0 and _OSLOTS == 4

    def first_body():
        _emit_step([fe_item(1, 1), joint_item(0, 0, _TJ), fe_item(0, 2), joint_item(1, 1, _TJ)],
                   inv_units(y_b, fbuf, fscale, 5 * _CB2, _CB2, mask0), mask0)
        for slot in range(2):
            for c in out_copies(slot, slot * _TJ, full):
                c.start()
    with jax.named_scope("first"):
        block(first_body, zd0)

    def joint_body(i2, carry):
        for j in range(2):
            tile = 2 * i2 + j
            oslot = (i2 % 2) * 2 + j
            t0 = tile * _TJ

            @pl.when(i2 >= 2)
            def _():
                for c in out_copies(oslot, t0 - _OSLOTS * _TJ, full):
                    c.wait()
            _emit_step([fe_item(1 - j, tile + 1), joint_item(j, oslot, _TJ)], [], None)
            for c in out_copies(oslot, t0, full):
                c.start()
        return carry
    with jax.named_scope("joint"):
        lax.fori_loop(1, nfull // 2, joint_body, 0)

    pending = {k: out_copies(k, (nfull - _OSLOTS + k) * _TJ, full) for k in range(_OSLOTS)}
    for tile in range(nfull, ntiles):
        oslot, t0 = tile % _OSLOTS, tile * _TJ
        tj = min(_TJ, _S2 - t0)
        rows_of = lambda s, t0=t0, tj=tj: max(0, min(tj, (_T2 - 7 * _S2 if s == 7 else _S2) - t0))
        for c in pending[oslot]:
            c.wait()
        items = ([fe_item(1 - tile % 2, tile + 1)] if tile + 1 < ntiles else []) + [
            joint_item(tile % 2, oslot, tj)]
        _emit_step(items, [], None)
        pending[oslot] = out_copies(oslot, t0, rows_of)
        for c in pending[oslot]:
            c.start()
    for k in range(_OSLOTS):
        for c in pending[k]:
            c.wait()


@jax.jit
def pallas_standalone__seq2seq_rnn_t_joint__speech_kernel(
    x: jax.Array,
    w1: jax.Array,
    w2: jax.Array,
    g: jax.Array,
    w_f: jax.Array,
    w_g: jax.Array,
    w_o: jax.Array,
):
    assert x.shape == (_B, _T, _D) and w1.shape == (_K, _D, _D) and w2.shape == (_K, _D, _D)
    assert g.shape == (_B, _U, _D)
    bf, f32 = jnp.bfloat16, jnp.float32
    m = _CB * 16
    scratch = [
        pltpu.VMEM((_NS, 4, 2, 72, 128), jnp.uint32),
        pltpu.VMEM((_NS, 4, 2, 72, 128), jnp.uint32),
        pltpu.VMEM((4, _NS, m + 8, 128), f32),
        pltpu.VMEM((4, _NS, m + 8, 128), f32),
        pltpu.VMEM((2, _NS, m + 8, 128), f32),
        pltpu.VMEM((2, _NS, m + 8, 128), f32),
        pltpu.VMEM((2, 2, _HROWS + 1, 8, 128), f32),
        pltpu.VMEM((2, 2, _XROWS, 128), jnp.uint32),
        pltpu.VMEM((_K, _D, _D), bf),
        pltpu.VMEM((_K, _D, _D), bf),
        pltpu.VMEM((_B, _U, _D), bf),
        pltpu.VMEM((_D, _D), bf),
        pltpu.VMEM((_D, _D), bf),
        pltpu.VMEM((_D, _D), bf),
        pltpu.VMEM((_B, _U, _D), f32),
        pltpu.VMEM((2, 2, _FROWS + 1, 8, 128), f32),
        pltpu.VMEM((2, _B, _TJ, 8, _D), f32),
        pltpu.VMEM((_OSLOTS, _B, 8, _TJ, _U, _D), bf),
        pltpu.SemaphoreType.DMA((_WPARTS + 1,)),
        pltpu.SemaphoreType.DMA((4,)),
        pltpu.SemaphoreType.DMA((_XPARTS,)),
        pltpu.SemaphoreType.DMA((_OSLOTS,)),
    ]
    any_spec = pl.BlockSpec(memory_space=pl.ANY)
    return pl.pallas_call(
        _kernel,
        out_shape=jax.ShapeDtypeStruct((_B, _T2, _U, _D), bf),
        in_specs=[any_spec] * 7,
        out_specs=any_spec,
        scratch_shapes=scratch,
        compiler_params=pltpu.CompilerParams(vmem_limit_bytes=127 * 1024 * 1024),
    )(x, w1, w2, g, w_f, w_g, w_o)
```

```python
import functools
import math

import numpy as np

import jax
import jax.numpy as jnp
from jax import lax
import jax.experimental.pallas as pl
import jax.experimental.pallas.tpu as pltpu


class _Prog:
    def __init__(self):
        self.ops = []
        self.cse = {}

    def _node(self, kind, a, b):
        key = (kind, a, b)
        if key not in self.cse:
            self.ops.append(key)
            self.cse[key] = len(self.ops) - 1
        return self.cse[key]

    def inp(self, i):
        return (self._node("in", i, None), 1)

    def neg(self, x):
        return None if x is None else (x[0], -x[1])

    def add(self, x, y):
        if x is None:
            return y
        if y is None:
            return x
        (a, sa), (b, sb) = x, y
        if sa == sb:
            return (self._node("add", min(a, b), max(a, b)), sa)
        if sa > 0:
            return (self._node("sub", a, b), 1)
        return (self._node("sub", b, a), 1)

    def sub(self, x, y):
        return self.add(x, self.neg(y))

    def mul(self, c, x):
        if x is None or c == 0:
            return None
        if c == 1:
            return x
        if c == -1:
            return self.neg(x)
        return (self._node("mul", x[0], abs(float(c))), x[1] * (1 if c > 0 else -1))

    def cadd(self, z, w):
        return (self.add(z[0], w[0]), self.add(z[1], w[1]))

    def csub(self, z, w):
        return (self.sub(z[0], w[0]), self.sub(z[1], w[1]))

    def cconj(self, z):
        return (z[0], self.neg(z[1]))

    def twiddle(self, z, num, den):
        num %= den
        a, b = z
        if (8 * num) % den == 0:
            e = (8 * num) // den
            r = math.sqrt(0.5)
            if e == 0:
                return (a, b)
            if e == 2:
                return (b, self.neg(a))
            if e == 4:
                return (self.neg(a), self.neg(b))
            if e == 6:
                return (self.neg(b), a)
            if e == 1:
                return (self.mul(r, self.add(a, b)), self.mul(r, self.sub(b, a)))
            if e == 3:
                return (self.mul(r, self.sub(b, a)), self.mul(-r, self.add(a, b)))
            if e == 5:
                return (self.mul(-r, self.add(a, b)), self.mul(r, self.sub(a, b)))
            return (self.mul(r, self.sub(a, b)), self.mul(r, self.add(a, b)))
        th = -2.0 * math.pi * num / den
        c, s = math.cos(th), math.sin(th)
        return (self.sub(self.mul(c, a), self.mul(s, b)), self.add(self.mul(s, a), self.mul(c, b)))

    def rfft(self, xs):
        n = len(xs)
        if n == 1:
            return [(xs[0], None)]
        if n == 2:
            return [(self.add(xs[0], xs[1]), None), (self.sub(xs[0], xs[1]), None)]
        if n == 4:
            a = self.add(xs[0], xs[2])
            b = self.sub(xs[0], xs[2])
            c = self.add(xs[1], xs[3])
            d = self.sub(xs[1], xs[3])
            return [(self.add(a, c), None), (b, self.neg(d)), (self.sub(a, c), None)]
        u = self.rfft(xs[0::2])
        z1 = self.rfft(xs[1::4])
        z3 = self.rfft(xs[3::4])

        def get_u(k):
            k %= n // 2
            return u[k] if k <= n // 4 else self.cconj(u[n // 2 - k])

        out = [None] * (n // 2 + 1)
        for k in range(n // 8 + 1):
            t1 = self.twiddle(z1[k], k, n)
            t3 = self.twiddle(z3[k], 3 * k, n)
            sm = self.cadd(t1, t3)
            df = self.csub(t1, t3)
            u0, u1 = get_u(k), get_u(k + n // 4)
            out[k] = self.cadd(u0, sm)
            out[n // 2 - k] = self.cconj(self.csub(u0, sm))
            mdf = (df[1], self.neg(df[0]))
            out[k + n // 4] = self.cadd(u1, mdf)
            if k > 0:
                out[n // 4 - k] = self.cconj(self.csub(u1, mdf))
        return out

    def order(self, outs):
        seen, order = set(), []
        for o in outs:
            if o is None or o[0] in seen:
                continue
            stack = [(o[0], False)]
            while stack:
                n, done = stack.pop()
                if done:
                    order.append(n)
                    continue
                if n in seen:
                    continue
                seen.add(n)
                stack.append((n, True))
                kind, a, b = self.ops[n]
                if kind in ("add", "sub"):
                    stack.append((b, False))
                    stack.append((a, False))
                elif kind == "mul":
                    stack.append((a, False))
        return order

    def transpose(self, outs):
        g = _Prog()
        adj = {}

        def acc(n, v):
            if v is not None:
                adj[n] = g.add(adj.get(n), v)

        for i, o in enumerate(outs):
            if o is not None:
                acc(o[0], g.mul(o[1], g.inp(i)))
        res = {}
        for n in sorted(set(self.order(outs)), reverse=True):
            kind, a, b = self.ops[n]
            v = adj.get(n)
            if v is None:
                continue
            if kind == "in":
                res[a] = v
            elif kind == "add":
                acc(a, v)
                acc(b, v)
            elif kind == "sub":
                acc(a, v)
                acc(b, g.neg(v))
            else:
                acc(a, g.mul(b, v))
        return g, res

    def run(self, outs, load, emit, keep_sign=True):
        val = {}
        want = {}
        for i, o in enumerate(outs):
            if o is not None:
                want.setdefault(o[0], []).append((i, o[1]))
        for n in self.order(outs):
            kind, a, b = self.ops[n]
            if kind == "in":
                v = load(a)
            elif kind == "add":
                v = val[a] + val[b]
            elif kind == "sub":
                v = val[a] - val[b]
            else:
                v = val[a] * np.float32(b)
            val[n] = v
            for i, sg in want.get(n, ()):
                emit(i, -v if (sg < 0 and keep_sign) else v)


def _lhs_outputs(p, spec, n):
    outs = [spec[0][0], spec[n // 2][0]]
    for k in range(1, n // 2):
        a, b = spec[k]
        outs += [p.add(a, b), a, b]
    return outs


class _Plan:
    def __init__(self, n):
        self.n = n
        self.taps = 16
        self.hop = n - self.taps + 1
        self.ns = 2 + 3 * (n // 2 - 1)
        self.fwd = _Prog()
        spec = self.fwd.rfft([self.fwd.inp(i) for i in range(n)])
        self.fwd_outs = _lhs_outputs(self.fwd, spec, n)
        lhs_sign = [o[1] for o in self.fwd_outs]
        p = _Prog()
        spec = p.rfft([p.inp(i) if i < self.hop else None for i in range(n)])
        self.inv, res = p.transpose(_lhs_outputs(p, spec, n))
        self.inv_outs = [res[t] for t in range(self.hop)]
        self.inv_src = [0, 1]
        for k in range(n // 2 - 1):
            base = 2 + 3 * k
            self.inv_src += [base, base + 2, base + 1]
        self.wprog, self.wouts, self.wtap = [], [], []
        for ph in range(2):
            p = _Prog()
            xs = [None] * n
            for j in range(self.taps):
                if not (ph == 0 and j == 0):
                    xs[j] = p.inp(2 * j - 1 if ph == 0 else 2 * j)
            spec = p.rfft(xs)
            outs = [p.mul(0.5, spec[0][0]), p.mul(0.5, spec[n // 2][0])]
            for k in range(1, n // 2):
                c, dm = spec[k]
                d = p.neg(dm)
                outs += [c, p.sub(d, c), p.neg(p.add(c, d))]
            outs = [(o[0], o[1] * s) for o, s in zip(outs, lhs_sign)]
            self.wprog.append(p)
            self.wouts.append(outs)


_FFT_N = 32
_PLAN = _Plan(_FFT_N)

_C0 = math.sqrt(2.0 / math.pi)
_KAPPA = 0.044715 / (_C0 * _C0)


def _gelu2(z):
    inner = z * (np.float32(_KAPPA) * (z * z) + np.float32(1.0))
    return z + z * jnp.tanh(inner)


_B, _T, _D, _K, _U = 2, 16000, 256, 31, 8
_T1, _T2 = _T // 2, _T // 4
_S2 = 502
_S1 = 2 * _S2
_HOP = _PLAN.hop
_NS = _PLAN.ns
_CB = 8
_C1 = [5] + [_CB] * 7
_CB2, _NSTEP2 = 5, 6
_NB1 = sum(_C1)
_XOFF = 24
_XROWS = -(-(7 * _S1 + _HOP * (_NB1 - 1) + _FFT_N) // 8) * 8
_HROWS = 2 * _HOP * (_CB2 * _NSTEP2 - 1) + 2 * _FFT_N
_FROWS = _HOP * _CB2 * _NSTEP2
_TJ = _HOP
_XPARTS = 8
_OSLOTS = 4
_WPARTS = 4
_NDEP = 2
_COST = {"fx": 262, "fh": 230, "inv": 350, "w": 280}


def _x_piece_bounds():
    edges = []
    for s in range(8):
        for p in range(_XPARTS):
            edges.append(min(max((s * _S1 + p * (_S1 // _XPARTS) - _XOFF) // 8 * 8, 0), _T1))
    edges.append(_T1)
    return edges


def _merge(*lists):
    lists = [l for l in lists if l]
    pos = [0] * len(lists)
    out = []
    for _ in range(sum(len(l) for l in lists)):
        j = min((q for q in range(len(lists)) if pos[q] < len(lists[q])),
                key=lambda q: (pos[q] + 0.5) / len(lists[q]))
        out.append(lists[j][pos[j]])
        pos[j] += 1
    return out


def _dyn8(v):
    return v if isinstance(v, int) else pl.multiple_of(v, 8)


def _emit_step(items, units, mask):
    starts = np.cumsum([0] + [2 * (rows // 8) for rows, _, _ in items])
    nev = int(starts[-1])
    tot = sum(c for c, _ in units) or 1
    margin = min(40, nev // 8)
    sched, cum = [], 0
    for cost, fn in units:
        evs = [min(int((cum + cost * q / _NDEP) / tot * (nev - margin)) + 1, nev - 1)
               for q in range(_NDEP)]
        cum += cost
        sched.append((fn, evs))
    results = {}

    def event(e):
        j = int(np.searchsorted(starts, e, side="right")) - 1
        rg, nn = divmod(e - int(starts[j]), 2)
        return results[j][rg * 8:(rg + 1) * 8, nn * 128:(nn + 1) * 128]

    pi = 0
    for j, (rows, dot_fn, post_fn) in enumerate(items):
        results[j] = dot_fn()
        while pi < len(sched) and max(sched[pi][1]) < starts[j + 1]:
            fn, evs = sched[pi]
            pi += 1
            fn([functools.partial(event, e) for e in evs])
        post_fn(results[j])
    assert pi == len(sched)


def _pick(cnt, total, deps):
    if not deps:
        return None
    j, rem = divmod(cnt * len(deps), total)
    return j if rem < len(deps) else None


def _kernel(x_hbm, w1_hbm, w2_hbm, g_hbm, wf_hbm, wg_hbm, wo_hbm, out_hbm,
            v1, v2, spec_a, spec_b, y_a, y_b, hbuf, xbuf, w1buf, w2buf,
            gbuf, wfbuf, wgbuf, wobuf, gebuf, fbuf, febuf, obuf,
            sem_w, sem_s, sem_x, sem_o):
    plan = _PLAN
    n, hop, ns = plan.n, plan.hop, plan.ns
    specs, ys = (spec_a, spec_b), (y_a, y_b)

    xu = x_hbm.bitcast(jnp.uint32)
    edges = _x_piece_bounds()

    def x_copies(part):
        cps = []
        for s in range(8):
            r0, r1 = edges[s * _XPARTS + part], edges[s * _XPARTS + part + 1]
            for cs in range(2):
                cps.append(pltpu.make_async_copy(
                    xu.at[:, pl.ds(r0, r1 - r0), pl.ds(cs * 128, 128)],
                    xbuf.at[:, cs, pl.ds(_XOFF + r0, r1 - r0), :],
                    sem_x.at[part]))
        return cps

    wrows = _D // _WPARTS
    w1_copies = [pltpu.make_async_copy(w1_hbm.at[:, pl.ds(p * wrows, wrows), :],
                                       w1buf.at[:, pl.ds(p * wrows, wrows), :], sem_w.at[p])
                 for p in range(_WPARTS)]
    cp_w2 = pltpu.make_async_copy(w2_hbm, w2buf, sem_w.at[_WPARTS])
    small = [pltpu.make_async_copy(src, dst, sem_s.at[i]) for i, (src, dst) in
             enumerate([(g_hbm, gbuf), (wf_hbm, wfbuf), (wg_hbm, wgbuf), (wo_hbm, wobuf)])]

    for c in w1_copies:
        c.start()
    zero8 = jnp.zeros((8, 128), jnp.uint32)
    for bb in range(2):
        for cs in range(2):
            for r in range(0, _XOFF, 8):
                xbuf[bb, cs, pl.ds(r, 8), :] = zero8
            for r in range(_XOFF + _T1, _XROWS, 8):
                xbuf[bb, cs, pl.ds(r, 8), :] = zero8
    zrow = jnp.zeros((8, 128), jnp.float32)
    for bb in range(2):
        for cs in range(2):
            for r in range(_NB1 * hop, _HROWS):
                hbuf[bb, cs, r] = zrow

    def w_unit(wbuf, vbuf, scale, row, half, ph, nt, deps=(), mask=None):
        cnt = [0]

        def load(tap):
            w = wbuf[tap, pl.ds(_dyn8(row + 8 * half), 8), pl.ds(nt * 128, 128)].astype(jnp.float32)
            j = _pick(cnt[0], 16, deps)
            cnt[0] += 1
            if j is not None:
                w = jnp.where(mask, w, deps[j]())
            return w * np.float32(scale)

        def emit(i, v):
            vbuf[i, 2 * ph + row // 128, nt, pl.ds(_dyn8((row % 128) // 2) + 4 * half, 4), :] = (
                pltpu.bitcast(v.astype(jnp.bfloat16), jnp.uint32))
        plan.wprog[ph].run(plan.wouts[ph], load, emit)

    def fwd_unit(load_in, spec, row, col, deps, mask):
        cnt = [0]

        def load(q):
            j = _pick(cnt[0], n, deps)
            cnt[0] += 1
            return load_in(q, None if j is None else deps[j], mask)

        def emit(i, v):
            spec[col // 128, i, pl.ds(row, 8), :] = v
        plan.fwd.run(plan.fwd_outs, load, emit, keep_sign=False)

    def fx_unit(spec, blk, be, bb, cs, ph, zd, deps=(), mask=None):
        base = blk * hop
        if ph == 1:
            base = base + zd

        def load_in(q, dep, mask):
            v = xbuf[bb, cs, pl.ds(base + q, 8, stride=_S1), :]
            if dep is not None:
                v = jnp.where(mask, v, lax.bitcast_convert_type(dep(), jnp.uint32))
            v = (v << 16) if ph == 0 else (v & jnp.uint32(0xFFFF0000))
            return lax.bitcast_convert_type(v, jnp.float32)
        fwd_unit(load_in, spec, _dyn8(be * 16 + bb * 8), ph * 256 + cs * 128, deps, mask)

    def fh_unit(spec, blk, be, bb, cs, ph, deps=(), mask=None):
        base = blk * 2 * hop + ph

        def load_in(q, dep, mask):
            v = hbuf[bb, cs, base + 2 * q]
            if dep is not None:
                v = jnp.where(mask, v, dep())
            return v
        fwd_unit(load_in, spec, _dyn8(be * 16 + bb * 8), ph * 256 + cs * 128, deps, mask)

    def inv_unit(ybuf, dst, scale, blk, be, bb, nt, deps=(), mask=None):
        cnt = [0]
        row = _dyn8(be * 16 + bb * 8)

        def load(i):
            v = ybuf[nt, plan.inv_src[i], pl.ds(row, 8), :]
            j = _pick(cnt[0], ns, deps)
            cnt[0] += 1
            if j is not None:
                v = jnp.where(mask, v, deps[j]())
            return v

        def store(t, z):
            hval = _gelu2(z)
            if scale != 1.0:
                hval = hval * np.float32(scale)
            dst[bb, nt, blk * hop + t] = hval
        plan.inv.run(plan.inv_outs, load, store)

    def fx_units(spec, blk0, nblk, zd, mask):
        return [(_COST["fx"], functools.partial(fx_unit, spec, blk0 + be, be, bb, cs, ph, zd, mask=mask))
                for be in range(nblk) for bb in range(2) for cs in range(2) for ph in range(2)]

    def fh_units(spec, blk0, nblk, mask):
        return [(_COST["fh"], functools.partial(fh_unit, spec, blk0 + be, be, bb, cs, ph, mask=mask))
                for be in range(nblk) for bb in range(2) for cs in range(2) for ph in range(2)]

    def inv_units(ybuf, dst, scale, blk0, nblk, mask):
        return [(_COST["inv"], functools.partial(inv_unit, ybuf, dst, scale, blk0 + be, be, bb, nt, mask=mask))
                for be in range(nblk) for bb in range(2) for nt in range(2)]

    def w2_units(rg0, nrg, mask):
        return [(_COST["w"], functools.partial(
                    w_unit, w2buf, v2, (2.0 / n) * 0.5, pl.multiple_of((rg0 + r) * 16, 16)
                    if not isinstance(rg0, int) else (rg0 + r) * 16, half, ph, nt, mask=mask))
                for r in range(nrg) for half in range(2) for ph in range(2) for nt in range(2)]

    def conv_items(vbuf, spec, ybuf, m):
        items = []
        for i in range(ns):
            hold = []

            def dot_fn(i=i, h=0):
                w = jnp.concatenate(
                    [jnp.concatenate(
                        [pltpu.bitcast(vbuf[i, 2 * h + q, nt, pl.ds(0, 64), :], jnp.bfloat16)
                         for q in range(2)], axis=0) for nt in range(2)], axis=1)
                lhs = jnp.concatenate([spec[2 * h + q, i, pl.ds(0, m), :] for q in range(2)], axis=1)
                return jnp.dot(lhs, w, preferred_element_type=jnp.float32)

            def post0(r, hold=hold):
                hold.append(r)

            def post1(r, i=i, hold=hold):
                y = hold[0] + r
                for nt in range(2):
                    ybuf[nt, i, pl.ds(0, m), :] = y[:, nt * 128:(nt + 1) * 128]
            items.append((m, functools.partial(dot_fn, i, 0), post0))
            items.append((m, functools.partial(dot_fn, i, 1), post1))
        return items

    def block(fn, zd):
        def body(_, c):
            fn()
            return c
        lax.fori_loop(0, 1 + zd, body, 0)

    def opaque_zero(i):
        return (i * (i + 1)) & 1

    def true_mask(zd):
        return jnp.full((8, 128), zd, jnp.int32) == 0

    c1_start = [int(v) for v in np.cumsum([0] + _C1)]

    def v1_body(rg, carry):
        for p in range(_WPARTS):
            @pl.when(rg == p * (wrows // 16))
            def _():
                w1_copies[p].wait()
                if p == 0:
                    for c in x_copies(0):
                        c.start()
                if p == 2:
                    for c in x_copies(1):
                        c.start()
        row = pl.multiple_of(rg * 16, 16)
        for half in range(2):
            for ph in range(2):
                for nt in range(2):
                    w_unit(w1buf, v1, (2.0 / n) * _C0, row, half, ph, nt)
        return carry
    with jax.named_scope("v1"):
        lax.fori_loop(0, _D // 16, v1_body, 0)

    zd0 = opaque_zero(xbuf[0, 0, 0, 0].astype(jnp.int32))
    mask0 = true_mask(zd0)

    need = {0: [1], 1: [2], 2: [3, 4], 3: [5], 4: [6], 5: [7], 6: []}

    def start_parts(c):
        for p in need.get(c, []):
            for cp in x_copies(p):
                cp.start()

    def wait_parts(c):
        for p in need.get(c, []):
            for cp in x_copies(p):
                cp.wait()

    with jax.named_scope("x0wait"):
        for c in x_copies(0):
            c.wait()

    def fill_body(u, carry):
        zd = opaque_zero(u)
        for cs in range(2):
            for ph in range(2):
                fx_unit(spec_a, u // 2, u // 2, u % 2, cs, ph, zd)
        return carry
    with jax.named_scope("fill"):
        lax.fori_loop(0, _C1[0] * 2, fill_body, 0)

    with jax.named_scope("x1wait"):
        wait_parts(0)
    cp_w2.start()
    start_parts(1)

    def step0_body():
        zd, mask = zd0, mask0
        _emit_step(conv_items(v1, spec_a, y_a, _C1[0] * 16),
                   fx_units(spec_b, c1_start[1], _CB, zd, mask), mask)
    with jax.named_scope("step0"):
        block(step0_body, zd0)

    def conv1_body(it, carry):
        zd = opaque_zero(it)
        mask = true_mask(zd)
        for par in (1, 0):
            c = 2 * it + (1 if par == 1 else 2)
            blk_c = _C1[0] + (c - 1) * _CB
            for k in range(3):
                @pl.when(it == k)
                def _():
                    ck = 2 * k + (1 if par == 1 else 2)
                    wait_parts(ck)
                    start_parts(ck + 1)
                    if ck == 1:
                        cp_w2.wait()
                    if ck == 5:
                        for cp in small:
                            cp.start()
            block(lambda: _emit_step(
                conv_items(v1, specs[par], ys[par], _CB * 16),
                _merge(fx_units(specs[1 - par], blk_c + _CB, _CB, zd, mask) +
                       inv_units(ys[1 - par], hbuf, 1.0,
                                 jnp.maximum(blk_c - _CB, 0), _CB, mask),
                       w2_units(2 * c - 2, 2, mask)), mask), zd)
        return carry
    with jax.named_scope("conv1"):
        lax.fori_loop(0, 3, conv1_body, 0)

    sub = lax.broadcasted_iota(jnp.int32, (8, 128), 0)

    def mask_rows(r0, r1, s):
        def body(r, carry):
            for bb in range(2):
                for cs in range(2):
                    hbuf[bb, cs, r] = jnp.where(sub == s, 0.0, hbuf[bb, cs, r])
            return carry
        lax.fori_loop(r0, r1, body, 0)
    mask_rows(0, 16, 0)

    def step7_body():
        zd, mask = zd0, mask0
        _emit_step(conv_items(v1, spec_b, y_b, _CB * 16),
                   _merge(fh_units(spec_a, 0, _CB2, mask),
                          inv_units(y_a, hbuf, 1.0, c1_start[6], _CB, mask),
                          w2_units(12, 4, mask)), mask)
    with jax.named_scope("step7"):
        block(step7_body, zd0)

    fscale = 0.5 / _C0

    def step8_body():
        zd, mask = zd0, mask0
        _emit_step(conv_items(v2, spec_a, y_a, _CB2 * 16),
                   _merge(fh_units(spec_b, _CB2, _CB2, mask),
                          inv_units(y_b, hbuf, 1.0, c1_start[7], _CB, mask)), mask)
    with jax.named_scope("step8"):
        block(step8_body, zd0)
    mask_rows(_T1 - 7 * _S1 + 16, _NB1 * hop, 7)

    def conv2_body(it, carry):
        zd = opaque_zero(it)
        mask = true_mask(zd)
        for par in (1, 0):
            c = 2 * it + (1 if par == 1 else 2)
            block(lambda: _emit_step(
                conv_items(v2, specs[par], ys[par], _CB2 * 16),
                (fh_units(specs[1 - par], (c + 1) * _CB2, _CB2, mask) +
                 inv_units(ys[1 - par], fbuf, fscale, (c - 1) * _CB2, _CB2, mask)),
                mask), zd)
        return carry
    with jax.named_scope("conv2"):
        lax.fori_loop(0, 2, conv2_body, 0)

    for c in small:
        c.wait()
    gebuf[...] = jnp.dot(gbuf[...].reshape(_B * _U, _D), wgbuf[...],
                         preferred_element_type=jnp.float32).reshape(_B, _U, _D)

    def fe_item(slot, tile):
        def dot_fn():
            f = jnp.concatenate(
                [jnp.concatenate(
                    [fbuf[bb, cs, pl.ds(tile * _TJ, _TJ)].reshape(_TJ * 8, 128) for cs in range(2)],
                    axis=1) for bb in range(2)], axis=0)
            return jnp.dot(f, wfbuf[...], preferred_element_type=jnp.float32)

        def post(r):
            febuf[slot] = r.reshape(_B, _TJ, 8, _D)
        return (_TJ * 16, dot_fn, post)

    def step13_body():
        zd, mask = zd0, mask0
        _emit_step(conv_items(v2, spec_b, y_b, _CB2 * 16) + [fe_item(0, 0)],
                   inv_units(y_a, fbuf, fscale, 4 * _CB2, _CB2, mask), mask)
    with jax.named_scope("step13"):
        block(step13_body, zd0)

    def out_copies(slot, t0, rows_of):
        cps = []
        for s in range(8):
            rows = rows_of(s)
            if rows > 0:
                cps.append(pltpu.make_async_copy(
                    obuf.at[slot, :, s, pl.ds(0, rows)],
                    out_hbm.at[:, pl.ds(s * _S2 + t0, rows)],
                    sem_o.at[slot]))
        return cps

    def joint_item(fslot, oslot, tj):
        def dot_fn():
            rows = []
            for tt in range(tj):
                for r in range(16):
                    fr = febuf[fslot, r // 8, tt, pl.ds(r % 8, 1), :]
                    rows.append(jnp.tanh(jnp.broadcast_to(fr, (_U, _D)) + gebuf[r // 8]))
            return jnp.dot(jnp.concatenate(rows, axis=0), wobuf[...],
                           preferred_element_type=jnp.float32)

        def post(o):
            o = o.reshape(tj, _B, 8, _U, _D).astype(jnp.bfloat16)
            for tt in range(tj):
                obuf[oslot, :, :, tt] = o[tt]
        return (tj * 16 * _U, dot_fn, post)

    full = lambda s: _TJ
    ntiles = -(-_S2 // _TJ)
    nfull = (_T2 - 7 * _S2) // _TJ
    assert nfull % _OSLOTS == 0 and _OSLOTS == 4

    def first_body():
        _emit_step([fe_item(1, 1), joint_item(0, 0, _TJ), fe_item(0, 2), joint_item(1, 1, _TJ)],
                   inv_units(y_b, fbuf, fscale, 5 * _CB2, _CB2, mask0), mask0)
        for slot in range(2):
            for c in out_copies(slot, slot * _TJ, full):
                c.start()
    with jax.named_scope("first"):
        block(first_body, zd0)

    def joint_body(i2, carry):
        @pl.when(i2 >= 2)
        def _():
            for j in range(2):
                for c in out_copies((i2 % 2) * 2 + j, (2 * i2 + j - _OSLOTS) * _TJ, full):
                    c.wait()
        for j in range(2):
            tile = 2 * i2 + j
            oslot = (i2 % 2) * 2 + j
            _emit_step([fe_item(1 - j, tile + 1), joint_item(j, oslot, _TJ)], [], None)
            for c in out_copies(oslot, tile * _TJ, full):
                c.start()
        return carry
    with jax.named_scope("joint"):
        lax.fori_loop(1, nfull // 2, joint_body, 0)

    pending = {k: out_copies(k, (nfull - _OSLOTS + k) * _TJ, full) for k in range(_OSLOTS)}
    for tile in range(nfull, ntiles):
        oslot, t0 = tile % _OSLOTS, tile * _TJ
        tj = min(_TJ, _S2 - t0)
        rows_of = lambda s, t0=t0, tj=tj: max(0, min(tj, (_T2 - 7 * _S2 if s == 7 else _S2) - t0))
        for c in pending[oslot]:
            c.wait()
        items = ([fe_item(1 - tile % 2, tile + 1)] if tile + 1 < ntiles else []) + [
            joint_item(tile % 2, oslot, tj)]
        _emit_step(items, [], None)
        pending[oslot] = out_copies(oslot, t0, rows_of)
        for c in pending[oslot]:
            c.start()
    for k in range(_OSLOTS):
        for c in pending[k]:
            c.wait()


@jax.jit
def pallas_standalone__seq2seq_rnn_t_joint__speech_kernel(
    x: jax.Array,
    w1: jax.Array,
    w2: jax.Array,
    g: jax.Array,
    w_f: jax.Array,
    w_g: jax.Array,
    w_o: jax.Array,
):
    assert x.shape == (_B, _T, _D) and w1.shape == (_K, _D, _D) and w2.shape == (_K, _D, _D)
    assert g.shape == (_B, _U, _D)
    bf, f32 = jnp.bfloat16, jnp.float32
    m = _CB * 16
    scratch = [
        pltpu.VMEM((_NS, 4, 2, 72, 128), jnp.uint32),
        pltpu.VMEM((_NS, 4, 2, 72, 128), jnp.uint32),
        pltpu.VMEM((4, _NS, m + 8, 128), f32),
        pltpu.VMEM((4, _NS, m + 8, 128), f32),
        pltpu.VMEM((2, _NS, m + 8, 128), f32),
        pltpu.VMEM((2, _NS, m + 8, 128), f32),
        pltpu.VMEM((2, 2, _HROWS + 1, 8, 128), f32),
        pltpu.VMEM((2, 2, _XROWS, 128), jnp.uint32),
        pltpu.VMEM((_K, _D, _D), bf),
        pltpu.VMEM((_K, _D, _D), bf),
        pltpu.VMEM((_B, _U, _D), bf),
        pltpu.VMEM((_D, _D), bf),
        pltpu.VMEM((_D, _D), bf),
        pltpu.VMEM((_D, _D), bf),
        pltpu.VMEM((_B, _U, _D), f32),
        pltpu.VMEM((2, 2, _FROWS + 1, 8, 128), f32),
        pltpu.VMEM((2, _B, _TJ, 8, _D), f32),
        pltpu.VMEM((_OSLOTS, _B, 8, _TJ, _U, _D), bf),
        pltpu.SemaphoreType.DMA((_WPARTS + 1,)),
        pltpu.SemaphoreType.DMA((4,)),
        pltpu.SemaphoreType.DMA((_XPARTS,)),
        pltpu.SemaphoreType.DMA((_OSLOTS,)),
    ]
    any_spec = pl.BlockSpec(memory_space=pl.ANY)
    return pl.pallas_call(
        _kernel,
        out_shape=jax.ShapeDtypeStruct((_B, _T2, _U, _D), bf),
        in_specs=[any_spec] * 7,
        out_specs=any_spec,
        scratch_shapes=scratch,
        compiler_params=pltpu.CompilerParams(vmem_limit_bytes=127 * 1024 * 1024),
    )(x, w1, w2, g, w_f, w_g, w_o)
```

```python
import functools
import math

import numpy as np

import jax
import jax.numpy as jnp
from jax import lax
import jax.experimental.pallas as pl
import jax.experimental.pallas.tpu as pltpu


class _Prog:
    def __init__(self):
        self.ops = []
        self.cse = {}

    def _node(self, kind, a, b):
        key = (kind, a, b)
        if key not in self.cse:
            self.ops.append(key)
            self.cse[key] = len(self.ops) - 1
        return self.cse[key]

    def inp(self, i):
        return (self._node("in", i, None), 1)

    def neg(self, x):
        return None if x is None else (x[0], -x[1])

    def add(self, x, y):
        if x is None:
            return y
        if y is None:
            return x
        (a, sa), (b, sb) = x, y
        if sa == sb:
            return (self._node("add", min(a, b), max(a, b)), sa)
        if sa > 0:
            return (self._node("sub", a, b), 1)
        return (self._node("sub", b, a), 1)

    def sub(self, x, y):
        return self.add(x, self.neg(y))

    def mul(self, c, x):
        if x is None or c == 0:
            return None
        if c == 1:
            return x
        if c == -1:
            return self.neg(x)
        return (self._node("mul", x[0], abs(float(c))), x[1] * (1 if c > 0 else -1))

    def cadd(self, z, w):
        return (self.add(z[0], w[0]), self.add(z[1], w[1]))

    def csub(self, z, w):
        return (self.sub(z[0], w[0]), self.sub(z[1], w[1]))

    def cconj(self, z):
        return (z[0], self.neg(z[1]))

    def twiddle(self, z, num, den):
        num %= den
        a, b = z
        if (8 * num) % den == 0:
            e = (8 * num) // den
            r = math.sqrt(0.5)
            if e == 0:
                return (a, b)
            if e == 2:
                return (b, self.neg(a))
            if e == 4:
                return (self.neg(a), self.neg(b))
            if e == 6:
                return (self.neg(b), a)
            if e == 1:
                return (self.mul(r, self.add(a, b)), self.mul(r, self.sub(b, a)))
            if e == 3:
                return (self.mul(r, self.sub(b, a)), self.mul(-r, self.add(a, b)))
            if e == 5:
                return (self.mul(-r, self.add(a, b)), self.mul(r, self.sub(a, b)))
            return (self.mul(r, self.sub(a, b)), self.mul(r, self.add(a, b)))
        th = -2.0 * math.pi * num / den
        c, s = math.cos(th), math.sin(th)
        return (self.sub(self.mul(c, a), self.mul(s, b)), self.add(self.mul(s, a), self.mul(c, b)))

    def rfft(self, xs):
        n = len(xs)
        if n == 1:
            return [(xs[0], None)]
        if n == 2:
            return [(self.add(xs[0], xs[1]), None), (self.sub(xs[0], xs[1]), None)]
        if n == 4:
            a = self.add(xs[0], xs[2])
            b = self.sub(xs[0], xs[2])
            c = self.add(xs[1], xs[3])
            d = self.sub(xs[1], xs[3])
            return [(self.add(a, c), None), (b, self.neg(d)), (self.sub(a, c), None)]
        u = self.rfft(xs[0::2])
        z1 = self.rfft(xs[1::4])
        z3 = self.rfft(xs[3::4])

        def get_u(k):
            k %= n // 2
            return u[k] if k <= n // 4 else self.cconj(u[n // 2 - k])

        out = [None] * (n // 2 + 1)
        for k in range(n // 8 + 1):
            t1 = self.twiddle(z1[k], k, n)
            t3 = self.twiddle(z3[k], 3 * k, n)
            sm = self.cadd(t1, t3)
            df = self.csub(t1, t3)
            u0, u1 = get_u(k), get_u(k + n // 4)
            out[k] = self.cadd(u0, sm)
            out[n // 2 - k] = self.cconj(self.csub(u0, sm))
            mdf = (df[1], self.neg(df[0]))
            out[k + n // 4] = self.cadd(u1, mdf)
            if k > 0:
                out[n // 4 - k] = self.cconj(self.csub(u1, mdf))
        return out

    def order(self, outs):
        seen, order = set(), []
        for o in outs:
            if o is None or o[0] in seen:
                continue
            stack = [(o[0], False)]
            while stack:
                n, done = stack.pop()
                if done:
                    order.append(n)
                    continue
                if n in seen:
                    continue
                seen.add(n)
                stack.append((n, True))
                kind, a, b = self.ops[n]
                if kind in ("add", "sub"):
                    stack.append((b, False))
                    stack.append((a, False))
                elif kind == "mul":
                    stack.append((a, False))
        return order

    def transpose(self, outs):
        g = _Prog()
        adj = {}

        def acc(n, v):
            if v is not None:
                adj[n] = g.add(adj.get(n), v)

        for i, o in enumerate(outs):
            if o is not None:
                acc(o[0], g.mul(o[1], g.inp(i)))
        res = {}
        for n in sorted(set(self.order(outs)), reverse=True):
            kind, a, b = self.ops[n]
            v = adj.get(n)
            if v is None:
                continue
            if kind == "in":
                res[a] = v
            elif kind == "add":
                acc(a, v)
                acc(b, v)
            elif kind == "sub":
                acc(a, v)
                acc(b, g.neg(v))
            else:
                acc(a, g.mul(b, v))
        return g, res

    def run(self, outs, load, emit, keep_sign=True):
        val = {}
        want = {}
        for i, o in enumerate(outs):
            if o is not None:
                want.setdefault(o[0], []).append((i, o[1]))
        for n in self.order(outs):
            kind, a, b = self.ops[n]
            if kind == "in":
                v = load(a)
            elif kind == "add":
                v = val[a] + val[b]
            elif kind == "sub":
                v = val[a] - val[b]
            else:
                v = val[a] * np.float32(b)
            val[n] = v
            for i, sg in want.get(n, ()):
                emit(i, -v if (sg < 0 and keep_sign) else v)


def _lhs_outputs(p, spec, n):
    outs = [spec[0][0], spec[n // 2][0]]
    for k in range(1, n // 2):
        a, b = spec[k]
        outs += [p.add(a, b), a, b]
    return outs


class _Plan:
    def __init__(self, n):
        self.n = n
        self.taps = 16
        self.hop = n - self.taps + 1
        self.ns = 2 + 3 * (n // 2 - 1)
        self.fwd = _Prog()
        spec = self.fwd.rfft([self.fwd.inp(i) for i in range(n)])
        self.fwd_outs = _lhs_outputs(self.fwd, spec, n)
        lhs_sign = [o[1] for o in self.fwd_outs]
        p = _Prog()
        spec = p.rfft([p.inp(i) if i < self.hop else None for i in range(n)])
        self.inv, res = p.transpose(_lhs_outputs(p, spec, n))
        self.inv_outs = [res[t] for t in range(self.hop)]
        self.inv_src = [0, 1]
        for k in range(n // 2 - 1):
            base = 2 + 3 * k
            self.inv_src += [base, base + 2, base + 1]
        self.wprog, self.wouts, self.wtap = [], [], []
        for ph in range(2):
            p = _Prog()
            xs = [None] * n
            for j in range(self.taps):
                if not (ph == 0 and j == 0):
                    xs[j] = p.inp(2 * j - 1 if ph == 0 else 2 * j)
            spec = p.rfft(xs)
            outs = [p.mul(0.5, spec[0][0]), p.mul(0.5, spec[n // 2][0])]
            for k in range(1, n // 2):
                c, dm = spec[k]
                d = p.neg(dm)
                outs += [c, p.sub(d, c), p.neg(p.add(c, d))]
            outs = [(o[0], o[1] * s) for o, s in zip(outs, lhs_sign)]
            self.wprog.append(p)
            self.wouts.append(outs)


_FFT_N = 32
_PLAN = _Plan(_FFT_N)

_C0 = math.sqrt(2.0 / math.pi)
_KAPPA = 0.044715 / (_C0 * _C0)


def _gelu2(z):
    inner = z * (np.float32(_KAPPA) * (z * z) + np.float32(1.0))
    return z + z * jnp.tanh(inner)


_B, _T, _D, _K, _U = 2, 16000, 256, 31, 8
_T1, _T2 = _T // 2, _T // 4
_S2 = 502
_S1 = 2 * _S2
_HOP = _PLAN.hop
_NS = _PLAN.ns
_CB = 5
_C1 = [_CB] * 11 + [6]
_CB2, _NSTEP2 = 5, 6
_NB1 = sum(_C1)
_XOFF = 24
_XROWS = -(-(7 * _S1 + _HOP * (_NB1 - 1) + _FFT_N) // 8) * 8
_HROWS = 2 * _HOP * (_CB2 * _NSTEP2 - 1) + 2 * _FFT_N
_FROWS = _HOP * _CB2 * _NSTEP2
_TJ = _HOP
_XPARTS = 8
_OSLOTS = 4
_WPARTS = 4
_NDEP = 3
_COST = {"fx": 262, "fh": 230, "inv": 350, "w": 280}


def _x_piece_bounds():
    edges = []
    for s in range(8):
        for p in range(_XPARTS):
            edges.append(min(max((s * _S1 + p * (_S1 // _XPARTS) - _XOFF) // 8 * 8, 0), _T1))
    edges.append(_T1)
    return edges


def _merge(*lists):
    lists = [l for l in lists if l]
    pos = [0] * len(lists)
    out = []
    for _ in range(sum(len(l) for l in lists)):
        j = min((q for q in range(len(lists)) if pos[q] < len(lists[q])),
                key=lambda q: (pos[q] + 0.5) / len(lists[q]))
        out.append(lists[j][pos[j]])
        pos[j] += 1
    return out


def _dyn8(v):
    return v if isinstance(v, int) else pl.multiple_of(v, 8)


def _emit_step(items, units, mask):
    starts = np.cumsum([0] + [2 * (rows // 8) for rows, _, _ in items])
    nev = int(starts[-1])
    tot = sum(c for c, _ in units) or 1
    margin = min(40, nev // 8)
    sched, cum = [], 0
    for cost, fn in units:
        evs = [min(int((cum + cost * q / _NDEP) / tot * (nev - margin)) + 1, nev - 1)
               for q in range(_NDEP)]
        cum += cost
        sched.append((fn, evs))
    results = {}

    def event(e):
        j = int(np.searchsorted(starts, e, side="right")) - 1
        rg, nn = divmod(e - int(starts[j]), 2)
        return results[j][rg * 8:(rg + 1) * 8, nn * 128:(nn + 1) * 128]

    pi = 0
    for j, (rows, dot_fn, post_fn) in enumerate(items):
        results[j] = dot_fn()
        while pi < len(sched) and max(sched[pi][1]) < starts[j + 1]:
            fn, evs = sched[pi]
            pi += 1
            fn([functools.partial(event, e) for e in evs])
        post_fn(results[j])
    assert pi == len(sched)


def _pick(cnt, total, deps):
    if not deps:
        return None
    j, rem = divmod(cnt * len(deps), total)
    return j if rem < len(deps) else None


def _kernel(x_hbm, w1_hbm, w2_hbm, g_hbm, wf_hbm, wg_hbm, wo_hbm, out_hbm,
            v1, v2, spec_a, spec_b, y_a, y_b, hbuf, xbuf, w1buf, w2buf,
            gbuf, wfbuf, wgbuf, wobuf, gebuf, fbuf, febuf, obuf,
            sem_w, sem_s, sem_x, sem_o):
    plan = _PLAN
    n, hop, ns = plan.n, plan.hop, plan.ns
    specs, ys = (spec_a, spec_b), (y_a, y_b)

    xu = x_hbm.bitcast(jnp.uint32)
    edges = _x_piece_bounds()

    def x_copies(part):
        cps = []
        for s in range(8):
            r0, r1 = edges[s * _XPARTS + part], edges[s * _XPARTS + part + 1]
            for cs in range(2):
                cps.append(pltpu.make_async_copy(
                    xu.at[:, pl.ds(r0, r1 - r0), pl.ds(cs * 128, 128)],
                    xbuf.at[:, cs, pl.ds(_XOFF + r0, r1 - r0), :],
                    sem_x.at[part]))
        return cps

    wrows = _D // _WPARTS
    w1_copies = [pltpu.make_async_copy(w1_hbm.at[:, pl.ds(p * wrows, wrows), :],
                                       w1buf.at[:, pl.ds(p * wrows, wrows), :], sem_w.at[p])
                 for p in range(_WPARTS)]
    cp_w2 = pltpu.make_async_copy(w2_hbm, w2buf, sem_w.at[_WPARTS])
    small = [pltpu.make_async_copy(src, dst, sem_s.at[i]) for i, (src, dst) in
             enumerate([(g_hbm, gbuf), (wf_hbm, wfbuf), (wg_hbm, wgbuf), (wo_hbm, wobuf)])]

    for c in w1_copies:
        c.start()
    zero8 = jnp.zeros((8, 128), jnp.uint32)
    for bb in range(2):
        for cs in range(2):
            for r in range(0, _XOFF, 8):
                xbuf[bb, cs, pl.ds(r, 8), :] = zero8
            for r in range(_XOFF + _T1, _XROWS, 8):
                xbuf[bb, cs, pl.ds(r, 8), :] = zero8
    zrow = jnp.zeros((8, 128), jnp.float32)
    for bb in range(2):
        for cs in range(2):
            for r in range(_NB1 * hop, _HROWS):
                hbuf[bb, cs, r] = zrow

    def w_unit(wbuf, vbuf, scale, row, half, ph, nt, deps=(), mask=None):
        cnt = [0]

        def load(tap):
            w = wbuf[tap, pl.ds(_dyn8(row + 8 * half), 8), pl.ds(nt * 128, 128)].astype(jnp.float32)
            j = _pick(cnt[0], 16, deps)
            cnt[0] += 1
            if j is not None:
                w = jnp.where(mask, w, deps[j]())
            return w * np.float32(scale)

        def emit(i, v):
            vbuf[i, 2 * ph + row // 128, nt, pl.ds(_dyn8((row % 128) // 2) + 4 * half, 4), :] = (
                pltpu.bitcast(v.astype(jnp.bfloat16), jnp.uint32))
        plan.wprog[ph].run(plan.wouts[ph], load, emit)

    def fwd_unit(load_in, spec, row, col, deps, mask):
        cnt = [0]

        def load(q):
            j = _pick(cnt[0], n, deps)
            cnt[0] += 1
            return load_in(q, None if j is None else deps[j], mask)

        def emit(i, v):
            spec[col // 128, i, pl.ds(row, 8), :] = v
        plan.fwd.run(plan.fwd_outs, load, emit, keep_sign=False)

    def fx_unit(spec, blk, be, bb, cs, ph, zd, deps=(), mask=None):
        base = blk * hop
        if ph == 1:
            base = base + zd

        def load_in(q, dep, mask):
            v = xbuf[bb, cs, pl.ds(base + q, 8, stride=_S1), :]
            if dep is not None:
                v = jnp.where(mask, v, lax.bitcast_convert_type(dep(), jnp.uint32))
            v = (v << 16) if ph == 0 else (v & jnp.uint32(0xFFFF0000))
            return lax.bitcast_convert_type(v, jnp.float32)
        fwd_unit(load_in, spec, _dyn8(be * 16 + bb * 8), ph * 256 + cs * 128, deps, mask)

    def fh_unit(spec, blk, be, bb, cs, ph, deps=(), mask=None):
        base = blk * 2 * hop + ph

        def load_in(q, dep, mask):
            v = hbuf[bb, cs, base + 2 * q]
            if dep is not None:
                v = jnp.where(mask, v, dep())
            return v
        fwd_unit(load_in, spec, _dyn8(be * 16 + bb * 8), ph * 256 + cs * 128, deps, mask)

    def inv_unit(ybuf, dst, scale, blk, be, bb, nt, deps=(), mask=None):
        cnt = [0]
        row = _dyn8(be * 16 + bb * 8)

        def load(i):
            v = ybuf[nt, plan.inv_src[i], pl.ds(row, 8), :]
            j = _pick(cnt[0], ns, deps)
            cnt[0] += 1
            if j is not None:
                v = jnp.where(mask, v, deps[j]())
            return v

        def store(t, z):
            hval = _gelu2(z)
            if scale != 1.0:
                hval = hval * np.float32(scale)
            dst[bb, nt, blk * hop + t] = hval
        plan.inv.run(plan.inv_outs, load, store)

    def fx_units(spec, blk0, nblk, zd, mask):
        return [(_COST["fx"], functools.partial(fx_unit, spec, blk0 + be, be, bb, cs, ph, zd, mask=mask))
                for be in range(nblk) for bb in range(2) for cs in range(2) for ph in range(2)]

    def fh_units(spec, blk0, nblk, mask):
        return [(_COST["fh"], functools.partial(fh_unit, spec, blk0 + be, be, bb, cs, ph, mask=mask))
                for be in range(nblk) for bb in range(2) for cs in range(2) for ph in range(2)]

    def inv_units(ybuf, dst, scale, blk0, nblk, mask):
        return [(_COST["inv"], functools.partial(inv_unit, ybuf, dst, scale, blk0 + be, be, bb, nt, mask=mask))
                for be in range(nblk) for bb in range(2) for nt in range(2)]

    def w2_units(rg0, nrg, mask):
        return [(_COST["w"], functools.partial(
                    w_unit, w2buf, v2, (2.0 / n) * 0.5, pl.multiple_of((rg0 + r) * 16, 16)
                    if not isinstance(rg0, int) else (rg0 + r) * 16, half, ph, nt, mask=mask))
                for r in range(nrg) for half in range(2) for ph in range(2) for nt in range(2)]

    def conv_items(vbuf, spec, ybuf, m):
        items = []
        for i in range(ns):
            hold = []

            def dot_fn(i=i, h=0):
                w = jnp.concatenate(
                    [jnp.concatenate(
                        [pltpu.bitcast(vbuf[i, 2 * h + q, nt, pl.ds(0, 64), :], jnp.bfloat16)
                         for q in range(2)], axis=0) for nt in range(2)], axis=1)
                lhs = jnp.concatenate([spec[2 * h + q, i, pl.ds(0, m), :] for q in range(2)], axis=1)
                return jnp.dot(lhs, w, preferred_element_type=jnp.float32)

            def post0(r, hold=hold):
                hold.append(r)

            def post1(r, i=i, hold=hold):
                y = hold[0] + r
                for nt in range(2):
                    ybuf[nt, i, pl.ds(0, m), :] = y[:, nt * 128:(nt + 1) * 128]
            items.append((m, functools.partial(dot_fn, i, 0), post0))
            items.append((m, functools.partial(dot_fn, i, 1), post1))
        return items

    def block(fn, zd):
        def body(_, c):
            fn()
            return c
        lax.fori_loop(0, 1 + zd, body, 0)

    def opaque_zero(i):
        return (i * (i + 1)) & 1

    def true_mask(zd):
        return jnp.full((8, 128), zd, jnp.int32) == 0

    c1_start = [int(v) for v in np.cumsum([0] + _C1)]

    def v1_body(rg, carry):
        for p in range(_WPARTS):
            @pl.when(rg == p * (wrows // 16))
            def _():
                w1_copies[p].wait()
                if p == 0:
                    for c in x_copies(0):
                        c.start()
                if p == 2:
                    for c in x_copies(1):
                        c.start()
        row = pl.multiple_of(rg * 16, 16)
        for half in range(2):
            for ph in range(2):
                for nt in range(2):
                    w_unit(w1buf, v1, (2.0 / n) * _C0, row, half, ph, nt)
        return carry
    with jax.named_scope("v1"):
        lax.fori_loop(0, _D // 16, v1_body, 0)

    zd0 = opaque_zero(xbuf[0, 0, 0, 0].astype(jnp.int32))
    mask0 = true_mask(zd0)

    need, have = {}, 0
    for c in range(len(_C1) - 1):
        top = hop * (c1_start[c + 2] - 1) + n - _XOFF
        req = min(_XPARTS - 1, max(
            p for s8 in range(8) for p in range(_XPARTS)
            if edges[s8 * _XPARTS + p] < min(s8 * _S1 + top, _T1)))
        need[c] = list(range(have + 1, req + 1))
        have = max(have, req)
    assert have == _XPARTS - 1

    def start_parts(c):
        for p in need.get(c, []):
            for cp in x_copies(p):
                cp.start()

    def wait_parts(c):
        for p in need.get(c, []):
            for cp in x_copies(p):
                cp.wait()

    with jax.named_scope("x0wait"):
        for c in x_copies(0):
            c.wait()

    def fill_body(u, carry):
        zd = opaque_zero(u)
        for cs in range(2):
            for ph in range(2):
                fx_unit(spec_a, u // 2, u // 2, u % 2, cs, ph, zd)
        return carry
    with jax.named_scope("fill"):
        lax.fori_loop(0, _C1[0] * 2, fill_body, 0)

    with jax.named_scope("x1wait"):
        wait_parts(0)
    cp_w2.start()
    start_parts(1)

    def step0_body():
        _emit_step(conv_items(v1, spec_a, y_a, _CB * 16),
                   fx_units(spec_b, c1_start[1], _CB, zd0, mask0), mask0)
    with jax.named_scope("step0"):
        block(step0_body, zd0)

    def before_step(c):
        wait_parts(c)
        start_parts(c + 1)
        if c == 1:
            cp_w2.wait()
        if c == 8:
            for cp in small:
                cp.start()

    def conv1_body(it, carry):
        zd = opaque_zero(it)
        mask = true_mask(zd)
        for par in (1, 0):
            c = 2 * it + (1 if par == 1 else 2)
            for k in range(4):
                pl.when(it == k)(functools.partial(before_step, 2 * k + (1 if par == 1 else 2)))
            block(lambda: _emit_step(
                conv_items(v1, specs[par], ys[par], _CB * 16),
                _merge(fx_units(specs[1 - par], (c + 1) * _CB, _CB, zd, mask) +
                       inv_units(ys[1 - par], hbuf, 1.0, (c - 1) * _CB, _CB, mask),
                       w2_units(c - 1, 1, mask)), mask), zd)
        return carry
    with jax.named_scope("conv1"):
        lax.fori_loop(0, 4, conv1_body, 0)

    sub = lax.broadcasted_iota(jnp.int32, (8, 128), 0)

    def mask_rows(r0, r1, s):
        def body(r, carry):
            for bb in range(2):
                for cs in range(2):
                    hbuf[bb, cs, r] = jnp.where(sub == s, 0.0, hbuf[bb, cs, r])
            return carry
        lax.fori_loop(r0, r1, body, 0)
    mask_rows(0, 16, 0)

    for c in (9, 10):
        par = c % 2
        before_step(c)
        with jax.named_scope("step%d" % c):
            block(lambda: _emit_step(
                conv_items(v1, specs[par], ys[par], _CB * 16),
                _merge(fx_units(specs[1 - par], c1_start[c + 1], _C1[c + 1], zd0, mask0) +
                       inv_units(ys[1 - par], hbuf, 1.0, c1_start[c - 1], _CB, mask0),
                       w2_units(8 + 2 * (c - 9), 2, mask0)), mask0), zd0)

    def step11_body():
        _emit_step(conv_items(v1, spec_b, y_b, _C1[11] * 16),
                   _merge(fh_units(spec_a, 0, _CB2, mask0) +
                          inv_units(y_a, hbuf, 1.0, c1_start[10], _CB, mask0),
                          w2_units(12, 4, mask0)), mask0)
    with jax.named_scope("step11"):
        block(step11_body, zd0)

    fscale = 0.5 / _C0

    def step8_body():
        zd, mask = zd0, mask0
        _emit_step(conv_items(v2, spec_a, y_a, _CB2 * 16),
                   fh_units(spec_b, _CB2, _CB2, mask) +
                   inv_units(y_b, hbuf, 1.0, c1_start[11], _C1[11], mask), mask)
    with jax.named_scope("step8"):
        block(step8_body, zd0)
    mask_rows(_T1 - 7 * _S1 + 16, _NB1 * hop, 7)

    def conv2_body(it, carry):
        zd = opaque_zero(it)
        mask = true_mask(zd)
        for par in (1, 0):
            c = 2 * it + (1 if par == 1 else 2)
            block(lambda: _emit_step(
                conv_items(v2, specs[par], ys[par], _CB2 * 16),
                (fh_units(specs[1 - par], (c + 1) * _CB2, _CB2, mask) +
                 inv_units(ys[1 - par], fbuf, fscale, (c - 1) * _CB2, _CB2, mask)),
                mask), zd)
        return carry
    with jax.named_scope("conv2"):
        lax.fori_loop(0, 2, conv2_body, 0)

    for c in small:
        c.wait()
    gebuf[...] = jnp.dot(gbuf[...].reshape(_B * _U, _D), wgbuf[...],
                         preferred_element_type=jnp.float32).reshape(_B, _U, _D)

    def fe_item(slot, tile):
        def dot_fn():
            f = jnp.concatenate(
                [jnp.concatenate(
                    [fbuf[bb, cs, pl.ds(tile * _TJ, _TJ)].reshape(_TJ * 8, 128) for cs in range(2)],
                    axis=1) for bb in range(2)], axis=0)
            return jnp.dot(f, wfbuf[...], preferred_element_type=jnp.float32)

        def post(r):
            febuf[slot] = r.reshape(_B, _TJ, 8, _D)
        return (_TJ * 16, dot_fn, post)

    def step13_body():
        zd, mask = zd0, mask0
        _emit_step(conv_items(v2, spec_b, y_b, _CB2 * 16) + [fe_item(0, 0)],
                   inv_units(y_a, fbuf, fscale, 4 * _CB2, _CB2, mask), mask)
    with jax.named_scope("step13"):
        block(step13_body, zd0)

    def out_copies(slot, t0, rows_of):
        cps = []
        for s in range(8):
            rows = rows_of(s)
            if rows > 0:
                cps.append(pltpu.make_async_copy(
                    obuf.at[slot, :, s, pl.ds(0, rows)],
                    out_hbm.at[:, pl.ds(s * _S2 + t0, rows)],
                    sem_o.at[slot]))
        return cps

    def joint_item(fslot, oslot, tj):
        def dot_fn():
            rows = []
            for tt in range(tj):
                for r in range(16):
                    fr = febuf[fslot, r // 8, tt, pl.ds(r % 8, 1), :]
                    rows.append(jnp.tanh(jnp.broadcast_to(fr, (_U, _D)) + gebuf[r // 8]))
            return jnp.dot(jnp.concatenate(rows, axis=0), wobuf[...],
                           preferred_element_type=jnp.float32)

        def post(o):
            o = o.reshape(tj, _B, 8, _U, _D).astype(jnp.bfloat16)
            for tt in range(tj):
                obuf[oslot, :, :, tt] = o[tt]
        return (tj * 16 * _U, dot_fn, post)

    full = lambda s: _TJ
    ntiles = -(-_S2 // _TJ)
    nfull = (_T2 - 7 * _S2) // _TJ
    assert nfull % _OSLOTS == 0 and _OSLOTS == 4

    def first_body():
        _emit_step([fe_item(1, 1), joint_item(0, 0, _TJ), fe_item(0, 2), joint_item(1, 1, _TJ)],
                   inv_units(y_b, fbuf, fscale, 5 * _CB2, _CB2, mask0), mask0)
        for slot in range(2):
            for c in out_copies(slot, slot * _TJ, full):
                c.start()
    with jax.named_scope("first"):
        block(first_body, zd0)

    def joint_body(i2, carry):
        @pl.when(i2 >= 2)
        def _():
            for j in range(2):
                for c in out_copies((i2 % 2) * 2 + j, (2 * i2 + j - _OSLOTS) * _TJ, full):
                    c.wait()
        for j in range(2):
            tile = 2 * i2 + j
            oslot = (i2 % 2) * 2 + j
            _emit_step([fe_item(1 - j, tile + 1), joint_item(j, oslot, _TJ)], [], None)
            for c in out_copies(oslot, tile * _TJ, full):
                c.start()
        return carry
    with jax.named_scope("joint"):
        lax.fori_loop(1, nfull // 2, joint_body, 0)

    pending = {k: out_copies(k, (nfull - _OSLOTS + k) * _TJ, full) for k in range(_OSLOTS)}
    for tile in range(nfull, ntiles):
        oslot, t0 = tile % _OSLOTS, tile * _TJ
        tj = min(_TJ, _S2 - t0)
        rows_of = lambda s, t0=t0, tj=tj: max(0, min(tj, (_T2 - 7 * _S2 if s == 7 else _S2) - t0))
        for c in pending[oslot]:
            c.wait()
        items = ([fe_item(1 - tile % 2, tile + 1)] if tile + 1 < ntiles else []) + [
            joint_item(tile % 2, oslot, tj)]
        _emit_step(items, [], None)
        pending[oslot] = out_copies(oslot, t0, rows_of)
        for c in pending[oslot]:
            c.start()
    for k in range(_OSLOTS):
        for c in pending[k]:
            c.wait()


@jax.jit
def pallas_standalone__seq2seq_rnn_t_joint__speech_kernel(
    x: jax.Array,
    w1: jax.Array,
    w2: jax.Array,
    g: jax.Array,
    w_f: jax.Array,
    w_g: jax.Array,
    w_o: jax.Array,
):
    assert x.shape == (_B, _T, _D) and w1.shape == (_K, _D, _D) and w2.shape == (_K, _D, _D)
    assert g.shape == (_B, _U, _D)
    bf, f32 = jnp.bfloat16, jnp.float32
    m = max(_C1 + [_CB2]) * 16
    scratch = [
        pltpu.VMEM((_NS, 4, 2, 72, 128), jnp.uint32),
        pltpu.VMEM((_NS, 4, 2, 72, 128), jnp.uint32),
        pltpu.VMEM((4, _NS, m + 8, 128), f32),
        pltpu.VMEM((4, _NS, m + 8, 128), f32),
        pltpu.VMEM((2, _NS, m + 8, 128), f32),
        pltpu.VMEM((2, _NS, m + 8, 128), f32),
        pltpu.VMEM((2, 2, _HROWS + 1, 8, 128), f32),
        pltpu.VMEM((2, 2, _XROWS, 128), jnp.uint32),
        pltpu.VMEM((_K, _D, _D), bf),
        pltpu.VMEM((_K, _D, _D), bf),
        pltpu.VMEM((_B, _U, _D), bf),
        pltpu.VMEM((_D, _D), bf),
        pltpu.VMEM((_D, _D), bf),
        pltpu.VMEM((_D, _D), bf),
        pltpu.VMEM((_B, _U, _D), f32),
        pltpu.VMEM((2, 2, _FROWS + 1, 8, 128), f32),
        pltpu.VMEM((2, _B, _TJ, 8, _D), f32),
        pltpu.VMEM((_OSLOTS, _B, 8, _TJ, _U, _D), bf),
        pltpu.SemaphoreType.DMA((_WPARTS + 1,)),
        pltpu.SemaphoreType.DMA((4,)),
        pltpu.SemaphoreType.DMA((_XPARTS,)),
        pltpu.SemaphoreType.DMA((_OSLOTS,)),
    ]
    any_spec = pl.BlockSpec(memory_space=pl.ANY)
    return pl.pallas_call(
        _kernel,
        out_shape=jax.ShapeDtypeStruct((_B, _T2, _U, _D), bf),
        in_specs=[any_spec] * 7,
        out_specs=any_spec,
        scratch_shapes=scratch,
        compiler_params=pltpu.CompilerParams(vmem_limit_bytes=127 * 1024 * 1024),
    )(x, w1, w2, g, w_f, w_g, w_o)
```

```python
import functools
import math

import numpy as np

import jax
import jax.numpy as jnp
from jax import lax
import jax.experimental.pallas as pl
import jax.experimental.pallas.tpu as pltpu


class _Prog:
    def __init__(self):
        self.ops = []
        self.cse = {}

    def _node(self, kind, a, b):
        key = (kind, a, b)
        if key not in self.cse:
            self.ops.append(key)
            self.cse[key] = len(self.ops) - 1
        return self.cse[key]

    def inp(self, i):
        return (self._node("in", i, None), 1)

    def neg(self, x):
        return None if x is None else (x[0], -x[1])

    def add(self, x, y):
        if x is None:
            return y
        if y is None:
            return x
        (a, sa), (b, sb) = x, y
        if sa == sb:
            return (self._node("add", min(a, b), max(a, b)), sa)
        if sa > 0:
            return (self._node("sub", a, b), 1)
        return (self._node("sub", b, a), 1)

    def sub(self, x, y):
        return self.add(x, self.neg(y))

    def mul(self, c, x):
        if x is None or c == 0:
            return None
        if c == 1:
            return x
        if c == -1:
            return self.neg(x)
        return (self._node("mul", x[0], abs(float(c))), x[1] * (1 if c > 0 else -1))

    def cadd(self, z, w):
        return (self.add(z[0], w[0]), self.add(z[1], w[1]))

    def csub(self, z, w):
        return (self.sub(z[0], w[0]), self.sub(z[1], w[1]))

    def cconj(self, z):
        return (z[0], self.neg(z[1]))

    def twiddle(self, z, num, den):
        num %= den
        a, b = z
        if (8 * num) % den == 0:
            e = (8 * num) // den
            r = math.sqrt(0.5)
            if e == 0:
                return (a, b)
            if e == 2:
                return (b, self.neg(a))
            if e == 4:
                return (self.neg(a), self.neg(b))
            if e == 6:
                return (self.neg(b), a)
            if e == 1:
                return (self.mul(r, self.add(a, b)), self.mul(r, self.sub(b, a)))
            if e == 3:
                return (self.mul(r, self.sub(b, a)), self.mul(-r, self.add(a, b)))
            if e == 5:
                return (self.mul(-r, self.add(a, b)), self.mul(r, self.sub(a, b)))
            return (self.mul(r, self.sub(a, b)), self.mul(r, self.add(a, b)))
        th = -2.0 * math.pi * num / den
        c, s = math.cos(th), math.sin(th)
        return (self.sub(self.mul(c, a), self.mul(s, b)), self.add(self.mul(s, a), self.mul(c, b)))

    def rfft(self, xs):
        n = len(xs)
        if n == 1:
            return [(xs[0], None)]
        if n == 2:
            return [(self.add(xs[0], xs[1]), None), (self.sub(xs[0], xs[1]), None)]
        if n == 4:
            a = self.add(xs[0], xs[2])
            b = self.sub(xs[0], xs[2])
            c = self.add(xs[1], xs[3])
            d = self.sub(xs[1], xs[3])
            return [(self.add(a, c), None), (b, self.neg(d)), (self.sub(a, c), None)]
        u = self.rfft(xs[0::2])
        z1 = self.rfft(xs[1::4])
        z3 = self.rfft(xs[3::4])

        def get_u(k):
            k %= n // 2
            return u[k] if k <= n // 4 else self.cconj(u[n // 2 - k])

        out = [None] * (n // 2 + 1)
        for k in range(n // 8 + 1):
            t1 = self.twiddle(z1[k], k, n)
            t3 = self.twiddle(z3[k], 3 * k, n)
            sm = self.cadd(t1, t3)
            df = self.csub(t1, t3)
            u0, u1 = get_u(k), get_u(k + n // 4)
            out[k] = self.cadd(u0, sm)
            out[n // 2 - k] = self.cconj(self.csub(u0, sm))
            mdf = (df[1], self.neg(df[0]))
            out[k + n // 4] = self.cadd(u1, mdf)
            if k > 0:
                out[n // 4 - k] = self.cconj(self.csub(u1, mdf))
        return out

    def order(self, outs):
        seen, order = set(), []
        for o in outs:
            if o is None or o[0] in seen:
                continue
            stack = [(o[0], False)]
            while stack:
                n, done = stack.pop()
                if done:
                    order.append(n)
                    continue
                if n in seen:
                    continue
                seen.add(n)
                stack.append((n, True))
                kind, a, b = self.ops[n]
                if kind in ("add", "sub"):
                    stack.append((b, False))
                    stack.append((a, False))
                elif kind == "mul":
                    stack.append((a, False))
        return order

    def transpose(self, outs):
        g = _Prog()
        adj = {}

        def acc(n, v):
            if v is not None:
                adj[n] = g.add(adj.get(n), v)

        for i, o in enumerate(outs):
            if o is not None:
                acc(o[0], g.mul(o[1], g.inp(i)))
        res = {}
        for n in sorted(set(self.order(outs)), reverse=True):
            kind, a, b = self.ops[n]
            v = adj.get(n)
            if v is None:
                continue
            if kind == "in":
                res[a] = v
            elif kind == "add":
                acc(a, v)
                acc(b, v)
            elif kind == "sub":
                acc(a, v)
                acc(b, g.neg(v))
            else:
                acc(a, g.mul(b, v))
        return g, res

    def run(self, outs, load, emit, keep_sign=True):
        val = {}
        want = {}
        for i, o in enumerate(outs):
            if o is not None:
                want.setdefault(o[0], []).append((i, o[1]))
        for n in self.order(outs):
            kind, a, b = self.ops[n]
            if kind == "in":
                v = load(a)
            elif kind == "add":
                v = val[a] + val[b]
            elif kind == "sub":
                v = val[a] - val[b]
            else:
                v = val[a] * np.float32(b)
            val[n] = v
            for i, sg in want.get(n, ()):
                emit(i, -v if (sg < 0 and keep_sign) else v)


def _lhs_outputs(p, spec, n):
    outs = [spec[0][0], spec[n // 2][0]]
    for k in range(1, n // 2):
        a, b = spec[k]
        outs += [p.add(a, b), a, b]
    return outs


class _Plan:
    def __init__(self, n):
        self.n = n
        self.taps = 16
        self.hop = n - self.taps + 1
        self.ns = 2 + 3 * (n // 2 - 1)
        self.fwd = _Prog()
        spec = self.fwd.rfft([self.fwd.inp(i) for i in range(n)])
        self.fwd_outs = _lhs_outputs(self.fwd, spec, n)
        lhs_sign = [o[1] for o in self.fwd_outs]
        p = _Prog()
        spec = p.rfft([p.inp(i) if i < self.hop else None for i in range(n)])
        self.inv, res = p.transpose(_lhs_outputs(p, spec, n))
        self.inv_outs = [res[t] for t in range(self.hop)]
        self.inv_src = [0, 1]
        for k in range(n // 2 - 1):
            base = 2 + 3 * k
            self.inv_src += [base, base + 2, base + 1]
        self.wprog, self.wouts, self.wtap = [], [], []
        for ph in range(2):
            p = _Prog()
            xs = [None] * n
            for j in range(self.taps):
                if not (ph == 0 and j == 0):
                    xs[j] = p.inp(2 * j - 1 if ph == 0 else 2 * j)
            spec = p.rfft(xs)
            outs = [p.mul(0.5, spec[0][0]), p.mul(0.5, spec[n // 2][0])]
            for k in range(1, n // 2):
                c, dm = spec[k]
                d = p.neg(dm)
                outs += [c, p.sub(d, c), p.neg(p.add(c, d))]
            outs = [(o[0], o[1] * s) for o, s in zip(outs, lhs_sign)]
            self.wprog.append(p)
            self.wouts.append(outs)


_FFT_N = 32
_PLAN = _Plan(_FFT_N)

_C0 = math.sqrt(2.0 / math.pi)
_KAPPA = 0.044715 / (_C0 * _C0)


def _gelu2(z):
    inner = z * (np.float32(_KAPPA) * (z * z) + np.float32(1.0))
    return z + z * jnp.tanh(inner)


_B, _T, _D, _K, _U = 2, 16000, 256, 31, 8
_T1, _T2 = _T // 2, _T // 4
_S2 = 502
_S1 = 2 * _S2
_HOP = _PLAN.hop
_NS = _PLAN.ns
_CB = 5
_C1 = [_CB] * 11 + [6]
_CB2, _NSTEP2 = 5, 6
_NB1 = sum(_C1)
_XOFF = 24
_XROWS = -(-(7 * _S1 + _HOP * (_NB1 - 1) + _FFT_N) // 8) * 8
_HROWS = 2 * _HOP * (_CB2 * _NSTEP2 - 1) + 2 * _FFT_N
_FROWS = _HOP * _CB2 * _NSTEP2
_TJ = _HOP
_XPARTS = 8
_OSLOTS = 4
_WPARTS = 4
_NDEP = 3
_COST = {"fx": 262, "fh": 230, "inv": 350, "w": 280}


def _x_piece_bounds():
    edges = []
    for s in range(8):
        for p in range(_XPARTS):
            edges.append(min(max((s * _S1 + p * (_S1 // _XPARTS) - _XOFF) // 8 * 8, 0), _T1))
    edges.append(_T1)
    return edges


def _merge(*lists):
    lists = [l for l in lists if l]
    pos = [0] * len(lists)
    out = []
    for _ in range(sum(len(l) for l in lists)):
        j = min((q for q in range(len(lists)) if pos[q] < len(lists[q])),
                key=lambda q: (pos[q] + 0.5) / len(lists[q]))
        out.append(lists[j][pos[j]])
        pos[j] += 1
    return out


def _dyn8(v):
    return v if isinstance(v, int) else pl.multiple_of(v, 8)


def _emit_step(items, units, mask):
    starts = np.cumsum([0] + [2 * (rows // 8) for rows, _, _ in items])
    nev = int(starts[-1])
    tot = sum(c for c, _ in units) or 1
    margin = min(40, nev // 8)
    sched, cum = [], 0
    for cost, fn in units:
        evs = [min(int((cum + cost * q / _NDEP) / tot * (nev - margin)) + 1, nev - 1)
               for q in range(_NDEP)]
        cum += cost
        sched.append((fn, evs))
    results = {}

    def event(e):
        j = int(np.searchsorted(starts, e, side="right")) - 1
        rg, nn = divmod(e - int(starts[j]), 2)
        return results[j][rg * 8:(rg + 1) * 8, nn * 128:(nn + 1) * 128]

    pi = 0
    for j, (rows, dot_fn, post_fn) in enumerate(items):
        results[j] = dot_fn()
        while pi < len(sched) and max(sched[pi][1]) < starts[j + 1]:
            fn, evs = sched[pi]
            pi += 1
            fn([functools.partial(event, e) for e in evs])
        post_fn(results[j])
    assert pi == len(sched)


def _pick(cnt, total, deps):
    if not deps:
        return None
    j, rem = divmod(cnt * len(deps), total)
    return j if rem < len(deps) else None


def _kernel(x_hbm, w1_hbm, w2_hbm, g_hbm, wf_hbm, wg_hbm, wo_hbm, out_hbm,
            v1, v2, spec_a, spec_b, y_a, y_b, hbuf, xbuf, w1buf, w2buf,
            gbuf, wfbuf, wgbuf, wobuf, gebuf, fbuf, febuf, obuf,
            sem_w, sem_s, sem_x, sem_o):
    plan = _PLAN
    n, hop, ns = plan.n, plan.hop, plan.ns
    specs, ys = (spec_a, spec_b), (y_a, y_b)

    xu = x_hbm.bitcast(jnp.uint32)
    edges = _x_piece_bounds()

    def x_copies(part):
        cps = []
        for s in range(8):
            r0, r1 = edges[s * _XPARTS + part], edges[s * _XPARTS + part + 1]
            for cs in range(2):
                cps.append(pltpu.make_async_copy(
                    xu.at[:, pl.ds(r0, r1 - r0), pl.ds(cs * 128, 128)],
                    xbuf.at[:, cs, pl.ds(_XOFF + r0, r1 - r0), :],
                    sem_x.at[part]))
        return cps

    w1_copies = [[pltpu.make_async_copy(w1_hbm.at[t], w1buf.at[t], sem_w.at[ph])
                  for t in range(1 - ph, _K, 2)] for ph in range(2)]
    wrows = _D // _WPARTS
    w2_copies = [pltpu.make_async_copy(w2_hbm.at[:, pl.ds(p * wrows, wrows), :],
                                       w2buf.at[:, pl.ds(p * wrows, wrows), :], sem_w.at[2 + p])
                 for p in range(_WPARTS)]
    small = [pltpu.make_async_copy(src, dst, sem_s.at[i]) for i, (src, dst) in
             enumerate([(g_hbm, gbuf), (wf_hbm, wfbuf), (wg_hbm, wgbuf), (wo_hbm, wobuf)])]

    for c in w1_copies[0]:
        c.start()
    zero8 = jnp.zeros((8, 128), jnp.uint32)
    for bb in range(2):
        for cs in range(2):
            for r in range(0, _XOFF, 8):
                xbuf[bb, cs, pl.ds(r, 8), :] = zero8
            for r in range(_XOFF + _T1, _XROWS, 8):
                xbuf[bb, cs, pl.ds(r, 8), :] = zero8
    zrow = jnp.zeros((8, 128), jnp.float32)
    for bb in range(2):
        for cs in range(2):
            for r in range(_NB1 * hop, _HROWS):
                hbuf[bb, cs, r] = zrow

    def w_unit(wbuf, vbuf, scale, row, half, ph, nt, deps=(), mask=None):
        cnt = [0]

        def load(tap):
            w = wbuf[tap, pl.ds(_dyn8(row + 8 * half), 8), pl.ds(nt * 128, 128)].astype(jnp.float32)
            j = _pick(cnt[0], 16, deps)
            cnt[0] += 1
            if j is not None:
                w = jnp.where(mask, w, deps[j]())
            return w * np.float32(scale)

        def emit(i, v):
            vbuf[i, 2 * ph + row // 128, nt, pl.ds(_dyn8((row % 128) // 2) + 4 * half, 4), :] = (
                pltpu.bitcast(v.astype(jnp.bfloat16), jnp.uint32))
        plan.wprog[ph].run(plan.wouts[ph], load, emit)

    def fwd_unit(load_in, spec, row, col, deps, mask):
        cnt = [0]

        def load(q):
            j = _pick(cnt[0], n, deps)
            cnt[0] += 1
            return load_in(q, None if j is None else deps[j], mask)

        def emit(i, v):
            spec[col // 128, i, pl.ds(row, 8), :] = v
        plan.fwd.run(plan.fwd_outs, load, emit, keep_sign=False)

    def fx_unit(spec, blk, be, bb, cs, ph, zd, deps=(), mask=None):
        base = blk * hop
        if ph == 1:
            base = base + zd

        def load_in(q, dep, mask):
            v = xbuf[bb, cs, pl.ds(base + q, 8, stride=_S1), :]
            if dep is not None:
                v = jnp.where(mask, v, lax.bitcast_convert_type(dep(), jnp.uint32))
            v = (v << 16) if ph == 0 else (v & jnp.uint32(0xFFFF0000))
            return lax.bitcast_convert_type(v, jnp.float32)
        fwd_unit(load_in, spec, _dyn8(be * 16 + bb * 8), ph * 256 + cs * 128, deps, mask)

    def fh_unit(spec, blk, be, bb, cs, ph, deps=(), mask=None):
        base = blk * 2 * hop + ph

        def load_in(q, dep, mask):
            v = hbuf[bb, cs, base + 2 * q]
            if dep is not None:
                v = jnp.where(mask, v, dep())
            return v
        fwd_unit(load_in, spec, _dyn8(be * 16 + bb * 8), ph * 256 + cs * 128, deps, mask)

    def inv_unit(ybuf, dst, scale, blk, be, bb, nt, deps=(), mask=None):
        cnt = [0]
        row = _dyn8(be * 16 + bb * 8)

        def load(i):
            v = ybuf[nt, plan.inv_src[i], pl.ds(row, 8), :]
            j = _pick(cnt[0], ns, deps)
            cnt[0] += 1
            if j is not None:
                v = jnp.where(mask, v, deps[j]())
            return v

        def store(t, z):
            hval = _gelu2(z)
            if scale != 1.0:
                hval = hval * np.float32(scale)
            dst[bb, nt, blk * hop + t] = hval
        plan.inv.run(plan.inv_outs, load, store)

    def fx_units(spec, blk0, nblk, zd, mask):
        return [(_COST["fx"], functools.partial(fx_unit, spec, blk0 + be, be, bb, cs, ph, zd, mask=mask))
                for be in range(nblk) for bb in range(2) for cs in range(2) for ph in range(2)]

    def fh_units(spec, blk0, nblk, mask):
        return [(_COST["fh"], functools.partial(fh_unit, spec, blk0 + be, be, bb, cs, ph, mask=mask))
                for be in range(nblk) for bb in range(2) for cs in range(2) for ph in range(2)]

    def inv_units(ybuf, dst, scale, blk0, nblk, mask):
        return [(_COST["inv"], functools.partial(inv_unit, ybuf, dst, scale, blk0 + be, be, bb, nt, mask=mask))
                for be in range(nblk) for bb in range(2) for nt in range(2)]

    def w2_units(rg0, nrg, mask):
        return [(_COST["w"], functools.partial(
                    w_unit, w2buf, v2, (2.0 / n) * 0.5, pl.multiple_of((rg0 + r) * 16, 16)
                    if not isinstance(rg0, int) else (rg0 + r) * 16, half, ph, nt, mask=mask))
                for r in range(nrg) for half in range(2) for ph in range(2) for nt in range(2)]

    def conv_items(vbuf, spec, ybuf, m, only=None):
        items = []
        for i in range(ns):
            hold = []

            def dot_fn(i=i, h=0):
                w = jnp.concatenate(
                    [jnp.concatenate(
                        [pltpu.bitcast(vbuf[i, 2 * h + q, nt, pl.ds(0, 64), :], jnp.bfloat16)
                         for q in range(2)], axis=0) for nt in range(2)], axis=1)
                lhs = jnp.concatenate([spec[2 * h + q, i, pl.ds(0, m), :] for q in range(2)], axis=1)
                return jnp.dot(lhs, w, preferred_element_type=jnp.float32)

            def post0(r, hold=hold):
                hold.append(r)

            def post1(r, i=i, hold=hold):
                y = hold[0] + r
                for nt in range(2):
                    ybuf[nt, i, pl.ds(0, m), :] = y[:, nt * 128:(nt + 1) * 128]
            def post_first(r, i=i):
                for nt in range(2):
                    ybuf[nt, i, pl.ds(0, m), :] = r[:, nt * 128:(nt + 1) * 128]

            def post_second(r, i=i):
                for nt in range(2):
                    ybuf[nt, i, pl.ds(0, m), :] = (
                        ybuf[nt, i, pl.ds(0, m), :] + r[:, nt * 128:(nt + 1) * 128])
            if only is None:
                items.append((m, functools.partial(dot_fn, i, 0), post0))
                items.append((m, functools.partial(dot_fn, i, 1), post1))
            else:
                items.append((m, functools.partial(dot_fn, i, only),
                              post_second if only else post_first))
        return items

    def block(fn, zd):
        def body(_, c):
            fn()
            return c
        lax.fori_loop(0, 1 + zd, body, 0)

    def opaque_zero(i):
        return (i * (i + 1)) & 1

    def true_mask(zd):
        return jnp.full((8, 128), zd, jnp.int32) == 0

    c1_start = [int(v) for v in np.cumsum([0] + _C1)]

    for c in x_copies(0):
        c.start()
    for c in w1_copies[0]:
        c.wait()
    for c in w1_copies[1]:
        c.start()

    def v1_body(i, carry):
        for r in range(2):
            row = pl.multiple_of((2 * i + r) * 16, 16)
            for half in range(2):
                for nt in range(2):
                    w_unit(w1buf, v1, (2.0 / n) * _C0, row, half, 0, nt)
        return carry
    with jax.named_scope("v1"):
        lax.fori_loop(0, _D // 32, v1_body, 0)

    zd0 = opaque_zero(xbuf[0, 0, 0, 0].astype(jnp.int32))
    mask0 = true_mask(zd0)

    need, have = {}, 0
    for c in range(len(_C1) - 1):
        top = hop * (c1_start[c + 2] - 1) + n - _XOFF
        req = min(_XPARTS - 1, max(
            p for s8 in range(8) for p in range(_XPARTS)
            if edges[s8 * _XPARTS + p] < min(s8 * _S1 + top, _T1)))
        need[c] = list(range(have + 1, req + 1))
        have = max(have, req)
    assert have == _XPARTS - 1

    def start_parts(c):
        for p in need.get(c, []):
            for cp in x_copies(p):
                cp.start()

    def wait_parts(c):
        for p in need.get(c, []):
            for cp in x_copies(p):
                cp.wait()

    with jax.named_scope("x0wait"):
        for c in x_copies(0):
            c.wait()
    start_parts(0)
    w2_copies[0].start()
    start_parts(1)

    def fill_body(u, carry):
        zd = opaque_zero(u)
        for cs in range(2):
            for ph in range(2):
                fx_unit(spec_a, u // 2, u // 2, u % 2, cs, ph, zd)
        return carry
    with jax.named_scope("fill"):
        lax.fori_loop(0, _C1[0] * 2, fill_body, 0)

    for c in w1_copies[1]:
        c.wait()

    def step0a_body():
        units = [(_COST["w"], functools.partial(w_unit, w1buf, v1, (2.0 / n) * _C0, rg * 16,
                                                half, 1, nt, mask=mask0))
                 for rg in range(_D // 16) for half in range(2) for nt in range(2)]
        _emit_step(conv_items(v1, spec_a, y_a, _CB * 16, only=0), units, mask0)
    with jax.named_scope("step0a"):
        block(step0a_body, zd0)

    with jax.named_scope("x1wait"):
        wait_parts(0)

    def step0b_body():
        _emit_step(conv_items(v1, spec_a, y_a, _CB * 16, only=1),
                   fx_units(spec_b, c1_start[1], _CB, zd0, mask0), mask0)
    with jax.named_scope("step0b"):
        block(step0b_body, zd0)

    def before_step(c):
        wait_parts(c)
        start_parts(c + 1)
        for p, first_use in enumerate((1, 5, 9, 11)):
            if c == first_use:
                w2_copies[p].wait()
            if p > 0 and c == first_use - 2:
                w2_copies[p].start()
        if c == 8:
            for cp in small:
                cp.start()

    def conv1_body(it, carry):
        zd = opaque_zero(it)
        mask = true_mask(zd)
        for par in (1, 0):
            c = 2 * it + (1 if par == 1 else 2)
            for k in range(4):
                pl.when(it == k)(functools.partial(before_step, 2 * k + (1 if par == 1 else 2)))
            block(lambda: _emit_step(
                conv_items(v1, specs[par], ys[par], _CB * 16),
                _merge(fx_units(specs[1 - par], (c + 1) * _CB, _CB, zd, mask) +
                       inv_units(ys[1 - par], hbuf, 1.0, (c - 1) * _CB, _CB, mask),
                       w2_units(c - 1, 1, mask)), mask), zd)
        return carry
    with jax.named_scope("conv1"):
        lax.fori_loop(0, 4, conv1_body, 0)

    sub = lax.broadcasted_iota(jnp.int32, (8, 128), 0)

    def mask_rows(r0, r1, s):
        def body(r, carry):
            for bb in range(2):
                for cs in range(2):
                    hbuf[bb, cs, r] = jnp.where(sub == s, 0.0, hbuf[bb, cs, r])
            return carry
        lax.fori_loop(r0, r1, body, 0)
    mask_rows(0, 16, 0)

    for c in (9, 10):
        par = c % 2
        before_step(c)
        with jax.named_scope("step%d" % c):
            block(lambda: _emit_step(
                conv_items(v1, specs[par], ys[par], _CB * 16),
                _merge(fx_units(specs[1 - par], c1_start[c + 1], _C1[c + 1], zd0, mask0) +
                       inv_units(ys[1 - par], hbuf, 1.0, c1_start[c - 1], _CB, mask0),
                       w2_units(8 + 2 * (c - 9), 2, mask0)), mask0), zd0)

    before_step(11)

    def step11_body():
        _emit_step(conv_items(v1, spec_b, y_b, _C1[11] * 16),
                   _merge(fh_units(spec_a, 0, _CB2, mask0) +
                          inv_units(y_a, hbuf, 1.0, c1_start[10], _CB, mask0),
                          w2_units(12, 4, mask0)), mask0)
    with jax.named_scope("step11"):
        block(step11_body, zd0)

    fscale = 0.5 / _C0

    def step8_body():
        zd, mask = zd0, mask0
        _emit_step(conv_items(v2, spec_a, y_a, _CB2 * 16),
                   fh_units(spec_b, _CB2, _CB2, mask) +
                   inv_units(y_b, hbuf, 1.0, c1_start[11], _C1[11], mask), mask)
    with jax.named_scope("step8"):
        block(step8_body, zd0)
    mask_rows(_T1 - 7 * _S1 + 16, _NB1 * hop, 7)

    def conv2_body(it, carry):
        zd = opaque_zero(it)
        mask = true_mask(zd)
        for par in (1, 0):
            c = 2 * it + (1 if par == 1 else 2)
            block(lambda: _emit_step(
                conv_items(v2, specs[par], ys[par], _CB2 * 16),
                (fh_units(specs[1 - par], (c + 1) * _CB2, _CB2, mask) +
                 inv_units(ys[1 - par], fbuf, fscale, (c - 1) * _CB2, _CB2, mask)),
                mask), zd)
        return carry
    with jax.named_scope("conv2"):
        lax.fori_loop(0, 2, conv2_body, 0)

    for c in small:
        c.wait()
    gebuf[...] = jnp.dot(gbuf[...].reshape(_B * _U, _D), wgbuf[...],
                         preferred_element_type=jnp.float32).reshape(_B, _U, _D)

    def fe_item(slot, tile):
        def dot_fn():
            f = jnp.concatenate(
                [jnp.concatenate(
                    [fbuf[bb, cs, pl.ds(tile * _TJ, _TJ)].reshape(_TJ * 8, 128) for cs in range(2)],
                    axis=1) for bb in range(2)], axis=0)
            return jnp.dot(f, wfbuf[...], preferred_element_type=jnp.float32)

        def post(r):
            febuf[slot] = r.reshape(_B, _TJ, 8, _D)
        return (_TJ * 16, dot_fn, post)

    def step13_body():
        zd, mask = zd0, mask0
        _emit_step(conv_items(v2, spec_b, y_b, _CB2 * 16) + [fe_item(0, 0)],
                   inv_units(y_a, fbuf, fscale, 4 * _CB2, _CB2, mask), mask)
    with jax.named_scope("step13"):
        block(step13_body, zd0)

    def out_copies(slot, t0, rows_of):
        cps = []
        for s in range(8):
            rows = rows_of(s)
            if rows > 0:
                cps.append(pltpu.make_async_copy(
                    obuf.at[slot, :, s, pl.ds(0, rows)],
                    out_hbm.at[:, pl.ds(s * _S2 + t0, rows)],
                    sem_o.at[slot]))
        return cps

    def joint_item(fslot, oslot, tj):
        def dot_fn():
            rows = []
            for tt in range(tj):
                for r in range(16):
                    fr = febuf[fslot, r // 8, tt, pl.ds(r % 8, 1), :]
                    rows.append(jnp.tanh(jnp.broadcast_to(fr, (_U, _D)) + gebuf[r // 8]))
            return jnp.dot(jnp.concatenate(rows, axis=0), wobuf[...],
                           preferred_element_type=jnp.float32)

        def post(o):
            o = o.reshape(tj, _B, 8, _U, _D).astype(jnp.bfloat16)
            for tt in range(tj):
                obuf[oslot, :, :, tt] = o[tt]
        return (tj * 16 * _U, dot_fn, post)

    full = lambda s: _TJ
    ntiles = -(-_S2 // _TJ)
    nfull = (_T2 - 7 * _S2) // _TJ
    assert nfull % _OSLOTS == 0 and _OSLOTS == 4

    def first_body():
        _emit_step([fe_item(1, 1), joint_item(0, 0, _TJ), fe_item(0, 2), joint_item(1, 1, _TJ)],
                   inv_units(y_b, fbuf, fscale, 5 * _CB2, _CB2, mask0), mask0)
        for slot in range(2):
            for c in out_copies(slot, slot * _TJ, full):
                c.start()
    with jax.named_scope("first"):
        block(first_body, zd0)

    def joint_body(i2, carry):
        @pl.when(i2 >= 2)
        def _():
            for j in range(2):
                for c in out_copies((i2 % 2) * 2 + j, (2 * i2 + j - _OSLOTS) * _TJ, full):
                    c.wait()
        for j in range(2):
            tile = 2 * i2 + j
            oslot = (i2 % 2) * 2 + j
            _emit_step([fe_item(1 - j, tile + 1), joint_item(j, oslot, _TJ)], [], None)
            for c in out_copies(oslot, tile * _TJ, full):
                c.start()
        return carry
    with jax.named_scope("joint"):
        lax.fori_loop(1, nfull // 2, joint_body, 0)

    pending = {k: out_copies(k, (nfull - _OSLOTS + k) * _TJ, full) for k in range(_OSLOTS)}
    for tile in range(nfull, ntiles):
        oslot, t0 = tile % _OSLOTS, tile * _TJ
        tj = min(_TJ, _S2 - t0)
        rows_of = lambda s, t0=t0, tj=tj: max(0, min(tj, (_T2 - 7 * _S2 if s == 7 else _S2) - t0))
        for c in pending[oslot]:
            c.wait()
        items = ([fe_item(1 - tile % 2, tile + 1)] if tile + 1 < ntiles else []) + [
            joint_item(tile % 2, oslot, tj)]
        _emit_step(items, [], None)
        pending[oslot] = out_copies(oslot, t0, rows_of)
        for c in pending[oslot]:
            c.start()
    for k in range(_OSLOTS):
        for c in pending[k]:
            c.wait()


@jax.jit
def pallas_standalone__seq2seq_rnn_t_joint__speech_kernel(
    x: jax.Array,
    w1: jax.Array,
    w2: jax.Array,
    g: jax.Array,
    w_f: jax.Array,
    w_g: jax.Array,
    w_o: jax.Array,
):
    assert x.shape == (_B, _T, _D) and w1.shape == (_K, _D, _D) and w2.shape == (_K, _D, _D)
    assert g.shape == (_B, _U, _D)
    bf, f32 = jnp.bfloat16, jnp.float32
    m = max(_C1 + [_CB2]) * 16
    scratch = [
        pltpu.VMEM((_NS, 4, 2, 72, 128), jnp.uint32),
        pltpu.VMEM((_NS, 4, 2, 72, 128), jnp.uint32),
        pltpu.VMEM((4, _NS, m + 8, 128), f32),
        pltpu.VMEM((4, _NS, m + 8, 128), f32),
        pltpu.VMEM((2, _NS, m + 8, 128), f32),
        pltpu.VMEM((2, _NS, m + 8, 128), f32),
        pltpu.VMEM((2, 2, _HROWS + 1, 8, 128), f32),
        pltpu.VMEM((2, 2, _XROWS, 128), jnp.uint32),
        pltpu.VMEM((_K, _D, _D), bf),
        pltpu.VMEM((_K, _D, _D), bf),
        pltpu.VMEM((_B, _U, _D), bf),
        pltpu.VMEM((_D, _D), bf),
        pltpu.VMEM((_D, _D), bf),
        pltpu.VMEM((_D, _D), bf),
        pltpu.VMEM((_B, _U, _D), f32),
        pltpu.VMEM((2, 2, _FROWS + 1, 8, 128), f32),
        pltpu.VMEM((2, _B, _TJ, 8, _D), f32),
        pltpu.VMEM((_OSLOTS, _B, 8, _TJ, _U, _D), bf),
        pltpu.SemaphoreType.DMA((_WPARTS + 2,)),
        pltpu.SemaphoreType.DMA((4,)),
        pltpu.SemaphoreType.DMA((_XPARTS,)),
        pltpu.SemaphoreType.DMA((_OSLOTS,)),
    ]
    any_spec = pl.BlockSpec(memory_space=pl.ANY)
    return pl.pallas_call(
        _kernel,
        out_shape=jax.ShapeDtypeStruct((_B, _T2, _U, _D), bf),
        in_specs=[any_spec] * 7,
        out_specs=any_spec,
        scratch_shapes=scratch,
        compiler_params=pltpu.CompilerParams(vmem_limit_bytes=127 * 1024 * 1024),
    )(x, w1, w2, g, w_f, w_g, w_o)
```

```python
import functools
import math

import numpy as np

import jax
import jax.numpy as jnp
from jax import lax
import jax.experimental.pallas as pl
import jax.experimental.pallas.tpu as pltpu


class _Prog:
    def __init__(self):
        self.ops = []
        self.cse = {}

    def _node(self, kind, a, b):
        key = (kind, a, b)
        if key not in self.cse:
            self.ops.append(key)
            self.cse[key] = len(self.ops) - 1
        return self.cse[key]

    def inp(self, i):
        return (self._node("in", i, None), 1)

    def neg(self, x):
        return None if x is None else (x[0], -x[1])

    def add(self, x, y):
        if x is None:
            return y
        if y is None:
            return x
        (a, sa), (b, sb) = x, y
        if sa == sb:
            return (self._node("add", min(a, b), max(a, b)), sa)
        if sa > 0:
            return (self._node("sub", a, b), 1)
        return (self._node("sub", b, a), 1)

    def sub(self, x, y):
        return self.add(x, self.neg(y))

    def mul(self, c, x):
        if x is None or c == 0:
            return None
        if c == 1:
            return x
        if c == -1:
            return self.neg(x)
        return (self._node("mul", x[0], abs(float(c))), x[1] * (1 if c > 0 else -1))

    def cadd(self, z, w):
        return (self.add(z[0], w[0]), self.add(z[1], w[1]))

    def csub(self, z, w):
        return (self.sub(z[0], w[0]), self.sub(z[1], w[1]))

    def cconj(self, z):
        return (z[0], self.neg(z[1]))

    def twiddle(self, z, num, den):
        num %= den
        a, b = z
        if (8 * num) % den == 0:
            e = (8 * num) // den
            r = math.sqrt(0.5)
            if e == 0:
                return (a, b)
            if e == 2:
                return (b, self.neg(a))
            if e == 4:
                return (self.neg(a), self.neg(b))
            if e == 6:
                return (self.neg(b), a)
            if e == 1:
                return (self.mul(r, self.add(a, b)), self.mul(r, self.sub(b, a)))
            if e == 3:
                return (self.mul(r, self.sub(b, a)), self.mul(-r, self.add(a, b)))
            if e == 5:
                return (self.mul(-r, self.add(a, b)), self.mul(r, self.sub(a, b)))
            return (self.mul(r, self.sub(a, b)), self.mul(r, self.add(a, b)))
        th = -2.0 * math.pi * num / den
        c, s = math.cos(th), math.sin(th)
        return (self.sub(self.mul(c, a), self.mul(s, b)), self.add(self.mul(s, a), self.mul(c, b)))

    def rfft(self, xs):
        n = len(xs)
        if n == 1:
            return [(xs[0], None)]
        if n == 2:
            return [(self.add(xs[0], xs[1]), None), (self.sub(xs[0], xs[1]), None)]
        if n == 4:
            a = self.add(xs[0], xs[2])
            b = self.sub(xs[0], xs[2])
            c = self.add(xs[1], xs[3])
            d = self.sub(xs[1], xs[3])
            return [(self.add(a, c), None), (b, self.neg(d)), (self.sub(a, c), None)]
        u = self.rfft(xs[0::2])
        z1 = self.rfft(xs[1::4])
        z3 = self.rfft(xs[3::4])

        def get_u(k):
            k %= n // 2
            return u[k] if k <= n // 4 else self.cconj(u[n // 2 - k])

        out = [None] * (n // 2 + 1)
        for k in range(n // 8 + 1):
            t1 = self.twiddle(z1[k], k, n)
            t3 = self.twiddle(z3[k], 3 * k, n)
            sm = self.cadd(t1, t3)
            df = self.csub(t1, t3)
            u0, u1 = get_u(k), get_u(k + n // 4)
            out[k] = self.cadd(u0, sm)
            out[n // 2 - k] = self.cconj(self.csub(u0, sm))
            mdf = (df[1], self.neg(df[0]))
            out[k + n // 4] = self.cadd(u1, mdf)
            if k > 0:
                out[n // 4 - k] = self.cconj(self.csub(u1, mdf))
        return out

    def order(self, outs):
        seen, order = set(), []
        for o in outs:
            if o is None or o[0] in seen:
                continue
            stack = [(o[0], False)]
            while stack:
                n, done = stack.pop()
                if done:
                    order.append(n)
                    continue
                if n in seen:
                    continue
                seen.add(n)
                stack.append((n, True))
                kind, a, b = self.ops[n]
                if kind in ("add", "sub"):
                    stack.append((b, False))
                    stack.append((a, False))
                elif kind == "mul":
                    stack.append((a, False))
        return order

    def transpose(self, outs):
        g = _Prog()
        adj = {}

        def acc(n, v):
            if v is not None:
                adj[n] = g.add(adj.get(n), v)

        for i, o in enumerate(outs):
            if o is not None:
                acc(o[0], g.mul(o[1], g.inp(i)))
        res = {}
        for n in sorted(set(self.order(outs)), reverse=True):
            kind, a, b = self.ops[n]
            v = adj.get(n)
            if v is None:
                continue
            if kind == "in":
                res[a] = v
            elif kind == "add":
                acc(a, v)
                acc(b, v)
            elif kind == "sub":
                acc(a, v)
                acc(b, g.neg(v))
            else:
                acc(a, g.mul(b, v))
        return g, res

    def run(self, outs, load, emit, keep_sign=True):
        val = {}
        want = {}
        for i, o in enumerate(outs):
            if o is not None:
                want.setdefault(o[0], []).append((i, o[1]))
        for n in self.order(outs):
            kind, a, b = self.ops[n]
            if kind == "in":
                v = load(a)
            elif kind == "add":
                v = val[a] + val[b]
            elif kind == "sub":
                v = val[a] - val[b]
            else:
                v = val[a] * np.float32(b)
            val[n] = v
            for i, sg in want.get(n, ()):
                emit(i, -v if (sg < 0 and keep_sign) else v)


def _lhs_outputs(p, spec, n):
    outs = [spec[0][0], spec[n // 2][0]]
    for k in range(1, n // 2):
        a, b = spec[k]
        outs += [p.add(a, b), a, b]
    return outs


class _Plan:
    def __init__(self, n):
        self.n = n
        self.taps = 16
        self.hop = n - self.taps + 1
        self.ns = 2 + 3 * (n // 2 - 1)
        self.fwd = _Prog()
        spec = self.fwd.rfft([self.fwd.inp(i) for i in range(n)])
        self.fwd_outs = _lhs_outputs(self.fwd, spec, n)
        lhs_sign = [o[1] for o in self.fwd_outs]
        p = _Prog()
        spec = p.rfft([p.inp(i) if i < self.hop else None for i in range(n)])
        self.inv, res = p.transpose(_lhs_outputs(p, spec, n))
        self.inv_outs = [res[t] for t in range(self.hop)]
        self.inv_src = [0, 1]
        for k in range(n // 2 - 1):
            base = 2 + 3 * k
            self.inv_src += [base, base + 2, base + 1]
        self.wprog, self.wouts, self.wtap = [], [], []
        for ph in range(2):
            p = _Prog()
            xs = [None] * n
            for j in range(self.taps):
                if not (ph == 0 and j == 0):
                    xs[j] = p.inp(2 * j - 1 if ph == 0 else 2 * j)
            spec = p.rfft(xs)
            outs = [p.mul(0.5, spec[0][0]), p.mul(0.5, spec[n // 2][0])]
            for k in range(1, n // 2):
                c, dm = spec[k]
                d = p.neg(dm)
                outs += [c, p.sub(d, c), p.neg(p.add(c, d))]
            outs = [(o[0], o[1] * s) for o, s in zip(outs, lhs_sign)]
            self.wprog.append(p)
            self.wouts.append(outs)


_FFT_N = 32
_PLAN = _Plan(_FFT_N)

_C0 = math.sqrt(2.0 / math.pi)
_KAPPA = 0.044715 / (_C0 * _C0)


def _gelu2(z):
    inner = z * (np.float32(_KAPPA) * (z * z) + np.float32(1.0))
    return z + z * jnp.tanh(inner)


_B, _T, _D, _K, _U = 2, 16000, 256, 31, 8
_T1, _T2 = _T // 2, _T // 4
_S2 = 502
_S1 = 2 * _S2
_HOP = _PLAN.hop
_NS = _PLAN.ns
_CB = 5
_C1 = [_CB] * 11 + [6]
_CB2, _NSTEP2 = 5, 6
_NB1 = sum(_C1)
_XOFF = 24
_XSLOTS = 4
_XSEG = 140
_HROWS = 2 * _HOP * (_CB2 * _NSTEP2 - 1) + 2 * _FFT_N
_FROWS = _HOP * _CB2 * _NSTEP2
_TJ = _HOP
_OSLOTS = 4
_WPARTS = 4
_NDEP = 3
_COST = {"fx": 262, "fh": 230, "inv": 350, "w": 280}


def _merge(*lists):
    lists = [l for l in lists if l]
    pos = [0] * len(lists)
    out = []
    for _ in range(sum(len(l) for l in lists)):
        j = min((q for q in range(len(lists)) if pos[q] < len(lists[q])),
                key=lambda q: (pos[q] + 0.5) / len(lists[q]))
        out.append(lists[j][pos[j]])
        pos[j] += 1
    return out


def _dyn8(v):
    return v if isinstance(v, int) else pl.multiple_of(v, 8)


def _emit_step(items, units, mask):
    starts = np.cumsum([0] + [2 * (rows // 8) for rows, _, _ in items])
    nev = int(starts[-1])
    tot = sum(c for c, _ in units) or 1
    margin = min(40, nev // 8)
    sched, cum = [], 0
    for cost, fn in units:
        evs = [min(int((cum + cost * q / _NDEP) / tot * (nev - margin)) + 1, nev - 1)
               for q in range(_NDEP)]
        cum += cost
        sched.append((fn, evs))
    results = {}

    def event(e):
        j = int(np.searchsorted(starts, e, side="right")) - 1
        rg, nn = divmod(e - int(starts[j]), 2)
        return results[j][rg * 8:(rg + 1) * 8, nn * 128:(nn + 1) * 128]

    pi = 0
    for j, (rows, dot_fn, post_fn) in enumerate(items):
        results[j] = dot_fn()
        while pi < len(sched) and max(sched[pi][1]) < starts[j + 1]:
            fn, evs = sched[pi]
            pi += 1
            fn([functools.partial(event, e) for e in evs])
        post_fn(results[j])
    assert pi == len(sched)


def _pick(cnt, total, deps):
    if not deps:
        return None
    j, rem = divmod(cnt * len(deps), total)
    return j if rem < len(deps) else None


def _kernel(x_hbm, w1_hbm, w2_hbm, g_hbm, wf_hbm, wg_hbm, wo_hbm, out_hbm,
            v1, v2, spec_a, spec_b, y_a, y_b, hbuf, xbuf, w1buf, w2buf,
            gbuf, wfbuf, wgbuf, wobuf, gebuf, fbuf, febuf, obuf,
            sem_w, sem_s, sem_x, sem_o):
    plan = _PLAN
    n, hop, ns = plan.n, plan.hop, plan.ns
    specs, ys = (spec_a, spec_b), (y_a, y_b)

    xu = x_hbm.bitcast(jnp.uint32)
    c1_start = [int(v) for v in np.cumsum([0] + _C1)]

    def x_window(chunk, s):
        delta = (hop * c1_start[chunk]) % 8
        n0 = s * _S1 - _XOFF + hop * c1_start[chunk]
        rows = -(-(7 + hop * (_C1[chunk] - 1) + n) // 8) * 8
        src, dst = n0 - n0 % 8, s * _XSEG + 8 + delta - n0 % 8
        assert src % 8 == 0 and dst % 8 == 0 and dst + rows <= (s + 1) * _XSEG + 4
        return src, dst, rows

    def x_copies(chunk):
        cps = []
        for s in range(8):
            src, dst, rows = x_window(chunk, s)
            lo, hi = max(src, 0), min(src + rows, _T1)
            for cs in range(2):
                cps.append(pltpu.make_async_copy(
                    xu.at[:, pl.ds(lo, hi - lo), pl.ds(cs * 128, 128)],
                    xbuf.at[chunk % _XSLOTS, :, cs, pl.ds(dst + lo - src, hi - lo), :],
                    sem_x.at[chunk % _XSLOTS]))
        return cps

    def start_x(chunk):
        if chunk >= len(_C1):
            return
        zero8 = jnp.zeros((8, 128), jnp.uint32)
        for s in range(8):
            src, dst, rows = x_window(chunk, s)
            for r in range(0, rows, 8):
                if src + r < 0 or src + r >= _T1:
                    for bb in range(2):
                        for cs in range(2):
                            xbuf[chunk % _XSLOTS, bb, cs, pl.ds(dst + r, 8), :] = zero8
        for cp in x_copies(chunk):
            cp.start()

    def wait_x(chunk):
        if chunk < len(_C1):
            for cp in x_copies(chunk):
                cp.wait()

    w1_copies = [[pltpu.make_async_copy(w1_hbm.at[t], w1buf.at[t], sem_w.at[ph])
                  for t in range(1 - ph, _K, 2)] for ph in range(2)]
    wrows = _D // _WPARTS
    w2_copies = [pltpu.make_async_copy(w2_hbm.at[:, pl.ds(p * wrows, wrows), :],
                                       w2buf.at[:, pl.ds(p * wrows, wrows), :], sem_w.at[2 + p])
                 for p in range(_WPARTS)]
    small = [pltpu.make_async_copy(src, dst, sem_s.at[i]) for i, (src, dst) in
             enumerate([(g_hbm, gbuf), (wf_hbm, wfbuf), (wg_hbm, wgbuf), (wo_hbm, wobuf)])]

    for c in w1_copies[0]:
        c.start()
    zrow = jnp.zeros((8, 128), jnp.float32)
    for bb in range(2):
        for cs in range(2):
            for r in range(_NB1 * hop, _HROWS):
                hbuf[bb, cs, r] = zrow

    def w_unit(wbuf, vbuf, scale, row, half, ph, nt, deps=(), mask=None):
        cnt = [0]

        def load(tap):
            w = wbuf[tap, pl.ds(_dyn8(row + 8 * half), 8), pl.ds(nt * 128, 128)].astype(jnp.float32)
            j = _pick(cnt[0], 16, deps)
            cnt[0] += 1
            if j is not None:
                w = jnp.where(mask, w, deps[j]())
            return w * np.float32(scale)

        def emit(i, v):
            vbuf[i, 2 * ph + (row >> 7), nt, pl.ds(_dyn8((row & 127) >> 1) + 4 * half, 4), :] = (
                pltpu.bitcast(v.astype(jnp.bfloat16), jnp.uint32))
        plan.wprog[ph].run(plan.wouts[ph], load, emit)

    def fwd_unit(load_in, spec, row, col, deps, mask):
        cnt = [0]

        def load(q):
            j = _pick(cnt[0], n, deps)
            cnt[0] += 1
            return load_in(q, None if j is None else deps[j], mask)

        def emit(i, v):
            spec[col // 128, i, pl.ds(row, 8), :] = v
        plan.fwd.run(plan.fwd_outs, load, emit, keep_sign=False)

    def fx_unit(spec, chunk, be, bb, cs, ph, zd, deps=(), mask=None):
        slot = chunk & (_XSLOTS - 1)
        base = 8 + ((chunk * (_CB * hop)) & 7) + be * hop
        if ph == 1:
            base = base + zd

        def load_in(q, dep, mask):
            v = xbuf[slot, bb, cs, pl.ds(base + q, 8, stride=_XSEG), :]
            if dep is not None:
                v = jnp.where(mask, v, lax.bitcast_convert_type(dep(), jnp.uint32))
            v = (v << 16) if ph == 0 else (v & jnp.uint32(0xFFFF0000))
            return lax.bitcast_convert_type(v, jnp.float32)
        fwd_unit(load_in, spec, _dyn8(be * 16 + bb * 8), ph * 256 + cs * 128, deps, mask)

    def fh_unit(spec, blk, be, bb, cs, ph, deps=(), mask=None):
        base = blk * 2 * hop + ph

        def load_in(q, dep, mask):
            v = hbuf[bb, cs, base + 2 * q]
            if dep is not None:
                v = jnp.where(mask, v, dep())
            return v
        fwd_unit(load_in, spec, _dyn8(be * 16 + bb * 8), ph * 256 + cs * 128, deps, mask)

    def inv_unit(ybuf, dst, scale, blk, be, bb, nt, deps=(), mask=None):
        cnt = [0]
        row = _dyn8(be * 16 + bb * 8)

        def load(i):
            v = ybuf[nt, plan.inv_src[i], pl.ds(row, 8), :]
            j = _pick(cnt[0], ns, deps)
            cnt[0] += 1
            if j is not None:
                v = jnp.where(mask, v, deps[j]())
            return v

        def store(t, z):
            hval = _gelu2(z)
            if scale != 1.0:
                hval = hval * np.float32(scale)
            dst[bb, nt, blk * hop + t] = hval
        plan.inv.run(plan.inv_outs, load, store)

    def fx_units(spec, chunk, nblk, zd, mask):
        return [(_COST["fx"], functools.partial(fx_unit, spec, chunk, be, bb, cs, ph, zd, mask=mask))
                for be in range(nblk) for bb in range(2) for cs in range(2) for ph in range(2)]

    def fh_units(spec, blk0, nblk, mask):
        return [(_COST["fh"], functools.partial(fh_unit, spec, blk0 + be, be, bb, cs, ph, mask=mask))
                for be in range(nblk) for bb in range(2) for cs in range(2) for ph in range(2)]

    def inv_units(ybuf, dst, scale, blk0, nblk, mask):
        return [(_COST["inv"], functools.partial(inv_unit, ybuf, dst, scale, blk0 + be, be, bb, nt, mask=mask))
                for be in range(nblk) for bb in range(2) for nt in range(2)]

    def w2_units(rg0, nrg, mask):
        return [(_COST["w"], functools.partial(
                    w_unit, w2buf, v2, (2.0 / n) * 0.5, pl.multiple_of((rg0 + r) * 16, 16)
                    if not isinstance(rg0, int) else (rg0 + r) * 16, half, ph, nt, mask=mask))
                for r in range(nrg) for half in range(2) for ph in range(2) for nt in range(2)]

    def conv_items(vbuf, spec, ybuf, m, only=None):
        items = []
        for i in range(ns):
            hold = []

            def dot_fn(i=i, h=0):
                w = jnp.concatenate(
                    [jnp.concatenate(
                        [pltpu.bitcast(vbuf[i, 2 * h + q, nt, pl.ds(0, 64), :], jnp.bfloat16)
                         for q in range(2)], axis=0) for nt in range(2)], axis=1)
                lhs = jnp.concatenate([spec[2 * h + q, i, pl.ds(0, m), :] for q in range(2)], axis=1)
                return jnp.dot(lhs, w, preferred_element_type=jnp.float32)

            def post0(r, hold=hold):
                hold.append(r)

            def post1(r, i=i, hold=hold):
                y = hold[0] + r
                for nt in range(2):
                    ybuf[nt, i, pl.ds(0, m), :] = y[:, nt * 128:(nt + 1) * 128]
            def post_first(r, i=i):
                for nt in range(2):
                    ybuf[nt, i, pl.ds(0, m), :] = r[:, nt * 128:(nt + 1) * 128]

            def post_second(r, i=i):
                for nt in range(2):
                    ybuf[nt, i, pl.ds(0, m), :] = (
                        ybuf[nt, i, pl.ds(0, m), :] + r[:, nt * 128:(nt + 1) * 128])
            if only is None:
                items.append((m, functools.partial(dot_fn, i, 0), post0))
                items.append((m, functools.partial(dot_fn, i, 1), post1))
            else:
                items.append((m, functools.partial(dot_fn, i, only),
                              post_second if only else post_first))
        return items

    def block(fn, zd):
        def body(_, c):
            fn()
            return c
        lax.fori_loop(0, 1 + zd, body, 0)

    def opaque_zero(i):
        return (i * (i + 1)) & 1

    def true_mask(zd):
        return jnp.full((8, 128), zd, jnp.int32) == 0

    start_x(0)
    for c in w1_copies[0]:
        c.wait()
    for c in w1_copies[1]:
        c.start()

    def v1_body(i, carry):
        for r in range(2):
            row = pl.multiple_of((2 * i + r) * 16, 16)
            for half in range(2):
                for nt in range(2):
                    w_unit(w1buf, v1, (2.0 / n) * _C0, row, half, 0, nt)
        return carry
    lax.fori_loop(0, _D // 32, v1_body, 0)

    zd0 = opaque_zero(hbuf[0, 0, _HROWS - 1, 0, 0].astype(jnp.int32))
    mask0 = true_mask(zd0)

    wait_x(0)
    start_x(1)
    w2_copies[0].start()
    start_x(2)

    def fill_body(u, carry):
        zd = opaque_zero(u)
        for cs in range(2):
            for ph in range(2):
                fx_unit(spec_a, 0, u >> 1, u & 1, cs, ph, zd)
        return carry
    lax.fori_loop(0, _C1[0] * 2, fill_body, 0)

    for c in w1_copies[1]:
        c.wait()

    def step0a_body():
        units = [(_COST["w"], functools.partial(w_unit, w1buf, v1, (2.0 / n) * _C0, rg * 16,
                                                half, 1, nt, mask=mask0))
                 for rg in range(_D // 16) for half in range(2) for nt in range(2)]
        _emit_step(conv_items(v1, spec_a, y_a, _CB * 16, only=0), units, mask0)
    block(step0a_body, zd0)

    wait_x(1)
    start_x(3)

    def step0b_body():
        _emit_step(conv_items(v1, spec_a, y_a, _CB * 16, only=1),
                   fx_units(spec_b, 1, _CB, zd0, mask0), mask0)
    block(step0b_body, zd0)

    def before_step(c):
        wait_x(c + 1)
        start_x(c + 3)
        for p, first_use in enumerate((1, 5, 9, 11)):
            if c == first_use:
                w2_copies[p].wait()
            if p > 0 and c == first_use - 2:
                w2_copies[p].start()
        if c == 8:
            for cp in small:
                cp.start()

    def conv1_body(it, carry):
        zd = opaque_zero(it)
        mask = true_mask(zd)
        for par in (1, 0):
            c = 2 * it + (1 if par == 1 else 2)
            for k in range(4):
                pl.when(it == k)(functools.partial(before_step, 2 * k + (1 if par == 1 else 2)))
            block(lambda: _emit_step(
                conv_items(v1, specs[par], ys[par], _CB * 16),
                _merge(fx_units(specs[1 - par], c + 1, _CB, zd, mask) +
                       inv_units(ys[1 - par], hbuf, 1.0, (c - 1) * _CB, _CB, mask),
                       w2_units(c - 1, 1, mask)), mask), zd)
        return carry
    lax.fori_loop(0, 4, conv1_body, 0)

    sub = lax.broadcasted_iota(jnp.int32, (8, 128), 0)

    def mask_rows(r0, r1, s):
        def body(r, carry):
            for bb in range(2):
                for cs in range(2):
                    hbuf[bb, cs, r] = jnp.where(sub == s, 0.0, hbuf[bb, cs, r])
            return carry
        lax.fori_loop(r0, r1, body, 0)
    mask_rows(0, 16, 0)

    for c in (9, 10):
        par = c % 2
        before_step(c)
        block(lambda: _emit_step(
            conv_items(v1, specs[par], ys[par], _CB * 16),
            _merge(fx_units(specs[1 - par], c + 1, _C1[c + 1], zd0, mask0) +
                   inv_units(ys[1 - par], hbuf, 1.0, c1_start[c - 1], _CB, mask0),
                   w2_units(8 + 2 * (c - 9), 2, mask0)), mask0), zd0)

    before_step(11)

    def step11_body():
        _emit_step(conv_items(v1, spec_b, y_b, _C1[11] * 16),
                   _merge(fh_units(spec_a, 0, _CB2, mask0) +
                          inv_units(y_a, hbuf, 1.0, c1_start[10], _CB, mask0),
                          w2_units(12, 4, mask0)), mask0)
    block(step11_body, zd0)

    fscale = 0.5 / _C0

    def step8_body():
        zd, mask = zd0, mask0
        _emit_step(conv_items(v2, spec_a, y_a, _CB2 * 16),
                   fh_units(spec_b, _CB2, _CB2, mask) +
                   inv_units(y_b, hbuf, 1.0, c1_start[11], _C1[11], mask), mask)
    block(step8_body, zd0)
    mask_rows(_T1 - 7 * _S1 + 16, _NB1 * hop, 7)

    def conv2_body(it, carry):
        zd = opaque_zero(it)
        mask = true_mask(zd)
        for par in (1, 0):
            c = 2 * it + (1 if par == 1 else 2)
            block(lambda: _emit_step(
                conv_items(v2, specs[par], ys[par], _CB2 * 16),
                (fh_units(specs[1 - par], (c + 1) * _CB2, _CB2, mask) +
                 inv_units(ys[1 - par], fbuf, fscale, (c - 1) * _CB2, _CB2, mask)),
                mask), zd)
        return carry
    lax.fori_loop(0, 2, conv2_body, 0)

    for c in small:
        c.wait()
    gebuf[...] = jnp.dot(gbuf[...].reshape(_B * _U, _D), wgbuf[...],
                         preferred_element_type=jnp.float32).reshape(_B, _U, _D)

    def fe_item(slot, tile):
        def dot_fn():
            f = jnp.concatenate(
                [jnp.concatenate(
                    [fbuf[bb, cs, pl.ds(tile * _TJ, _TJ)].reshape(_TJ * 8, 128) for cs in range(2)],
                    axis=1) for bb in range(2)], axis=0)
            return jnp.dot(f, wfbuf[...], preferred_element_type=jnp.float32)

        def post(r):
            febuf[slot] = r.reshape(_B, _TJ, 8, _D)
        return (_TJ * 16, dot_fn, post)

    def step13_body():
        zd, mask = zd0, mask0
        _emit_step(conv_items(v2, spec_b, y_b, _CB2 * 16) + [fe_item(0, 0)],
                   inv_units(y_a, fbuf, fscale, 4 * _CB2, _CB2, mask), mask)
    block(step13_body, zd0)

    def out_copies(slot, t0, rows_of):
        cps = []
        for s in range(8):
            rows = rows_of(s)
            if rows > 0:
                cps.append(pltpu.make_async_copy(
                    obuf.at[slot, :, s, pl.ds(0, rows)],
                    out_hbm.at[:, pl.ds(s * _S2 + t0, rows)],
                    sem_o.at[slot]))
        return cps

    def joint_item(fslot, oslot, tj):
        def dot_fn():
            rows = []
            for tt in range(tj):
                for r in range(16):
                    fr = febuf[fslot, r // 8, tt, pl.ds(r % 8, 1), :]
                    rows.append(jnp.tanh(jnp.broadcast_to(fr, (_U, _D)) + gebuf[r // 8]))
            return jnp.dot(jnp.concatenate(rows, axis=0), wobuf[...],
                           preferred_element_type=jnp.float32)

        def post(o):
            o = o.reshape(tj, _B, 8, _U, _D).astype(jnp.bfloat16)
            for tt in range(tj):
                obuf[oslot, :, :, tt] = o[tt]
        return (tj * 16 * _U, dot_fn, post)

    full = lambda s: _TJ
    ntiles = -(-_S2 // _TJ)
    nfull = (_T2 - 7 * _S2) // _TJ
    assert nfull % _OSLOTS == 0 and _OSLOTS == 4

    def first_body():
        _emit_step([fe_item(1, 1), joint_item(0, 0, _TJ), fe_item(0, 2), joint_item(1, 1, _TJ)],
                   inv_units(y_b, fbuf, fscale, 5 * _CB2, _CB2, mask0), mask0)
        for slot in range(2):
            for c in out_copies(slot, slot * _TJ, full):
                c.start()
    block(first_body, zd0)

    def joint_body(i2, carry):
        @pl.when(i2 >= 2)
        def _():
            for j in range(2):
                for c in out_copies((i2 & 1) * 2 + j, (2 * i2 + j - _OSLOTS) * _TJ, full):
                    c.wait()
        for j in range(2):
            tile = 2 * i2 + j
            oslot = (i2 & 1) * 2 + j
            _emit_step([fe_item(1 - j, tile + 1), joint_item(j, oslot, _TJ)], [], None)
            for c in out_copies(oslot, tile * _TJ, full):
                c.start()
        return carry
    lax.fori_loop(1, nfull // 2, joint_body, 0)

    pending = {k: out_copies(k, (nfull - _OSLOTS + k) * _TJ, full) for k in range(_OSLOTS)}
    for tile in range(nfull, ntiles):
        oslot, t0 = tile % _OSLOTS, tile * _TJ
        tj = min(_TJ, _S2 - t0)
        rows_of = lambda s, t0=t0, tj=tj: max(0, min(tj, (_T2 - 7 * _S2 if s == 7 else _S2) - t0))
        for c in pending[oslot]:
            c.wait()
        items = ([fe_item(1 - tile % 2, tile + 1)] if tile + 1 < ntiles else []) + [
            joint_item(tile % 2, oslot, tj)]
        _emit_step(items, [], None)
        pending[oslot] = out_copies(oslot, t0, rows_of)
        for c in pending[oslot]:
            c.start()
    for k in range(_OSLOTS):
        for c in pending[k]:
            c.wait()


@jax.jit
def pallas_standalone__seq2seq_rnn_t_joint__speech_kernel(
    x: jax.Array,
    w1: jax.Array,
    w2: jax.Array,
    g: jax.Array,
    w_f: jax.Array,
    w_g: jax.Array,
    w_o: jax.Array,
):
    assert x.shape == (_B, _T, _D) and w1.shape == (_K, _D, _D) and w2.shape == (_K, _D, _D)
    assert g.shape == (_B, _U, _D)
    bf, f32 = jnp.bfloat16, jnp.float32
    m = max(_C1 + [_CB2]) * 16
    scratch = [
        pltpu.VMEM((_NS, 4, 2, 72, 128), jnp.uint32),
        pltpu.VMEM((_NS, 4, 2, 72, 128), jnp.uint32),
        pltpu.VMEM((4, _NS, m + 8, 128), f32),
        pltpu.VMEM((4, _NS, m + 8, 128), f32),
        pltpu.VMEM((2, _NS, m + 8, 128), f32),
        pltpu.VMEM((2, _NS, m + 8, 128), f32),
        pltpu.VMEM((2, 2, _HROWS + 1, 8, 128), f32),
        pltpu.VMEM((_XSLOTS, 2, 2, 8 * _XSEG + 8, 128), jnp.uint32),
        pltpu.VMEM((_K, _D, _D), bf),
        pltpu.VMEM((_K, _D, _D), bf),
        pltpu.VMEM((_B, _U, _D), bf),
        pltpu.VMEM((_D, _D), bf),
        pltpu.VMEM((_D, _D), bf),
        pltpu.VMEM((_D, _D), bf),
        pltpu.VMEM((_B, _U, _D), f32),
        pltpu.VMEM((2, 2, _FROWS + 1, 8, 128), f32),
        pltpu.VMEM((2, _B, _TJ, 8, _D), f32),
        pltpu.VMEM((_OSLOTS, _B, 8, _TJ, _U, _D), bf),
        pltpu.SemaphoreType.DMA((_WPARTS + 2,)),
        pltpu.SemaphoreType.DMA((4,)),
        pltpu.SemaphoreType.DMA((_XSLOTS,)),
        pltpu.SemaphoreType.DMA((_OSLOTS,)),
    ]
    any_spec = pl.BlockSpec(memory_space=pl.ANY)
    return pl.pallas_call(
        _kernel,
        out_shape=jax.ShapeDtypeStruct((_B, _T2, _U, _D), bf),
        in_specs=[any_spec] * 7,
        out_specs=any_spec,
        scratch_shapes=scratch,
        compiler_params=pltpu.CompilerParams(vmem_limit_bytes=127 * 1024 * 1024),
    )(x, w1, w2, g, w_f, w_g, w_o)
```
